```python
import jax
import jax.numpy as jnp

def _softmax(x, axis=-1):
    return jax.nn.softmax(x, axis=axis)
def _gelu(x):
    return jax.nn.gelu(x, approximate=True)
def _silu(x):
    return jax.nn.silu(x)
def _sigmoid(x):
    return jax.nn.sigmoid(x)
def _layernorm(x, axis=-1, eps=1e-5):
    m = jnp.mean(x, axis=axis, keepdims=True)
    v = jnp.var(x, axis=axis, keepdims=True)
    return (x - m) / jnp.sqrt(v + eps)
def _scatter_add(tgt, idx, src, axis=0):
    return tgt.at[idx].add(src)
def _segment_sum(src, seg, n):
    return jax.ops.segment_sum(src, seg, n)
class _Rng:
    def __init__(self, key):
        self._k = key
    def _next(self):
        self._k, sub = jax.random.split(self._k)
        return sub
    def normal(self, shape):
        return jax.random.normal(self._next(), shape, dtype=jnp.bfloat16)
    def randint(self, lo, hi, shape):
        return jax.random.randint(self._next(), shape, lo, hi, dtype=jnp.int32)
    def uniform(self, shape, lo=0.0, hi=1.0):
        return jax.random.uniform(self._next(), shape, jnp.bfloat16, lo, hi)
    def permutation(self, n):
        return jax.random.permutation(self._next(), n)


kernel_name = 'standalone__adm_resblock__diffusion'

def setup_inputs():
    _rng = _Rng(jax.random.key(int.from_bytes(__import__("os").urandom(4), "little")))
    _w = (lambda a: (lambda t: t.astype(jnp.bfloat16) if jnp.issubdtype(t.dtype, jnp.floating) else t)(jnp.asarray(a)))
    B, C, HW, E = 2, 512, 64, 1152
    sc = (9.0 * C) ** -0.5
    return {
        "x": _w((lambda *s: _rng.normal(s) * 0.05)(B, C, HW, HW)),
        "t_emb": _w((lambda *s: _rng.normal(s) * 0.05)(B, E)),
        "g1": _w(1.0 + 0.1 * (lambda *s: _rng.normal(s) * 0.05)(C)),
        "be1": _w(0.1 * (lambda *s: _rng.normal(s) * 0.05)(C)),
        "w1": _w((lambda *s: _rng.normal(s) * 0.05)(C, C, 3, 3) * sc),
        "w_emb": _w((lambda *s: _rng.normal(s) * 0.05)(E, C) * (E ** -0.5)),
        "g2": _w(1.0 + 0.1 * (lambda *s: _rng.normal(s) * 0.05)(C)),
        "be2": _w(0.1 * (lambda *s: _rng.normal(s) * 0.05)(C)),
        "w2": _w((lambda *s: _rng.normal(s) * 0.05)(C, C, 3, 3) * sc),
    }

def reference(x, t_emb, g1, be1, w1, w_emb, g2, be2, w2):
    B, C, H, W = x.shape
    G, eps = 4, 1e-5
    def gn(z, gamma, beta):
        zr = z.reshape(B, G, (C // G) * H * W)
        mu = zr.mean(-1).reshape(B, G, 1)
        var = ((zr - mu) ** 2).mean(-1).reshape(B, G, 1)
        zn = ((zr - mu) / jnp.sqrt(var + eps)).reshape(B, C, H, W)
        return zn * gamma.reshape(1, C, 1, 1) + beta.reshape(1, C, 1, 1)
    def conv3(z, w):
        zp = jnp.pad(z, ((0, 0), (0, 0), (1, 1), (1, 1)))
        taps = [jnp.einsum("bchw,oc->bohw", zp[:, :, i:i+H, j:j+W], w[:, :, i, j]) for i in range(3) for j in range(3)]
        out = taps[0]
        for t in taps[1:]:
            out = out + t
        return out
    h = conv3(_silu(gn(x, g1, be1)), w1)
    emb = _silu(t_emb) @ w_emb
    h = h + emb.reshape(B, C, 1, 1)
    h = conv3(_silu(gn(h, g2, be2)), w2)
    return x + h
```

```python
import itertools

import jax
import jax.numpy as jnp
from jax import lax
import jax.experimental.pallas as pl
import jax.experimental.pallas.tpu as pltpu

F32 = jnp.float32
BF16 = jnp.bfloat16
U32 = jnp.uint32

PA = 2.0 / 3.0
PB = 1.5
A2, B2 = PA * PA, PB * PB
NA = 1.0 / (2 * A2 * (A2 - B2))
NB = 1.0 / (2 * B2 * (B2 - A2))
RT = PB / PA
GS = PA ** 3

TPOS = (0, 24, 32, 40, 48, 56, 64, 16)
TREC = 72
MROW = 264
MSLOT = 36 * MROW
K_A2, K_B2, K_SHIFT, K_MASK, K_SCALE = (i * MROW + 256 for i in range(5))


def _bt(d0, d1, d2, d3, d4, d5, a2=A2, b2=B2):
    t, u = a2 * d2, b2 * d2
    ea, eb = d4 - u, d4 - t
    v0 = ea - t
    if d0 is not None:
        v0 = v0 + d0
    t3, u3 = a2 * d3, b2 * d3
    pa, pb = t3 - d1, u3 - d1
    v5 = (d5 - pa) - u3 if d5 is not None else (d1 - t3) - u3
    oa, ob = PB * pa, PA * pb
    return v0, ea + oa, ea - oa, eb + ob, eb - ob, v5


def _at(m0, m1, m2, m3, m4, m5):
    sa, ta, sb, tb = m1 + m2, m1 - m2, m3 + m4, m3 - m4
    return (m0 + sa) + sb, ta + RT * tb, sa + (RT * RT) * sb, (ta + m5) + (RT * RT * RT) * tb


def _gt(g0, g1, g2, k):
    ea, oa = (k * NA) * g0 + (k * NA * A2) * g2, (k * NA * PA) * g1
    eb, ob = (k * NB) * g0 + (k * NB * B2) * g2, (k * NB * PB) * g1
    k5 = k / PA ** 3
    u0 = g0 if abs(k - 1.0) < 1e-12 else k * g0
    u5 = g2 if abs(k5 - 1.0) < 1e-12 else k5 * g2
    return u0, ea + oa, ea - oa, eb + ob, eb - ob, u5


def _pack(lo, hi):
    return pltpu.pack_elementwise([lo, hi], packed_dtype=BF16)


def _unpack(w, i):
    return pltpu.unpack_elementwise(w, index=i, packed_dtype=BF16, unpacked_dtype=F32)


def _tree(xs):
    while len(xs) > 1:
        xs = [xs[i] + xs[i + 1] for i in range(0, len(xs), 2)]
    return xs[0]


def _acc(a, x):
    return x if a is None else a + x


class _Rows:
    def __init__(self, ref, base=0):
        self.ref, self.base = ref, base

    def ld(self, off, n=8, stride=1):
        return self.ref[pl.ds(self.base + off, n, stride=stride), :]

    def st(self, off, val, stride=1):
        self.ref[pl.ds(self.base + off, val.shape[0], stride=stride), :] = val


def _splitter(const):
    sh = lax.bitcast_convert_type(const.ld(K_SHIFT), U32)
    mk = lax.bitcast_convert_type(const.ld(K_MASK), U32)
    return lambda w: (lax.bitcast_convert_type(w << sh, F32), lax.bitcast_convert_type(w & mk, F32))


def _job_u(w, u, const):
    def gen():
        for r in range(0, 64, 8):
            def taps(rows):
                split = _splitter(const)
                return [list(zip(*[split(w.ld((3 * i + j) * 64 + r)) for j in range(3)])) for i in rows]

            def emit(i, row, k):
                lo, hi = _gt(*row[0], k), _gt(*row[1], k)
                for j in range(6):
                    u.st((i * 6 + j) * 64 + r, _pack(lo[j], hi[j]))

            emit(0, taps([0])[0], GS)
            yield 38
            emit(5, taps([2])[0], 1.0)
            yield 38
            for i, nn, p in ((1, NA, PA), (3, NB, PB)):
                g0, g1, g2 = taps([0, 1, 2])
                e = [[nn * g0[h][j] + (nn * p * p) * g2[h][j] for j in range(3)] for h in range(2)]
                o = [[(nn * p) * g1[h][j] for j in range(3)] for h in range(2)]
                emit(i, [[e[h][j] + o[h][j] for j in range(3)] for h in range(2)], GS)
                emit(i + 1, [[e[h][j] - o[h][j] for j in range(3)] for h in range(2)], GS)
                yield 118

    return gen(), 8 * 312


def _gn_coeffs(s, q, e, gamma, beta, ab):
    s = jnp.sum(s, axis=0, keepdims=True) * (1.0 / 4096)
    q = jnp.sum(q, axis=0, keepdims=True) * (1.0 / 4096)
    var_c = jnp.maximum(q - s * s, 0.0)
    mean_c = s if e is None else s + e
    mu = jnp.sum(mean_c, axis=1, keepdims=True) * (1.0 / 128)
    dm = mean_c - mu
    var = jnp.sum(var_c + dm * dm, axis=1, keepdims=True) * (1.0 / 128)
    a = 0.5 * gamma * lax.rsqrt(var + 1e-5)
    b = 0.5 * beta + a * (-mu if e is None else e - mu)
    ab.st(0, jnp.broadcast_to(a, (8, 128)))
    ab.st(8, jnp.broadcast_to(b, (8, 128)))


def _job_c0(x, h, gamma, beta, ab, const):
    def gen():
        s = q = None
        for y in range(64):
            split = _splitter(const)
            vals = []
            for k in range(2):
                for sub in range(2):
                    for i, v in enumerate(split(x.ld(y * 32 + sub * 16 + k, 8, 2))):
                        h.st(y * 64 + (2 * k + i) * 16 + sub * 8, v)
                        vals.append(v)
            s = _acc(s, _tree(vals))
            q = _acc(q, _tree([v * v for v in vals]))
            yield 32
        _gn_coeffs(s, q, None, gamma[...], beta[...], ab)
        yield 40

    return gen(), 64 * 32 + 40


def _job_a(h, ab, t, v, const):
    def gen():
        const.st(K_SCALE, ab.ld(0))
        b = ab.ld(8)

        def act(y, q, a):
            if y > 63:
                return None
            u = h.ld(y * 64 + (q % 4) * 16 + q // 4, 8, 2) * a + b
            return u * jnp.tanh(u) + u

        for q in range(8):
            d4, d5 = None, act(0, q, const.ld(K_SCALE))
            for ty in range(16):
                a = const.ld(K_SCALE)
                d0, d1 = d4, d5
                d2, d3, d4, d5 = (act(4 * ty + k, q, a) for k in range(1, 5))
                for i, val in enumerate(_bt(d0, d1, d2, d3, d4, d5)):
                    t.st((ty * 6 + i) * TREC + TPOS[q], val)
                yield 34
        for ty in range(16):
            for i in range(6):
                offs = (TPOS[7] - 1,) + TPOS + (TPOS[0] + 1,)
                d = [t.ld((ty * 6 + i) * TREC + o) for o in offs]
                a2, b2 = const.ld(K_A2), const.ld(K_B2)
                for j, (lo, hi) in enumerate(zip(_bt(*d[0:6], a2, b2), _bt(*d[4:10], a2, b2))):
                    v.st((i * 6 + j) * 128 + ty * 8, _pack(lo, hi))
                yield 42

    return gen(), 128 * 34 + 96 * 42


def _tiles_out(m, r0, finish, cost):
    def row(i):
        return _at(*[m.ld((i * 6 + j) * MROW + r0) for j in range(6)])

    def done(i, ys):
        finish(i, [y if i + j == 3 else (PA ** (i + j) / GS) * y for j, y in enumerate(ys)])

    r1 = row(1)
    yield 13
    r2 = row(2)
    sa, ta = [x + y for x, y in zip(r1, r2)], [x - y for x, y in zip(r1, r2)]
    yield 21
    r3 = row(3)
    yield 13
    r4 = row(4)
    sb, tb = [x + y for x, y in zip(r3, r4)], [x - y for x, y in zip(r3, r4)]
    done(1, [x + RT * y for x, y in zip(ta, tb)])
    yield 32 + cost
    done(2, [x + (RT * RT) * y for x, y in zip(sa, sb)])
    done(0, [(x + y) + w for x, y, w in zip(sa, sb, row(0))])
    yield 35 + 2 * cost
    done(3, [(x + (RT * RT * RT) * y) + w for x, y, w in zip(ta, tb, row(5))])
    yield 28 + cost


def _job_c1(m, h, e, gamma, beta, ab):
    def gen():
        sq = [None, None]
        for ty in range(16):
            for sub in range(2):
                def finish(i, ys):
                    sq[0] = _acc(sq[0], _tree(ys))
                    sq[1] = _acc(sq[1], _tree([y * y for y in ys]))
                    for j in range(4):
                        h.st((4 * ty + i) * 64 + j * 16 + sub * 8, ys[j])

                yield from _tiles_out(m, ty * 16 + sub * 8, finish, 12)
        _gn_coeffs(sq[0], sq[1], e[...], gamma[...], beta[...], ab)
        yield 40

    return gen(), 32 * (142 + 48) + 40


def _job_c2(m, x):
    def gen():
        for ty in range(16):
            for sub in range(2):
                def finish(i, ys):
                    for k in range(2):
                        off = (4 * ty + i) * 32 + sub * 16 + k
                        w = x.ld(off, 8, 2)
                        x.st(off, _pack(_unpack(w, 0) + ys[2 * k], _unpack(w, 1) + ys[2 * k + 1]), 2)

                yield from _tiles_out(m, ty * 16 + sub * 8, finish, 10)

    return gen(), 32 * (142 + 40)


def _run(*jobs):
    for gen, _ in jobs:
        for _ in gen:
            pass


def _step(v, u, m, jobs, rows=16, lead=8, tail=0):
    total = sum(c for _, c in jobs)
    pieces = itertools.chain(*[g for g, _ in jobs])
    span = 36 * 256 // rows + lead - tail
    spent = 0

    def advance(limit):
        nonlocal spent
        while spent < limit:
            cost = next(pieces, None)
            if cost is None:
                return
            spent += cost

    tick = lead
    advance(total * tick / span)
    for xi in range(36):
        lhs = jnp.concatenate([pltpu.bitcast(r.ld(xi * 128, 128), BF16) for r in v], axis=1)
        rhs = jnp.concatenate([pltpu.bitcast(r.ld(xi * 64, 64), BF16) for r in u], axis=1)
        res = lax.dot_general(lhs, rhs, (((1,), (1,)), ((), ())), preferred_element_type=F32)
        for r in range(0, 256, rows):
            m.st(xi * MROW + r, res[r:r + rows])
            tick += 1
            advance(total * tick / span)
    advance(float("inf"))


def _kernel(x_hbm, t_ref, g1_ref, be1_ref, w1_hbm, we_hbm, g2_ref, be2_ref, w2_hbm, o_hbm,
            xbuf, wbuf, webuf, hbuf, abuf, tbuf, v0, v1, u1, u2, mbuf, par, emb, slots,
            xsem, wsem, esem, osem):
    x32 = xbuf.bitcast(U32)
    w32 = wbuf.bitcast(U32)

    def lanes(g):
        return pl.ds(g * 128 if isinstance(g, int) else pl.multiple_of(g * 128, 128), 128)

    def x_copy(j):
        return pltpu.make_async_copy(x_hbm.at[j // 4, :, lanes(j % 4)], xbuf.at[j], xsem.at[j])

    def o_copy(j):
        return pltpu.make_async_copy(xbuf.at[j], o_hbm.at[j // 4, :, lanes(j % 4)], osem.at[j])

    def w_copy(conv, k):
        src = (w1_hbm, w2_hbm)[conv]
        return pltpu.make_async_copy(
            src.at[:, lanes(k // 4), lanes(k % 4)], wbuf.at[conv * 16 + k], wsem.at[conv * 16 + k])

    e_copy = pltpu.make_async_copy(we_hbm, webuf, esem.at[0])

    for k in range(4):
        w_copy(0, k).start()
    for j in range(4):
        x_copy(j).start()
    for k in range(4, 12):
        w_copy(0, k).start()

    slots[0] = 0
    slots[1] = MSLOT
    t = _Rows(tbuf)
    for r in range(96):
        t.st(r * TREC + 8, jnp.zeros((8, 128), F32))
    for base in (0, MSLOT):
        c = _Rows(mbuf, base)
        c.st(K_A2, jnp.full((8, 128), A2, F32))
        c.st(K_B2, jnp.full((8, 128), B2, F32))
        c.st(K_SHIFT, lax.bitcast_convert_type(jnp.full((8, 128), 16, U32), F32))
        c.st(K_MASK, lax.bitcast_convert_type(jnp.full((8, 128), 0xFFFF0000, U32), F32))
    for k, ref in enumerate((g1_ref, be1_ref, g2_ref, be2_ref)):
        val = ref[...].astype(F32).reshape(4, 128)
        for g in range(4):
            par[k * 4 + g] = val[g:g + 1]

    def m_slot(s):
        return _Rows(mbuf, pl.multiple_of(slots[s % 2], 8))

    def h_slot(j):
        return _Rows(hbuf, j * 4096)

    def ab_slot(j):
        return _Rows(abuf, j * 16)

    def job_u(conv, k, const):
        w = w32.at[conv * 16 + k]
        taps = type("Taps", (), {"ld": staticmethod(lambda off: w[off // 64, pl.ds(off % 64, 8), :])})
        return _job_u(taps, _Rows((u1, u2)[conv].at[k]), const)

    def job_c0(j, const):
        return _job_c0(_Rows(x32.at[j]), h_slot(j), par.at[j % 4], par.at[4 + j % 4], ab_slot(j), const)

    def job_a(j, v, const):
        return _job_a(h_slot(j), ab_slot(j), t, _Rows(v.at[j % 4]), const)

    def job_c1(j, m):
        return _job_c1(m, h_slot(j), emb.at[j], par.at[8 + j % 4], par.at[12 + j % 4], ab_slot(j))

    def job_c2(j, m):
        return _job_c2(m, _Rows(x32.at[j]))

    def step(s, v, u, jobs):
        _step([_Rows(v.at[g]) for g in range(4)], [_Rows(u.at[(s % 4) * 4 + g]) for g in range(4)],
              m_slot(s), jobs)

    const0 = _Rows(mbuf)

    @pl.loop(0, 4)
    def _(k):
        w_copy(0, k).wait()
        _run(job_u(0, k, const0))

    @pl.loop(0, 4)
    def _(j):
        x_copy(j).wait()
        x_copy(j + 4).start()
        w_copy(0, j + 12).start()
        _run(job_c0(j, const0), job_a(j, v0, const0))

    e_copy.start()
    for k in range(4, 12):
        w_copy(0, k).wait()
    prev = m_slot(1)
    step(0, v0, u1, [job_u(0, k, prev) for k in range(4, 12)])

    for k in range(4):
        x_copy(k + 4).wait()
        w_copy(0, k + 12).wait()
    e_copy.wait()
    for k in range(16):
        w_copy(1, k).start()
    th = t_ref[...].astype(F32) * 0.5
    e = jnp.dot((th * jnp.tanh(th) + th).astype(BF16), webuf[...], preferred_element_type=F32)
    for j in range(8):
        emb[j] = e[j // 4:j // 4 + 1, (j % 4) * 128:(j % 4 + 1) * 128]
    prev = m_slot(0)
    step(1, v0, u1, [job_c1(0, prev)] + [job_c0(j, prev) for j in range(4, 8)]
         + [job_u(0, k, prev) for k in range(12, 16)])

    @pl.loop(2, 4)
    def _(s):
        prev = m_slot(s + 1)
        step(s, v0, u1, [job_c1(s - 1, prev), job_a(2 * s, v1, prev), job_a(2 * s + 1, v1, prev)])

    for k in range(16):
        w_copy(1, k).wait()

    @pl.loop(4, 8)
    def _(s):
        prev = m_slot(s + 1)
        step(s, v1, u1, [job_c1(s - 1, prev)] + [job_u(1, 3 * (s - 4) + k, prev) for k in range(3)]
             + [job_a(s - 4, v0, prev)])

    prev = m_slot(1)
    step(8, v0, u2, [job_c1(7, prev)] + [job_u(1, k, prev) for k in range(12, 16)] + [job_a(4, v1, prev)])

    @pl.loop(9, 12)
    def _(s):
        prev = m_slot(s + 1)
        step(s, v0, u2, [job_c2(s - 9, prev), job_a(s - 4, v1, prev)])
        o_copy(s - 9).start()

    @pl.loop(12, 16)
    def _(s):
        prev = m_slot(s + 1)
        step(s, v1, u2, [job_c2(s - 9, prev)])
        o_copy(s - 9).start()

    _run(job_c2(7, _Rows(mbuf, MSLOT)))
    o_copy(7).start()
    for j in range(8):
        o_copy(j).wait()


@jax.jit
def pallas_standalone__adm_resblock__diffusion_kernel(
    x: jax.Array,
    t_emb: jax.Array,
    g1: jax.Array,
    be1: jax.Array,
    w1: jax.Array,
    w_emb: jax.Array,
    g2: jax.Array,
    be2: jax.Array,
    w2: jax.Array,
):
    B, C, H, W = x.shape
    assert (B, C, H, W) == (2, 512, 64, 64)
    xt = jnp.transpose(x, (0, 2, 3, 1)).reshape(B, H * W, C)
    w1t = jnp.transpose(w1, (2, 3, 0, 1)).reshape(9, C, C)
    w2t = jnp.transpose(w2, (2, 3, 0, 1)).reshape(9, C, C)
    hbm = pl.BlockSpec(memory_space=pl.ANY)
    vmem = pl.BlockSpec(memory_space=pltpu.VMEM)
    out = pl.pallas_call(
        _kernel,
        out_shape=jax.ShapeDtypeStruct((B, H * W, C), x.dtype),
        in_specs=[hbm, vmem, vmem, vmem, hbm, hbm, vmem, vmem, hbm],
        out_specs=hbm,
        scratch_shapes=[
            pltpu.VMEM((8, 4096, 128), BF16),
            pltpu.VMEM((32, 9, 128, 128), BF16),
            pltpu.VMEM(w_emb.shape, BF16),
            pltpu.VMEM((8 * 4096, 128), F32),
            pltpu.VMEM((8 * 16, 128), F32),
            pltpu.VMEM((96 * TREC, 128), F32),
            pltpu.VMEM((4, 36 * 128, 128), U32),
            pltpu.VMEM((4, 36 * 128, 128), U32),
            pltpu.VMEM((16, 36 * 64, 128), U32),
            pltpu.VMEM((16, 36 * 64, 128), U32),
            pltpu.VMEM((2 * MSLOT, 128), F32),
            pltpu.VMEM((16, 1, 128), F32),
            pltpu.VMEM((8, 1, 128), F32),
            pltpu.SMEM((2,), jnp.int32),
            pltpu.SemaphoreType.DMA((8,)),
            pltpu.SemaphoreType.DMA((32,)),
            pltpu.SemaphoreType.DMA((1,)),
            pltpu.SemaphoreType.DMA((8,)),
        ],
        compiler_params=pltpu.CompilerParams(vmem_limit_bytes=120 * 2**20),
        name="resblk",
    )(xt, t_emb, g1, be1, w1t, w_emb, g2, be2, w2t)
    return jnp.transpose(out.reshape(B, H, W, C), (0, 3, 1, 2))
```

```python
import itertools

import jax
import jax.numpy as jnp
from jax import lax
import jax.experimental.pallas as pl
import jax.experimental.pallas.tpu as pltpu

F32 = jnp.float32
BF16 = jnp.bfloat16
U32 = jnp.uint32

PA = 2.0 / 3.0
PB = 1.5
A2, B2 = PA * PA, PB * PB
NA = 1.0 / (2 * A2 * (A2 - B2))
NB = 1.0 / (2 * B2 * (B2 - A2))
RT = PB / PA
GS = PA ** 3

TPOS = (0, 24, 32, 40, 48, 56, 64, 16)
TREC = 72
C0COST = 38
A1COST = 34
A2COST = 46
FINCOST = 40
ZMOD = 4
ZFIN = 40
XCH = 4
MROW = 264
MSLOT = 36 * MROW
K_A2, K_B2, K_SHIFT, K_MASK, K_SUM, K_SQ, K_SCALE = (i * MROW + 256 for i in range(7))


def _bt(d0, d1, d2, d3, d4, d5, a2=A2, b2=B2):
    t, u = a2 * d2, b2 * d2
    ea, eb = d4 - u, d4 - t
    v0 = ea - t
    if d0 is not None:
        v0 = v0 + d0
    t3, u3 = a2 * d3, b2 * d3
    pa, pb = t3 - d1, u3 - d1
    v5 = (d5 - pa) - u3 if d5 is not None else (d1 - t3) - u3
    oa, ob = PB * pa, PA * pb
    return v0, ea + oa, ea - oa, eb + ob, eb - ob, v5


def _at(m0, m1, m2, m3, m4, m5):
    sa, ta, sb, tb = m1 + m2, m1 - m2, m3 + m4, m3 - m4
    return (m0 + sa) + sb, ta + RT * tb, sa + (RT * RT) * sb, (ta + m5) + (RT * RT * RT) * tb


def _gt(g0, g1, g2, k):
    ea, oa = (k * NA) * g0 + (k * NA * A2) * g2, (k * NA * PA) * g1
    eb, ob = (k * NB) * g0 + (k * NB * B2) * g2, (k * NB * PB) * g1
    k5 = k / PA ** 3
    u0 = g0 if abs(k - 1.0) < 1e-12 else k * g0
    u5 = g2 if abs(k5 - 1.0) < 1e-12 else k5 * g2
    return u0, ea + oa, ea - oa, eb + ob, eb - ob, u5


def _pack(lo, hi):
    return pltpu.pack_elementwise([lo, hi], packed_dtype=BF16)


def _unpack(w, i):
    return pltpu.unpack_elementwise(w, index=i, packed_dtype=BF16, unpacked_dtype=F32)


def _tree(xs):
    while len(xs) > 1:
        xs = [xs[i] + xs[i + 1] for i in range(0, len(xs), 2)]
    return xs[0]


def _acc(a, x):
    return x if a is None else a + x


class _Rows:
    def __init__(self, ref, base=0):
        self.ref, self.base = ref, base

    def as_u32(self):
        return _Rows(self.ref.bitcast(U32), self.base)

    def ld(self, off, n=8, stride=1):
        return self.ref[pl.ds(self.base + off, n, stride=stride), :]

    def st(self, off, val, stride=1):
        self.ref[pl.ds(self.base + off, val.shape[0], stride=stride), :] = val


def _splitter(const):
    sh, mk = const.as_u32().ld(K_SHIFT), const.as_u32().ld(K_MASK)
    return lambda w: (lax.bitcast_convert_type(w << sh, F32), lax.bitcast_convert_type(w & mk, F32))


def _job_u(w, u, const):
    def gen():
        for r in range(0, 64, 8):
            def taps(rows):
                split = _splitter(const)
                return [list(zip(*[split(w[3 * i + j].ld(r)) for j in range(3)])) for i in rows]

            def emit(i, row, k):
                lo, hi = _gt(*row[0], k), _gt(*row[1], k)
                for j in range(6):
                    u.st((i * 6 + j) * 64 + r, _pack(lo[j], hi[j]))

            emit(0, taps([0])[0], GS)
            yield 38
            emit(5, taps([2])[0], 1.0)
            yield 38
            for i, nn, p in ((1, NA, PA), (3, NB, PB)):
                g0, g1, g2 = taps([0, 1, 2])
                e = [[nn * g0[h][j] + (nn * p * p) * g2[h][j] for j in range(3)] for h in range(2)]
                o = [[(nn * p) * g1[h][j] for j in range(3)] for h in range(2)]
                emit(i, [[e[h][j] + o[h][j] for j in range(3)] for h in range(2)], GS)
                emit(i + 1, [[e[h][j] - o[h][j] for j in range(3)] for h in range(2)], GS)
                yield 118

    return gen(), 8 * 312


def _gn_coeffs(s, q, e, gamma, beta, ab):
    s = jnp.sum(s, axis=0, keepdims=True) * (1.0 / 4096)
    q = jnp.sum(q, axis=0, keepdims=True) * (1.0 / 4096)
    var_c = jnp.maximum(q - s * s, 0.0)
    mean_c = s if e is None else s + e
    mu = jnp.sum(mean_c, axis=1, keepdims=True) * (1.0 / 128)
    dm = mean_c - mu
    var = jnp.sum(var_c + dm * dm, axis=1, keepdims=True) * (1.0 / 128)
    a = 0.5 * gamma * lax.rsqrt(var + 1e-5)
    b = 0.5 * beta + a * (-mu if e is None else e - mu)
    ab.st(0, jnp.broadcast_to(a, (8, 128)))
    ab.st(8, jnp.broadcast_to(b, (8, 128)))


def _unpack_row(load, h, y, split):
    vals = []
    for k in range(2):
        for sub in range(2):
            for i, v in enumerate(split(load(sub * 16 + k))):
                h.st(y * 64 + (2 * k + i) * 16 + sub * 8, v)
                vals.append(v)
    return _tree(vals), _tree([v * v for v in vals])


def _job_c0(x, h, gamma, beta, ab, const):
    def gen():
        s = q = None
        for y in range(64):
            part = _Rows(x.at[y // (64 // XCH)], (y % (64 // XCH)) * 32)
            ds, dq = _unpack_row(lambda off: part.ld(off, 8, 2), h, y, _splitter(const))
            if y % ZMOD == 0 and y > 1:
                const.st(K_SUM, old[0])
                const.st(K_SQ, old[1])
            old = (s, q)
            s, q = _acc(s, ds), _acc(q, dq)
            yield C0COST
        _gn_coeffs(s, q, None, gamma[...], beta[...], ab)
        yield ZFIN

    return gen(), 64 * C0COST + ZFIN


def _job_a(h, ab, t, v, const, k):
    scale, shift = K_SCALE + 2 * k * MROW, K_SCALE + (2 * k + 1) * MROW
    const.st(scale, ab.ld(0))
    const.st(shift, ab.ld(8))

    def gen():
        b = const.ld(shift)

        def act(y, q, a):
            if y > 63:
                return None
            u = h.ld(y * 64 + (q % 4) * 16 + q // 4, 8, 2) * a + b
            return u * jnp.tanh(u) + u

        for q in range(8):
            d4, d5 = None, act(0, q, const.ld(scale))
            for ty in range(16):
                a = const.ld(scale)
                d0, d1 = d4, d5
                d2, d3, d4, d5 = (act(4 * ty + k, q, a) for k in range(1, 5))
                for i, val in enumerate(_bt(d0, d1, d2, d3, d4, d5)):
                    t.st((ty * 6 + i) * TREC + TPOS[q], val)
                yield A1COST
        for ty in range(16):
            for i in range(6):
                offs = (TPOS[7] - 1,) + TPOS + (TPOS[0] + 1,)
                d = [t.ld((ty * 6 + i) * TREC + o) for o in offs]
                a2, b2 = const.ld(K_A2), const.ld(K_B2)
                for j, (lo, hi) in enumerate(zip(_bt(*d[0:6], a2, b2), _bt(*d[4:10], a2, b2))):
                    v.st((i * 6 + j) * 128 + ty * 8, _pack(lo, hi))
                yield A2COST

    return gen(), 128 * A1COST + 96 * A2COST


def _tiles_out(m, r0, finish, cost):
    def row(i):
        return _at(*[m.ld((i * 6 + j) * MROW + r0) for j in range(6)])

    def done(i, ys):
        finish(i, [y if i + j == 3 else (PA ** (i + j) / GS) * y for j, y in enumerate(ys)])

    r1 = row(1)
    yield 13
    r2 = row(2)
    sa, ta = [x + y for x, y in zip(r1, r2)], [x - y for x, y in zip(r1, r2)]
    yield 21
    r3 = row(3)
    yield 13
    r4 = row(4)
    sb, tb = [x + y for x, y in zip(r3, r4)], [x - y for x, y in zip(r3, r4)]
    done(1, [x + RT * y for x, y in zip(ta, tb)])
    yield 32 + cost
    done(2, [x + (RT * RT) * y for x, y in zip(sa, sb)])
    done(0, [(x + y) + w for x, y, w in zip(sa, sb, row(0))])
    yield 35 + 2 * cost
    done(3, [(x + (RT * RT * RT) * y) + w for x, y, w in zip(ta, tb, row(5))])
    yield 28 + cost


def _job_c1(m, h, e, gamma, beta, ab):
    def gen():
        sq = [None, None]
        for ty in range(16):
            for sub in range(2):
                def finish(i, ys):
                    sq[0] = _acc(sq[0], _tree(ys))
                    sq[1] = _acc(sq[1], _tree([y * y for y in ys]))
                    for j in range(4):
                        h.st((4 * ty + i) * 64 + j * 16 + sub * 8, ys[j])

                before = tuple(sq)
                for n, cost in enumerate(_tiles_out(m, ty * 16 + sub * 8, finish, 12)):
                    if n == 1 and before[0] is not None:
                        m.st(K_SUM, before[0])
                        m.st(K_SQ, before[1])
                    yield cost
        _gn_coeffs(sq[0], sq[1], e[...], gamma[...], beta[...], ab)
        yield FINCOST

    return gen(), 32 * (142 + 48) + FINCOST


def _residual_out(m, x):
    for ty in range(16 // XCH):
        for sub in range(2):
            def finish(i, ys):
                for k in range(2):
                    off = (4 * ty + i) * 32 + sub * 16 + k
                    w = x.ld(off, 8, 2)
                    x.st(off, _pack(_unpack(w, 0) + ys[2 * k], _unpack(w, 1) + ys[2 * k + 1]), 2)

            yield from _tiles_out(m, ty * 16 + sub * 8, finish, 10)


def _job_c2(m, x):
    def gen():
        for c in range(XCH):
            yield from _residual_out(_Rows(m.ref, m.base + c * (256 // XCH)), _Rows(x.at[c]))

    return gen(), 32 * (142 + 40)


def _run(*jobs):
    for gen, _ in jobs:
        for _ in gen:
            pass


def _step(v, u, m, jobs, rows=16, lead=300, tail=5):
    total = sum(c for _, c in jobs)
    pieces = itertools.chain(*[g for g, _ in jobs])
    span = 36 * 256 // rows - tail
    spent = 0

    def advance(limit):
        nonlocal spent
        while spent < limit:
            cost = next(pieces, None)
            if cost is None:
                return
            spent += cost

    tick = 0
    advance(lead)
    for xi in range(36):
        lhs = jnp.concatenate([pltpu.bitcast(r.ld(xi * 128, 128), BF16) for r in v], axis=1)
        rhs = jnp.concatenate([pltpu.bitcast(r.ld(xi * 64, 64), BF16) for r in u], axis=1)
        res = lax.dot_general(lhs, rhs, (((1,), (1,)), ((), ())), preferred_element_type=F32)
        for r in range(0, 256, rows):
            m.st(xi * MROW + r, res[r:r + rows])
            tick += 1
            advance(lead + (total - lead) * tick / span)
    advance(float("inf"))


def _kernel(x_hbm, t_hbm, g1_hbm, be1_hbm, w1_hbm, we_hbm, g2_hbm, be2_hbm, w2_hbm, o_hbm,
            t_ref, g1_ref, be1_ref, g2_ref, be2_ref,
            xbuf, wbuf, webuf, hbuf, abuf, t0, t1, v0, v1, u1, u2, mbuf, par, emb, slots,
            xsem, csem, wsem, esem, psem, osem):
    x32 = xbuf.bitcast(U32)
    w32 = wbuf.bitcast(U32)

    def lanes(g):
        return pl.ds(g * 128 if isinstance(g, int) else pl.multiple_of(g * 128, 128), 128)

    def x_copy(j):
        return pltpu.make_async_copy(x_hbm.at[j // 4, :, :, lanes(j % 4)], xbuf.at[j], xsem.at[j])

    def x_chunk_copy(c):
        return pltpu.make_async_copy(x_hbm.at[0, c, :, lanes(0)], xbuf.at[0, c], csem.at[c])

    def o_copy(j):
        return pltpu.make_async_copy(xbuf.at[j], o_hbm.at[j // 4, :, :, lanes(j % 4)], osem.at[j])

    def o_chunk_copy(c):
        return pltpu.make_async_copy(xbuf.at[7, c], o_hbm.at[1, c, :, lanes(3)], csem.at[c])

    def w1_copy(part, c):
        rows = (pl.ds(0, 128), pl.ds(128, 256), pl.ds(384, 128))[part]
        return pltpu.make_async_copy(w1_hbm.at[:, rows, lanes(c)], wbuf.at[c, :, rows], wsem.at[part, c])

    def w2_copy(c):
        return pltpu.make_async_copy(w2_hbm.at[:, :, lanes(c)], wbuf.at[4 + c], wsem.at[3, c])

    e_copy = pltpu.make_async_copy(we_hbm, webuf, esem.at[0])

    p_copies = [pltpu.make_async_copy(src, dst, psem.at[k]) for k, (src, dst) in enumerate(
        ((g1_hbm, g1_ref), (be1_hbm, be1_ref), (g2_hbm, g2_ref), (be2_hbm, be2_ref), (t_hbm, t_ref)))]

    x_chunk_copy(0).start()
    for cp in p_copies:
        cp.start()
    for c in range(1, XCH):
        x_chunk_copy(c).start()
    w1_copy(0, 0).start()
    x_copy(1).start()
    w1_copy(0, 1).start()
    x_copy(2).start()

    slots[0] = 0
    slots[1] = MSLOT
    for t in (t0, t1):
        for r in range(96):
            _Rows(t).st(r * TREC + 8, jnp.zeros((8, 128), F32))
    for base in (0, MSLOT):
        c = _Rows(mbuf, base)
        c.st(K_A2, jnp.full((8, 128), A2, F32))
        c.st(K_B2, jnp.full((8, 128), B2, F32))
        c.as_u32().st(K_SHIFT, jnp.full((8, 128), 16, U32))
        c.as_u32().st(K_MASK, jnp.full((8, 128), 0xFFFF0000, U32))
    for cp in p_copies:
        cp.wait()
    for k, ref in enumerate((g1_ref, be1_ref, g2_ref, be2_ref)):
        val = ref[...].astype(F32).reshape(4, 128)
        for g in range(4):
            par[k * 4 + g] = val[g:g + 1]

    def m_slot(s):
        return _Rows(mbuf, pl.multiple_of(slots[s % 2], 8))

    def h_slot(j):
        return _Rows(hbuf, j * 4096)

    def ab_slot(j):
        return _Rows(abuf, j * 16)

    def job_u(conv, n, c, const):
        rows = n * 64 if isinstance(n, int) else pl.multiple_of(n * 64, 64)
        taps = [_Rows(w32.at[conv * 4 + c, k], rows) for k in range(9)]
        return _job_u(taps, _Rows((u1, u2)[conv].at[n * 4 + c]), const)

    def job_c0(j, const):
        return _job_c0(x32.at[j], h_slot(j), par.at[j % 4], par.at[4 + j % 4], ab_slot(j), const)

    def job_a(j, v, const, k=0):
        return _job_a(h_slot(j), ab_slot(j), _Rows((t0, t1)[k]), _Rows(v.at[j % 4]), const, k)

    def job_c1(j, m):
        return _job_c1(m, h_slot(j), emb.at[j], par.at[8 + j % 4], par.at[12 + j % 4], ab_slot(j))

    def job_c2(j, m):
        return _job_c2(m, x32.at[j])

    def step(s, v, u, jobs):
        _step([_Rows(v.at[g]) for g in range(4)], [_Rows(u.at[(s % 4) * 4 + g]) for g in range(4)],
              m_slot(s), jobs)

    const0 = _Rows(mbuf)

    @pl.loop(0, 4)
    def _(j):
        def unpack_chunk(c, sums):
            @pl.when(j == 0)
            def _():
                x_chunk_copy(c).wait()

            x = _Rows(x32.at[j, c])
            h = _Rows(hbuf, j * 4096 + c * (4096 // XCH))
            s, q = sums
            for y in range(64 // XCH):
                ds, dq = _unpack_row(lambda off: x.ld(y * 32 + off, 8, 2), h, y,
                                     lambda w: (_unpack(w, 0), _unpack(w, 1)))
                s, q = s + ds, q + dq
            return s, q

        s, q = lax.fori_loop(0, XCH, unpack_chunk, (jnp.zeros((8, 128), F32),) * 2)
        w1_copy(0, j).wait()
        _gn_coeffs(s, q, None, par[j], par[4 + j], ab_slot(j))
        _run(job_u(0, 0, j, const0))

        @pl.when(j == 0)
        def _():
            w1_copy(0, 2).start()
            x_copy(3).start()
            w1_copy(0, 3).start()

        @pl.when(j == 1)
        def _():
            for c in range(4):
                w1_copy(1, c).start()

        @pl.when(j == 2)
        def _():
            for c in range(4, 7):
                x_copy(c).start()

        @pl.when(j == 3)
        def _():
            for c in range(4):
                w1_copy(2, c).start()
            x_copy(7).start()
            e_copy.start()

        _run(job_a(j, v0, const0))

        @pl.when(j < 3)
        def _():
            x_copy(j + 1).wait()

    for c in range(4):
        w1_copy(1, c).wait()
    prev = m_slot(1)
    step(0, v0, u1, [job_u(0, n, c, prev) for n in (1, 2) for c in range(4)])

    def embed():
        x_copy(7).wait()
        e_copy.wait()
        th = t_ref[...].astype(F32) * 0.5
        e = jnp.dot((th * jnp.tanh(th) + th).astype(BF16), webuf[...], preferred_element_type=F32)
        for j in range(8):
            emb[j] = e[j // 4:j // 4 + 1, (j % 4) * 128:(j % 4 + 1) * 128]
        yield 0

    for c in range(4):
        w1_copy(2, c).wait()
    for c in range(4, 7):
        x_copy(c).wait()
    for c in range(4):
        w2_copy(c).start()
    prev = m_slot(0)
    step(1, v0, u1, [job_c0(4, prev), job_c0(5, prev), job_c0(6, prev), job_u(0, 3, 0, prev),
                     job_u(0, 3, 1, prev), (embed(), 0), job_c0(7, prev), job_c1(0, prev),
                     job_u(0, 3, 2, prev), job_u(0, 3, 3, prev)])

    @pl.loop(2, 4)
    def _(s):
        prev = m_slot(s + 1)
        step(s, v0, u1, [job_a(2 * s, v1, prev), job_a(2 * s + 1, v1, prev, 1), job_c1(s - 1, prev), (iter([500]), 500)])

    for c in range(4):
        w2_copy(c).wait()

    @pl.loop(4, 8)
    def _(s):
        prev = m_slot(s + 1)
        step(s, v1, u1, [job_a(s - 4, v0, prev), job_c1(s - 1, prev)]
             + [job_u(1, n, s - 4, prev) for n in range(3)])

    prev = m_slot(1)
    step(8, v0, u2, [job_a(4, v1, prev), job_c1(7, prev)] + [job_u(1, 3, c, prev) for c in range(4)])

    @pl.loop(9, 12)
    def _(s):
        prev = m_slot(s + 1)
        step(s, v0, u2, [job_a(s - 4, v1, prev), job_c2(s - 9, prev)])
        o_copy(s - 9).start()

    @pl.loop(12, 16)
    def _(s):
        prev = m_slot(s + 1)
        step(s, v1, u2, [job_c2(s - 9, prev)])
        o_copy(s - 9).start()

    @pl.loop(0, XCH)
    def _(c):
        for _ in _residual_out(_Rows(mbuf, MSLOT + c * (256 // XCH)), _Rows(x32.at[7, c])):
            pass
        o_chunk_copy(c).start()

    for j in range(7):
        o_copy(j).wait()
    for c in range(XCH):
        o_chunk_copy(c).wait()


@jax.jit
def pallas_standalone__adm_resblock__diffusion_kernel(
    x: jax.Array,
    t_emb: jax.Array,
    g1: jax.Array,
    be1: jax.Array,
    w1: jax.Array,
    w_emb: jax.Array,
    g2: jax.Array,
    be2: jax.Array,
    w2: jax.Array,
):
    B, C, H, W = x.shape
    assert (B, C, H, W) == (2, 512, 64, 64)
    xt = jnp.transpose(x, (0, 2, 3, 1)).reshape(B, XCH, H * W // XCH, C)
    w1t = jnp.transpose(w1, (2, 3, 0, 1)).reshape(9, C, C)
    w2t = jnp.transpose(w2, (2, 3, 0, 1)).reshape(9, C, C)
    hbm = pl.BlockSpec(memory_space=pl.ANY)
    out = pl.pallas_call(
        _kernel,
        out_shape=jax.ShapeDtypeStruct(xt.shape, x.dtype),
        in_specs=[hbm] * 9,
        out_specs=hbm,
        scratch_shapes=[
            pltpu.VMEM(t_emb.shape, BF16),
            pltpu.VMEM(g1.shape, BF16),
            pltpu.VMEM(be1.shape, BF16),
            pltpu.VMEM(g2.shape, BF16),
            pltpu.VMEM(be2.shape, BF16),
            pltpu.VMEM((8, XCH, 4096 // XCH, 128), BF16),
            pltpu.VMEM((8, 9, 512, 128), BF16),
            pltpu.VMEM(w_emb.shape, BF16),
            pltpu.VMEM((8 * 4096, 128), F32),
            pltpu.VMEM((8 * 16, 128), F32),
            pltpu.VMEM((96 * TREC, 128), F32),
            pltpu.VMEM((96 * TREC, 128), F32),
            pltpu.VMEM((4, 36 * 128, 128), U32),
            pltpu.VMEM((4, 36 * 128, 128), U32),
            pltpu.VMEM((16, 36 * 64, 128), U32),
            pltpu.VMEM((16, 36 * 64, 128), U32),
            pltpu.VMEM((2 * MSLOT, 128), F32),
            pltpu.VMEM((16, 1, 128), F32),
            pltpu.VMEM((8, 1, 128), F32),
            pltpu.SMEM((2,), jnp.int32),
            pltpu.SemaphoreType.DMA((8,)),
            pltpu.SemaphoreType.DMA((XCH,)),
            pltpu.SemaphoreType.DMA((4, 4)),
            pltpu.SemaphoreType.DMA((1,)),
            pltpu.SemaphoreType.DMA((5,)),
            pltpu.SemaphoreType.DMA((8,)),
        ],
        compiler_params=pltpu.CompilerParams(vmem_limit_bytes=120 * 2**20),
        name="resblk",
    )(xt, t_emb, g1, be1, w1t, w_emb, g2, be2, w2t)
    return jnp.transpose(out.reshape(B, H, W, C), (0, 3, 1, 2))
```

```python
import itertools

import jax
import jax.numpy as jnp
from jax import lax
import jax.experimental.pallas as pl
import jax.experimental.pallas.tpu as pltpu

F32 = jnp.float32
BF16 = jnp.bfloat16
U32 = jnp.uint32

PA = 2.0 / 3.0
PB = 1.5
A2, B2 = PA * PA, PB * PB
NA = 1.0 / (2 * A2 * (A2 - B2))
NB = 1.0 / (2 * B2 * (B2 - A2))
RT = PB / PA
GS = PA ** 3
ROWS = (0, 5, 1, 2, 3, 4)

TPOS = (0, 24, 32, 40, 48, 56, 64, 16)
TREC = 72
XCH = 4
MROW = 264
MSLOT = 36 * MROW
M_SLOT = (0, 1, 2, 3, 4, 0, 1, 2, 3, 4, 0, 1, 3, 4, 2, 0)
K_A2, K_B2, K_SHIFT, K_MASK, K_SUM, K_SQ, K_GN = (i * MROW + 256 for i in range(7))

C0COST, A1COST, A2COST = 38, 34, 46


def _bt(d0, d1, d2, d3, d4, d5, a2=A2, b2=B2):
    t, u = a2 * d2, b2 * d2
    ea, eb = d4 - u, d4 - t
    v0 = ea - t
    if d0 is not None:
        v0 = v0 + d0
    t3, u3 = a2 * d3, b2 * d3
    pa, pb = t3 - d1, u3 - d1
    v5 = (d5 - pa) - u3 if d5 is not None else (d1 - t3) - u3
    oa, ob = PB * pa, PA * pb
    return v0, ea + oa, ea - oa, eb + ob, eb - ob, v5


def _at(m0, m1, m2, m3, m4, m5):
    sa, ta, sb, tb = m1 + m2, m1 - m2, m3 + m4, m3 - m4
    return (m0 + sa) + sb, ta + RT * tb, sa + (RT * RT) * sb, (ta + m5) + (RT * RT * RT) * tb


def _gt(g0, g1, g2, k):
    ea, oa = (k * NA) * g0 + (k * NA * A2) * g2, (k * NA * PA) * g1
    eb, ob = (k * NB) * g0 + (k * NB * B2) * g2, (k * NB * PB) * g1
    k5 = k / PA ** 3
    u0 = g0 if abs(k - 1.0) < 1e-12 else k * g0
    u5 = g2 if abs(k5 - 1.0) < 1e-12 else k5 * g2
    return u0, ea + oa, ea - oa, eb + ob, eb - ob, u5


def _pack(lo, hi):
    return pltpu.pack_elementwise([lo, hi], packed_dtype=BF16)


def _unpack(w):
    return tuple(pltpu.unpack_elementwise(w, index=i, packed_dtype=BF16, unpacked_dtype=F32) for i in range(2))


def _tree(xs):
    while len(xs) > 1:
        xs = [xs[i] + xs[i + 1] for i in range(0, len(xs), 2)]
    return xs[0]


def _acc(a, x):
    return x if a is None else a + x


class _Rows:
    def __init__(self, ref, base=0):
        self.ref, self.base = ref, base

    def as_u32(self):
        return _Rows(self.ref.bitcast(U32), self.base)

    def ld(self, off, n=8, stride=1):
        return self.ref[pl.ds(self.base + off, n, stride=stride), :]

    def st(self, off, val, stride=1):
        self.ref[pl.ds(self.base + off, val.shape[0], stride=stride), :] = val


def _splitter(const):
    bits = const.as_u32()
    sh, mk = bits.ld(K_SHIFT), bits.ld(K_MASK)
    return lambda w: (lax.bitcast_convert_type(w << sh, F32), lax.bitcast_convert_type(w & mk, F32))


def _job_u(w, u, const, row):
    cost = 38 if row in (0, 5) else 118

    def gen():
        for r in range(0, 64, 8):
            split = _splitter(const)

            def taps(i):
                return list(zip(*[split(w[3 * i + j].ld(r)) for j in range(3)]))

            def emit(i, vals, k):
                lo, hi = _gt(*vals[0], k), _gt(*vals[1], k)
                for j in range(6):
                    u.st((i * 6 + j) * 64 + r, _pack(lo[j], hi[j]))

            if row == 0:
                emit(0, taps(0), GS)
            elif row == 5:
                emit(5, taps(2), 1.0)
            else:
                nn, p = (NA, PA) if row == 1 else (NB, PB)
                g0, g1, g2 = taps(0), taps(1), taps(2)
                e = [[nn * g0[h][j] + (nn * p * p) * g2[h][j] for j in range(3)] for h in range(2)]
                o = [[(nn * p) * g1[h][j] for j in range(3)] for h in range(2)]
                emit(row, [[e[h][j] + o[h][j] for j in range(3)] for h in range(2)], GS)
                emit(row + 1, [[e[h][j] - o[h][j] for j in range(3)] for h in range(2)], GS)
            yield cost

    return gen(), 8 * cost


def _gn_coeffs(s, q, e, gamma, beta, ab):
    s = jnp.sum(s, axis=0, keepdims=True) * (1.0 / 4096)
    q = jnp.sum(q, axis=0, keepdims=True) * (1.0 / 4096)
    var_c = jnp.maximum(q - s * s, 0.0)
    mean_c = s if e is None else s + e
    mu = jnp.sum(mean_c, axis=1, keepdims=True) * (1.0 / 128)
    second = jnp.sum(var_c + mean_c * mean_c, axis=1, keepdims=True) * (1.0 / 128)
    var = jnp.maximum(second - mu * mu, 0.0)
    a = 0.5 * gamma * lax.rsqrt(var + 1e-5)
    b = 0.5 * beta + a * (-mu if e is None else e - mu)
    ab.st(0, jnp.broadcast_to(a, (8, 128)))
    ab.st(8, jnp.broadcast_to(b, (8, 128)))


def _unpack_row(x, h, y, split):
    vals = []
    for k in range(2):
        for sub in range(2):
            for i, v in enumerate(split(x.ld(sub * 16 + k, 8, 2))):
                h.st(y * 64 + (2 * k + i) * 16 + sub * 8, v)
                vals.append(v)
    return _tree(vals), _tree([v * v for v in vals])


def _job_c0(x, h, gamma, beta, ab, const):
    def gen():
        s = q = None
        for y in range(64):
            ds, dq = _unpack_row(_Rows(x.at[y // (64 // XCH)], (y % (64 // XCH)) * 32), h, y, _splitter(const))
            if y % 4 == 0 and y > 0:
                const.st(K_SUM, old[0])
                const.st(K_SQ, old[1])
            old = (s, q)
            s, q = _acc(s, ds), _acc(q, dq)
            yield C0COST
        _gn_coeffs(s, q, None, gamma[...], beta[...], ab)
        yield 40

    return gen(), 64 * C0COST + 40


def _job_a1(h, ab, t, const, k):
    def gen():
        scale = K_GN + k * MROW
        const.st(scale, ab.ld(0))
        b = ab.ld(8)

        def act(y, q, a):
            if y > 63:
                return None
            u = h.ld(y * 64 + (q % 4) * 16 + q // 4, 8, 2) * a + b
            return u * jnp.tanh(u) + u

        for q in range(8):
            d4, d5 = None, act(0, q, const.ld(scale))
            for ty in range(16):
                a = const.ld(scale)
                d0, d1 = d4, d5
                d2, d3, d4, d5 = (act(4 * ty + k, q, a) for k in range(1, 5))
                for i, val in enumerate(_bt(d0, d1, d2, d3, d4, d5)):
                    t.st((ty * 6 + i) * TREC + TPOS[q], val)
                yield A1COST

    return gen(), 128 * A1COST


def _job_a2(t, v, const, rows):
    def gen():
        for i in rows:
            for ty in range(16):
                offs = (TPOS[7] - 1,) + TPOS + (TPOS[0] + 1,)
                d = [t.ld((ty * 6 + i) * TREC + o) for o in offs]
                a2, b2 = const.ld(K_A2), const.ld(K_B2)
                for j, (lo, hi) in enumerate(zip(_bt(*d[0:6], a2, b2), _bt(*d[4:10], a2, b2))):
                    v.st((i * 6 + j) * 128 + ty * 8, _pack(lo, hi))
                yield A2COST

    return gen(), 16 * len(rows) * A2COST


def _tiles_out(m, r0, finish, cost):
    def row(i):
        return _at(*[m.ld((i * 6 + j) * MROW + r0) for j in range(6)])

    def done(i, ys):
        finish(i, [y if i + j == 3 else (PA ** (i + j) / GS) * y for j, y in enumerate(ys)])

    r1 = row(1)
    yield 13
    r2 = row(2)
    sa, ta = [x + y for x, y in zip(r1, r2)], [x - y for x, y in zip(r1, r2)]
    yield 21
    r3 = row(3)
    yield 13
    r4 = row(4)
    sb, tb = [x + y for x, y in zip(r3, r4)], [x - y for x, y in zip(r3, r4)]
    done(1, [x + RT * y for x, y in zip(ta, tb)])
    yield 32 + cost
    done(2, [x + (RT * RT) * y for x, y in zip(sa, sb)])
    done(0, [(x + y) + w for x, y, w in zip(sa, sb, row(0))])
    yield 35 + 2 * cost
    done(3, [(x + (RT * RT * RT) * y) + w for x, y, w in zip(ta, tb, row(5))])
    yield 28 + cost


def _job_c1(m, h, e, gamma, beta, ab):
    def gen():
        sq = [None, None]
        for ty in range(16):
            for sub in range(2):
                def finish(i, ys):
                    sq[0] = _acc(sq[0], _tree(ys))
                    sq[1] = _acc(sq[1], _tree([y * y for y in ys]))
                    for j in range(4):
                        h.st((4 * ty + i) * 64 + j * 16 + sub * 8, ys[j])

                before = tuple(sq)
                for n, cost in enumerate(_tiles_out(m, ty * 16 + sub * 8, finish, 12)):
                    if n == 1 and before[0] is not None:
                        m.st(K_SUM, before[0])
                        m.st(K_SQ, before[1])
                    yield cost
        _gn_coeffs(sq[0], sq[1], e[...], gamma[...], beta[...], ab)
        yield 40

    return gen(), 32 * (142 + 48) + 40


def _residual_out(m, x):
    for ty in range(16 // XCH):
        for sub in range(2):
            def finish(i, ys):
                for k in range(2):
                    off = (4 * ty + i) * 32 + sub * 16 + k
                    lo, hi = _unpack(x.ld(off, 8, 2))
                    x.st(off, _pack(lo + ys[2 * k], hi + ys[2 * k + 1]), 2)

            yield from _tiles_out(m, ty * 16 + sub * 8, finish, 10)


def _job_c2(m, x):
    return _residual_out(m, x), (32 // XCH) * (142 + 40)


def _run(*jobs):
    for gen, _ in jobs:
        for _ in gen:
            pass


def _step(v, u, m, jobs, add=False, tile_rows=ROWS, tiles=(0, 256), rows=16, tail=5):
    total = sum(c for _, c in jobs)
    pieces = itertools.chain(*[g for g, _ in jobs])
    first, count = tiles
    span = len(tile_rows) * 6 * count // rows - tail
    lead = 7 * total / span
    spent = 0

    def advance(limit):
        nonlocal spent
        while spent < limit:
            cost = next(pieces, None)
            if cost is None:
                return
            spent += cost

    tick = 0
    advance(lead)
    for xi in (6 * i + j for i in tile_rows for j in range(6)):
        lhs = jnp.concatenate([pltpu.bitcast(r.ld(xi * 128 + first // 2, count // 2), BF16) for r in v], axis=1)
        rhs = jnp.concatenate(
            [jnp.concatenate([pltpu.bitcast(r.ld(xi * 64, 64), BF16) for r in un], axis=1) for un in u], axis=0)
        res = lax.dot_general(lhs, rhs, (((1,), (1,)), ((), ())), preferred_element_type=F32)
        for r in range(0, count, rows):
            for n, mn in enumerate(m):
                val = res[r:r + rows, n * 128:(n + 1) * 128]
                at = xi * MROW + first + r
                mn.st(at, val + mn.ld(at, rows) if add else val)
            tick += 1
            advance(lead + (total - lead) * tick / span)
    advance(float("inf"))


def _kernel(x_hbm, t_hbm, g1_hbm, be1_hbm, w1_hbm, we_hbm, g2_hbm, be2_hbm, w2_hbm, o_hbm,
            t_ref, g1_ref, be1_ref, g2_ref, be2_ref,
            xbuf, wbuf, webuf, hbuf, abuf, t0, t1, t2, v0, v1, u1, u2, mbuf, par, emb, slots,
            xsem, csem, wsem, psem, osem):
    x32 = xbuf.bitcast(U32)
    w32 = wbuf.bitcast(U32)

    def lanes(g):
        return pl.ds(g * 128 if isinstance(g, int) else pl.multiple_of(g * 128, 128), 128)

    def x_copy(j):
        return pltpu.make_async_copy(x_hbm.at[j // 4, :, :, lanes(j % 4)], xbuf.at[j], xsem.at[j])

    def x_chunk_copy(j, c):
        return pltpu.make_async_copy(x_hbm.at[0, c, :, lanes(j)], xbuf.at[j, c], csem.at[j, c])

    def o_copy(b, g):
        return pltpu.make_async_copy(xbuf.at[b * 4 + g], o_hbm.at[b, :, :, lanes(g)], osem.at[b * 4 + g])

    def o_chunk_copy(c):
        return pltpu.make_async_copy(xbuf.at[7, c], o_hbm.at[1, c, :, lanes(3)], csem.at[0, c])

    def w1_copy(out_half, c):
        rows = pl.ds(out_half * 256, 256)
        return pltpu.make_async_copy(w1_hbm.at[:, rows, lanes(c)], wbuf.at[c, :, rows], wsem.at[out_half, c])

    def w1_copies(out_half, in_half):
        return [w1_copy(out_half, 2 * in_half + c) for c in range(2)]

    def w2_copies():
        return [pltpu.make_async_copy(w2_hbm.at[:, :, lanes(c)], wbuf.at[4 + c], wsem.at[2, c]) for c in range(4)]

    def p_copies(ks):
        pairs = ((g1_hbm, g1_ref), (be1_hbm, be1_ref), (g2_hbm, g2_ref), (be2_hbm, be2_ref), (t_hbm, t_ref),
                 (we_hbm, webuf))
        return [pltpu.make_async_copy(*pairs[k], psem.at[k]) for k in ks]

    def start(copies):
        for cp in copies:
            cp.start()

    def wait(copies):
        for cp in copies:
            cp.wait()

    def load_params(ks):
        wait(p_copies(ks))
        for k in ks:
            val = (g1_ref, be1_ref, g2_ref, be2_ref)[k][...].astype(F32).reshape(4, 128)
            for g in range(4):
                par[k * 4 + g] = val[g:g + 1]

    start(p_copies((0, 1)))

    @pl.loop(0, 2 * XCH)
    def _(i):
        x_chunk_copy(i // XCH, i % XCH).start()

    @pl.loop(0, 2)
    def _(c):
        w1_copy(0, c).start()

    for t in (t0, t1, t2):
        for r in range(96):
            _Rows(t).st(r * TREC + 8, jnp.zeros((8, 128), F32))
    for k, slot in enumerate(M_SLOT):
        slots[k] = slot * MSLOT
        slots[16 + k] = slot * MSLOT
    fixed = _Rows(mbuf)
    fixed.st(K_A2, jnp.full((8, 128), A2, F32))
    fixed.st(K_B2, jnp.full((8, 128), B2, F32))
    fixed.as_u32().st(K_SHIFT, jnp.full((8, 128), 16, U32))
    fixed.as_u32().st(K_MASK, jnp.full((8, 128), 0xFFFF0000, U32))

    def m_in(k):
        return _Rows(mbuf, pl.multiple_of(slots[k], 8))

    def m_out(k, count=1):
        base = pl.multiple_of(slots[16 + k], 8)
        return [_Rows(mbuf, base + i * MSLOT) for i in range(count)]

    def h_slot(j):
        return _Rows(hbuf, j * 4096)

    def ab_slot(j):
        return _Rows(abuf, j * 16)

    def taps(conv, n, c):
        rows = n * 64 if isinstance(n, int) else pl.multiple_of(n * 64, 64)
        return [_Rows(w32.at[conv * 4 + c, k], rows) for k in range(9)]

    def u1_jobs(blocks, rows, const):
        return [_job_u(taps(0, n, c), _Rows(u1.at[n * 4 + c]), const, row) for n, c in blocks for row in rows]

    def u2_jobs(u, n, first, cs):
        return [_job_u(taps(1, n, c), _Rows(u.at[(n - first) * 4 + c]), const, row)
                for c in cs for row in (0, 5, 1, 3)]

    def quad(out_half, in_half):
        return [(2 * out_half + n, 2 * in_half + c) for n in range(2) for c in range(2)]

    def c0(j):
        return _job_c0(x32.at[j], h_slot(j), par.at[j % 4], par.at[4 + j % 4], ab_slot(j), const)

    def a1(j, k):
        return _job_a1(h_slot(j), ab_slot(j), _Rows((t0, t1, t2)[k]), const, k)

    def a2(v, g, k, rows=ROWS):
        return _job_a2(_Rows((t0, t1, t2)[k]), _Rows(v.at[g]), const, rows)

    def c1(j):
        return _job_c1(m_in(j), h_slot(j), emb.at[j], par.at[8 + j % 4], par.at[12 + j % 4], ab_slot(j))

    def c2(j, c):
        m = m_in(8 + j)
        return _job_c2(_Rows(mbuf, m.base + c * (256 // XCH)), _Rows(x32.at[j, c]))

    def block(fn):
        pl.when(slots[0] == 0)(fn)

    def half_step(out_half, in_half, jobs, rows=ROWS):
        ins = (2 * in_half, 2 * in_half + 1)
        outs = (2 * out_half, 2 * out_half + 1)
        block(lambda: _step([_Rows(v0.at[c]) for c in ins], [[_Rows(u1.at[n * 4 + c]) for c in ins] for n in outs],
                            m_out(outs[0], 2), jobs, add=bool(in_half), tile_rows=rows, rows=8, tail=8))

    def step(slot, v, u, n, jobs, **kwargs):
        block(lambda: _step([_Rows(v.at[c]) for c in range(4)], [[_Rows(u.at[n * 4 + c]) for c in range(4)]],
                            m_out(slot), jobs, **kwargs))

    @pl.loop(0, 2)
    def _(j):
        def unpack_chunk(c, sums):
            x_chunk_copy(j, c).wait()
            h = _Rows(hbuf, j * 4096 + c * (4096 // XCH))
            s, q = sums
            for y in range(64 // XCH):
                ds, dq = _unpack_row(_Rows(x32.at[j, c], y * 32), h, y, _unpack)
                s, q = s + ds, q + dq
            return s, q

        s, q = lax.fori_loop(0, XCH, unpack_chunk, (jnp.zeros((8, 128), F32),) * 2)

        @pl.when(j == 0)
        def _():
            load_params((0, 1))
            x_copy(2).start()
            _gn_coeffs(s, q, None, par[0], par[4], ab_slot(0))

        @pl.when(j == 1)
        def _():
            _gn_coeffs(s, q, None, par[1], par[5], ab_slot(1))
            _run(_job_a2(_Rows(t0), _Rows(v0.at[0]), fixed, ROWS[4:]))

        _run(_job_a1(h_slot(j), ab_slot(j), _Rows(t0), fixed, 0),
             _job_a2(_Rows(t0), _Rows(v0.at[j]), fixed, ROWS[:4]))

        @pl.when(j == 0)
        def _():
            start(w1_copies(1, 0))

    x_copy(3).start()

    @pl.loop(0, 2)
    def _(c):
        w1_copy(0, c).wait()
        w1_copy(0, 2 + c).start()
        _run(*u1_jobs([(0, c), (1, c)], (0, 5), fixed))

    const = m_in(0)
    every = (0, 5, 1, 3)
    start(w1_copies(1, 1))
    half_step(0, 0, u1_jobs(quad(0, 0), (1, 3), const) + [a2(v0, 1, 0, ROWS[4:])], ROWS[:2])
    wait([x_copy(2)] + w1_copies(1, 0))
    start([x_copy(j) for j in range(4, 8)])
    half_step(0, 0, [c0(2)] + u1_jobs(quad(1, 0), every, const) + [a1(2, 1)], ROWS[2:])
    wait([x_copy(3)] + w1_copies(0, 1))
    start(p_copies((5, 2, 3, 4)) + w2_copies())
    half_step(1, 0, [c0(3), a2(v0, 2, 1), a1(3, 0), a2(v0, 3, 0)] + u1_jobs(quad(0, 1), every, const))
    wait(w1_copies(1, 1) + [x_copy(j) for j in range(4, 8)])
    half_step(0, 1, [job for i, b in enumerate(quad(1, 1)) for job in [c0(4 + i)] + u1_jobs([b], every, const)]
              + [a1(4, 1)])
    half_step(1, 1, [a2(v1, 0, 1), a1(5, 0), a1(6, 1), a1(7, 2)] + [a2(v1, 1 + k, k, ROWS[:3]) for k in range(3)])

    load_params((2, 3))
    wait(p_copies((4, 5)) + w2_copies())

    def embed():
        th = t_ref[...].astype(F32) * 0.5
        e = jnp.dot((th * jnp.tanh(th) + th).astype(BF16), webuf[...], preferred_element_type=F32)
        for j in range(8):
            emb[j] = e[j // 4:j // 4 + 1, (j % 4) * 128:(j % 4 + 1) * 128]
        yield 0

    step(4, v1, u1, 0, [(embed(), 0)] + [a2(v1, 1 + k, k, (i,)) for i in ROWS[3:] for k in range(3)] + [c1(0), c1(1)]
         + u2_jobs(u2, 0, 0, (0, 1)))
    step(5, v1, u1, 1, [a1(0, 0), a2(v0, 0, 0), c1(2), c1(3)] + u2_jobs(u2, 0, 0, (2, 3)))
    step(6, v1, u1, 2, [a1(1, 1), a2(v0, 1, 1), a1(2, 2), a2(v0, 2, 2), c1(4), (iter([500]), 500)])
    step(7, v1, u1, 3, [a1(3, 0), a2(v0, 3, 0), c1(5)] + u2_jobs(u2, 1, 0, range(4)))

    @pl.loop(0, 2)
    def _(n):
        step(8 + n, v0, u2, n, [a1(4 + n, 1), a2(v1, n, 1), c1(6 + n)] + u2_jobs(u1, 2 + n, 0, range(4)))

    @pl.loop(2, 4)
    def _(n):
        step(8 + n, v0, u1, n, [a1(4 + n, 0), a2(v1, n, 0)] + [c2(n - 2, c) for c in range(XCH)])
        o_copy(0, n - 2).start()

    step(14, v1, u1, 2, [c2(j, c) for j in (2, 3) for c in range(XCH)])
    start([o_copy(0, 2), o_copy(0, 3)])

    @pl.loop(0, 2)
    def _(n):
        done = 2 - 2 * n
        step(12 + n, v1, u2, n, [c2(4 + done, c) for c in range(XCH)])
        o_copy(1, done).start()

    step(15, v1, u1, 3, [c2(5, c) for c in range(XCH)], tiles=(0, 128))
    o_copy(1, 1).start()
    step(15, v1, u1, 3, [c2(7, c) for c in range(XCH // 2)], tiles=(128, 128))
    start([o_chunk_copy(c) for c in range(XCH // 2)])

    @pl.loop(XCH // 2, XCH)
    def _(c):
        _run(c2(7, c))
        o_chunk_copy(c).start()

    wait([o_copy(j // 4, j % 4) for j in range(7)] + [o_chunk_copy(c) for c in range(XCH)])


@jax.jit
def pallas_standalone__adm_resblock__diffusion_kernel(
    x: jax.Array,
    t_emb: jax.Array,
    g1: jax.Array,
    be1: jax.Array,
    w1: jax.Array,
    w_emb: jax.Array,
    g2: jax.Array,
    be2: jax.Array,
    w2: jax.Array,
):
    B, C, H, W = x.shape
    assert (B, C, H, W) == (2, 512, 64, 64)
    xt = jnp.transpose(x, (0, 2, 3, 1)).reshape(B, XCH, H * W // XCH, C)
    w1t = jnp.transpose(w1, (2, 3, 0, 1)).reshape(9, C, C)
    w2t = jnp.transpose(w2, (2, 3, 0, 1)).reshape(9, C, C)
    hbm = pl.BlockSpec(memory_space=pl.ANY)
    out = pl.pallas_call(
        _kernel,
        out_shape=jax.ShapeDtypeStruct(xt.shape, x.dtype),
        in_specs=[hbm] * 9,
        out_specs=hbm,
        scratch_shapes=[
            pltpu.VMEM(t_emb.shape, BF16),
            pltpu.VMEM(g1.shape, BF16),
            pltpu.VMEM(be1.shape, BF16),
            pltpu.VMEM(g2.shape, BF16),
            pltpu.VMEM(be2.shape, BF16),
            pltpu.VMEM((8, XCH, 4096 // XCH, 128), BF16),
            pltpu.VMEM((8, 9, 512, 128), BF16),
            pltpu.VMEM(w_emb.shape, BF16),
            pltpu.VMEM((8 * 4096, 128), F32),
            pltpu.VMEM((8 * 16, 128), F32),
            pltpu.VMEM((96 * TREC, 128), F32),
            pltpu.VMEM((96 * TREC, 128), F32),
            pltpu.VMEM((96 * TREC, 128), F32),
            pltpu.VMEM((4, 36 * 128, 128), U32),
            pltpu.VMEM((4, 36 * 128, 128), U32),
            pltpu.VMEM((16, 36 * 64, 128), U32),
            pltpu.VMEM((8, 36 * 64, 128), U32),
            pltpu.VMEM((5 * MSLOT, 128), F32),
            pltpu.VMEM((16, 1, 128), F32),
            pltpu.VMEM((8, 1, 128), F32),
            pltpu.SMEM((32,), jnp.int32),
            pltpu.SemaphoreType.DMA((8,)),
            pltpu.SemaphoreType.DMA((2, XCH)),
            pltpu.SemaphoreType.DMA((3, 4)),
            pltpu.SemaphoreType.DMA((6,)),
            pltpu.SemaphoreType.DMA((7,)),
        ],
        compiler_params=pltpu.CompilerParams(vmem_limit_bytes=120 * 2**20, disable_bounds_checks=True),
        name="resblk",
    )(xt, t_emb, g1, be1, w1t, w_emb, g2, be2, w2t)
    return jnp.transpose(out.reshape(B, H, W, C), (0, 3, 1, 2))
```

```python
import itertools

import jax
import jax.numpy as jnp
from jax import lax
import jax.experimental.pallas as pl
import jax.experimental.pallas.tpu as pltpu

F32 = jnp.float32
BF16 = jnp.bfloat16
U32 = jnp.uint32

PA = 2.0 / 3.0
PB = 1.5
A2, B2 = PA * PA, PB * PB
NA = 1.0 / (2 * A2 * (A2 - B2))
NB = 1.0 / (2 * B2 * (B2 - A2))
RT = PB / PA
GS = PA ** 3
ROWS = (0, 5, 1, 2, 3, 4)

TPOS = (0, 24, 32, 40, 48, 56, 64, 16)
TREC = 72
XCH = 4
MROW = 264
MSLOT = 36 * MROW
M_SLOT = (0, 1, 2, 3, 4, 0, 1, 2, 3, 4, 0, 1, 3, 4, 2, 0)
K_A2, K_B2, K_SHIFT, K_MASK, K_SUM, K_SQ, K_GN = (i * MROW + 256 for i in range(7))

C0COST, A1COST, A2COST = 38, 34, 46


def _bt(d0, d1, d2, d3, d4, d5, a2=A2, b2=B2):
    t, u = a2 * d2, b2 * d2
    ea, eb = d4 - u, d4 - t
    v0 = ea - t
    if d0 is not None:
        v0 = v0 + d0
    t3, u3 = a2 * d3, b2 * d3
    pa, pb = t3 - d1, u3 - d1
    v5 = (d5 - pa) - u3 if d5 is not None else (d1 - t3) - u3
    oa, ob = PB * pa, PA * pb
    return v0, ea + oa, ea - oa, eb + ob, eb - ob, v5


def _at(m0, m1, m2, m3, m4, m5):
    sa, ta, sb, tb = m1 + m2, m1 - m2, m3 + m4, m3 - m4
    return (m0 + sa) + sb, ta + RT * tb, sa + (RT * RT) * sb, (ta + m5) + (RT * RT * RT) * tb


def _gt(g0, g1, g2, k):
    ea, oa = (k * NA) * g0 + (k * NA * A2) * g2, (k * NA * PA) * g1
    eb, ob = (k * NB) * g0 + (k * NB * B2) * g2, (k * NB * PB) * g1
    k5 = k / PA ** 3
    u0 = g0 if abs(k - 1.0) < 1e-12 else k * g0
    u5 = g2 if abs(k5 - 1.0) < 1e-12 else k5 * g2
    return u0, ea + oa, ea - oa, eb + ob, eb - ob, u5


def _pack(lo, hi):
    return pltpu.pack_elementwise([lo, hi], packed_dtype=BF16)


def _unpack(w):
    return tuple(pltpu.unpack_elementwise(w, index=i, packed_dtype=BF16, unpacked_dtype=F32) for i in range(2))


def _tree(xs):
    while len(xs) > 1:
        xs = [xs[i] + xs[i + 1] for i in range(0, len(xs), 2)]
    return xs[0]


def _acc(a, x):
    return x if a is None else a + x


class _Rows:
    def __init__(self, ref, base=0):
        self.ref, self.base = ref, base

    def as_u32(self):
        return _Rows(self.ref.bitcast(U32), self.base)

    def ld(self, off, n=8, stride=1):
        return self.ref[pl.ds(self.base + off, n, stride=stride), :]

    def st(self, off, val, stride=1):
        self.ref[pl.ds(self.base + off, val.shape[0], stride=stride), :] = val


def _splitter(const):
    bits = const.as_u32()
    sh, mk = bits.ld(K_SHIFT), bits.ld(K_MASK)
    return lambda w: (lax.bitcast_convert_type(w << sh, F32), lax.bitcast_convert_type(w & mk, F32))


def _job_u(w, u, const, row):
    cost = 38 if row in (0, 5) else 118

    def gen():
        for r in range(0, 64, 8):
            split = _splitter(const)

            def taps(i):
                return list(zip(*[split(w[3 * i + j].ld(r)) for j in range(3)]))

            def emit(i, vals, k):
                lo, hi = _gt(*vals[0], k), _gt(*vals[1], k)
                for j in range(6):
                    u.st((i * 6 + j) * 64 + r, _pack(lo[j], hi[j]))

            if row == 0:
                emit(0, taps(0), GS)
            elif row == 5:
                emit(5, taps(2), 1.0)
            else:
                nn, p = (NA, PA) if row == 1 else (NB, PB)
                g0, g1, g2 = taps(0), taps(1), taps(2)
                e = [[nn * g0[h][j] + (nn * p * p) * g2[h][j] for j in range(3)] for h in range(2)]
                o = [[(nn * p) * g1[h][j] for j in range(3)] for h in range(2)]
                emit(row, [[e[h][j] + o[h][j] for j in range(3)] for h in range(2)], GS)
                emit(row + 1, [[e[h][j] - o[h][j] for j in range(3)] for h in range(2)], GS)
            yield cost

    return gen(), 8 * cost


def _gn_coeffs(s, q, e, gamma, beta, ab):
    s = jnp.sum(s, axis=0, keepdims=True) * (1.0 / 4096)
    q = jnp.sum(q, axis=0, keepdims=True) * (1.0 / 4096)
    var_c = jnp.maximum(q - s * s, 0.0)
    mean_c = s if e is None else s + e
    mu = jnp.sum(mean_c, axis=1, keepdims=True) * (1.0 / 128)
    second = jnp.sum(var_c + mean_c * mean_c, axis=1, keepdims=True) * (1.0 / 128)
    var = jnp.maximum(second - mu * mu, 0.0)
    a = 0.5 * gamma * lax.rsqrt(var + 1e-5)
    b = 0.5 * beta + a * (-mu if e is None else e - mu)
    ab.st(0, jnp.broadcast_to(a, (8, 128)))
    ab.st(8, jnp.broadcast_to(b, (8, 128)))


def _unpack_row(x, h, y, split):
    vals = []
    for k in range(2):
        for sub in range(2):
            for i, v in enumerate(split(x.ld(sub * 16 + k, 8, 2))):
                h.st(y * 64 + (2 * k + i) * 16 + sub * 8, v)
                vals.append(v)
    return _tree(vals), _tree([v * v for v in vals])


def _job_c0(x, h, gamma, beta, ab, const):
    def gen():
        s = q = None
        for y in range(64):
            ds, dq = _unpack_row(_Rows(x.at[y // (64 // XCH)], (y % (64 // XCH)) * 32), h, y, _splitter(const))
            if y % 4 == 0 and y > 0:
                const.st(K_SUM, old[0])
                const.st(K_SQ, old[1])
            old = (s, q)
            s, q = _acc(s, ds), _acc(q, dq)
            yield C0COST
        _gn_coeffs(s, q, None, gamma[...], beta[...], ab)
        yield 40

    return gen(), 64 * C0COST + 40


def _job_a1(h, ab, t, const, k):
    def gen():
        scale = K_GN + k * MROW
        const.st(scale, ab.ld(0))
        b = ab.ld(8)

        def act(y, q, a):
            if y > 63:
                return None
            u = h.ld(y * 64 + (q % 4) * 16 + q // 4, 8, 2) * a + b
            return u * jnp.tanh(u) + u

        for q in range(8):
            d4, d5 = None, act(0, q, const.ld(scale))
            for ty in range(16):
                a = const.ld(scale)
                d0, d1 = d4, d5
                d2, d3, d4, d5 = (act(4 * ty + k, q, a) for k in range(1, 5))
                for i, val in enumerate(_bt(d0, d1, d2, d3, d4, d5)):
                    t.st((ty * 6 + i) * TREC + TPOS[q], val)
                yield A1COST

    return gen(), 128 * A1COST


def _job_a2(t, v, const, rows):
    def gen():
        for i in rows:
            for ty in range(16):
                offs = (TPOS[7] - 1,) + TPOS + (TPOS[0] + 1,)
                d = [t.ld((ty * 6 + i) * TREC + o) for o in offs]
                a2, b2 = const.ld(K_A2), const.ld(K_B2)
                for j, (lo, hi) in enumerate(zip(_bt(*d[0:6], a2, b2), _bt(*d[4:10], a2, b2))):
                    v.st((i * 6 + j) * 128 + ty * 8, _pack(lo, hi))
                yield A2COST

    return gen(), 16 * len(rows) * A2COST


def _tiles_out(m, r0, finish, cost):
    def row(i):
        return _at(*[m.ld((i * 6 + j) * MROW + r0) for j in range(6)])

    def done(i, ys):
        finish(i, [y if i + j == 3 else (PA ** (i + j) / GS) * y for j, y in enumerate(ys)])

    r1 = row(1)
    yield 13
    r2 = row(2)
    sa, ta = [x + y for x, y in zip(r1, r2)], [x - y for x, y in zip(r1, r2)]
    yield 21
    r3 = row(3)
    yield 13
    r4 = row(4)
    sb, tb = [x + y for x, y in zip(r3, r4)], [x - y for x, y in zip(r3, r4)]
    done(1, [x + RT * y for x, y in zip(ta, tb)])
    yield 32 + cost
    done(2, [x + (RT * RT) * y for x, y in zip(sa, sb)])
    done(0, [(x + y) + w for x, y, w in zip(sa, sb, row(0))])
    yield 35 + 2 * cost
    done(3, [(x + (RT * RT * RT) * y) + w for x, y, w in zip(ta, tb, row(5))])
    yield 28 + cost


def _job_c1(m, h, e, gamma, beta, ab):
    def gen():
        sq = [None, None]
        for ty in range(16):
            for sub in range(2):
                def finish(i, ys):
                    sq[0] = _acc(sq[0], _tree(ys))
                    sq[1] = _acc(sq[1], _tree([y * y for y in ys]))
                    for j in range(4):
                        h.st((4 * ty + i) * 64 + j * 16 + sub * 8, ys[j])

                before = tuple(sq)
                for n, cost in enumerate(_tiles_out(m, ty * 16 + sub * 8, finish, 12)):
                    if n == 1 and before[0] is not None:
                        m.st(K_SUM, before[0])
                        m.st(K_SQ, before[1])
                    yield cost
        _gn_coeffs(sq[0], sq[1], e[...], gamma[...], beta[...], ab)
        yield 40

    return gen(), 32 * (142 + 48) + 40


def _residual_out(m, x):
    for ty in range(16 // XCH):
        for sub in range(2):
            def finish(i, ys):
                for k in range(2):
                    off = (4 * ty + i) * 32 + sub * 16 + k
                    lo, hi = _unpack(x.ld(off, 8, 2))
                    x.st(off, _pack(lo + ys[2 * k], hi + ys[2 * k + 1]), 2)

            yield from _tiles_out(m, ty * 16 + sub * 8, finish, 10)


def _job_c2(m, x):
    return _residual_out(m, x), (32 // XCH) * (142 + 40)


def _run(*jobs):
    for gen, _ in jobs:
        for _ in gen:
            pass


def _step(v, u, m, jobs, add=False, tile_rows=ROWS, tiles=(0, 256), rows=16, tail=5):
    total = sum(c for _, c in jobs)
    pieces = itertools.chain(*[g for g, _ in jobs])
    first, count = tiles
    span = len(tile_rows) * 6 * count // rows - tail
    lead = 7 * total / span
    spent = 0

    def advance(limit):
        nonlocal spent
        while spent < limit:
            cost = next(pieces, None)
            if cost is None:
                return
            spent += cost

    tick = 0
    advance(lead)
    for xi in (6 * i + j for i in tile_rows for j in range(6)):
        lhs = jnp.concatenate([pltpu.bitcast(r.ld(xi * 128 + first // 2, count // 2), BF16) for r in v], axis=1)
        rhs = jnp.concatenate(
            [jnp.concatenate([pltpu.bitcast(r.ld(xi * 64, 64), BF16) for r in un], axis=1) for un in u], axis=0)
        res = lax.dot_general(lhs, rhs, (((1,), (1,)), ((), ())), preferred_element_type=F32)
        for r in range(0, count, rows):
            for n, mn in enumerate(m):
                val = res[r:r + rows, n * 128:(n + 1) * 128]
                at = xi * MROW + first + r
                mn.st(at, val + mn.ld(at, rows) if add else val)
            tick += 1
            advance(lead + (total - lead) * tick / span)
    advance(float("inf"))


def _kernel(x_hbm, t_hbm, g1_hbm, be1_hbm, w1_hbm, we_hbm, g2_hbm, be2_hbm, w2_hbm, o_hbm,
            t_ref, g1_ref, be1_ref, g2_ref, be2_ref,
            xbuf, wbuf, webuf, hbuf, abuf, t0, t1, t2, v0, v1, u1, u2, mbuf, par, emb, slots,
            xsem, csem, wsem, psem, osem):
    x32 = xbuf.bitcast(U32)
    w32 = wbuf.bitcast(U32)

    def lanes(g):
        return pl.ds(g * 128 if isinstance(g, int) else pl.multiple_of(g * 128, 128), 128)

    def x_copy(j):
        return pltpu.make_async_copy(x_hbm.at[j // 4, :, :, lanes(j % 4)], xbuf.at[j], xsem.at[j])

    def x_chunk_copy(j, c):
        return pltpu.make_async_copy(x_hbm.at[0, c, :, lanes(j)], xbuf.at[j, c], csem.at[j, c])

    def o_copy(b, g):
        return pltpu.make_async_copy(xbuf.at[b * 4 + g], o_hbm.at[b, :, :, lanes(g)], osem.at[b * 4 + g])

    def o_chunk_copy(c):
        return pltpu.make_async_copy(xbuf.at[7, c], o_hbm.at[1, c, :, lanes(3)], csem.at[0, c])

    def w1_copy(out_half, c):
        rows = pl.ds(out_half * 256, 256)
        return pltpu.make_async_copy(w1_hbm.at[:, rows, lanes(c)], wbuf.at[c, :, rows], wsem.at[out_half, c])

    def w1_copies(out_half, in_half):
        return [w1_copy(out_half, 2 * in_half + c) for c in range(2)]

    def w2_copies(cs):
        return [pltpu.make_async_copy(w2_hbm.at[:, :, lanes(c)], wbuf.at[4 + c], wsem.at[2, c]) for c in cs]

    def p_copies(ks):
        pairs = ((g1_hbm, g1_ref), (be1_hbm, be1_ref), (g2_hbm, g2_ref), (be2_hbm, be2_ref), (t_hbm, t_ref),
                 (we_hbm, webuf))
        return [pltpu.make_async_copy(*pairs[k], psem.at[k]) for k in ks]

    def start(copies):
        for cp in copies:
            cp.start()

    def wait(copies):
        for cp in copies:
            cp.wait()

    def load_params(ks):
        wait(p_copies(ks))
        for k in ks:
            val = (g1_ref, be1_ref, g2_ref, be2_ref)[k][...].astype(F32).reshape(4, 128)
            for g in range(4):
                par[k * 4 + g] = val[g:g + 1]

    start(p_copies((0, 1)))

    @pl.loop(0, 2 * XCH)
    def _(i):
        x_chunk_copy(i // XCH, i % XCH).start()

    @pl.loop(0, 2)
    def _(c):
        w1_copy(0, c).start()

    for t in (t0, t1, t2):
        for r in range(96):
            _Rows(t).st(r * TREC + 8, jnp.zeros((8, 128), F32))
    for k, slot in enumerate(M_SLOT):
        slots[k] = slot * MSLOT
        slots[16 + k] = slot * MSLOT
    fixed = _Rows(mbuf)
    fixed.st(K_A2, jnp.full((8, 128), A2, F32))
    fixed.st(K_B2, jnp.full((8, 128), B2, F32))
    fixed.as_u32().st(K_SHIFT, jnp.full((8, 128), 16, U32))
    fixed.as_u32().st(K_MASK, jnp.full((8, 128), 0xFFFF0000, U32))

    def m_in(k):
        return _Rows(mbuf, pl.multiple_of(slots[k], 8))

    def m_out(k, count=1):
        base = pl.multiple_of(slots[16 + k], 8)
        return [_Rows(mbuf, base + i * MSLOT) for i in range(count)]

    def h_slot(j):
        return _Rows(hbuf, j * 4096)

    def ab_slot(j):
        return _Rows(abuf, j * 16)

    def taps(conv, n, c):
        rows = n * 64 if isinstance(n, int) else pl.multiple_of(n * 64, 64)
        return [_Rows(w32.at[conv * 4 + c, k], rows) for k in range(9)]

    def u1_jobs(blocks, rows, const):
        return [_job_u(taps(0, n, c), _Rows(u1.at[n * 4 + c]), const, row) for n, c in blocks for row in rows]

    def u2_jobs(u, n, first, cs):
        return [_job_u(taps(1, n, c), _Rows(u.at[(n - first) * 4 + c]), const, row)
                for c in cs for row in (0, 5, 1, 3)]

    def quad(out_half, in_half):
        return [(2 * out_half + n, 2 * in_half + c) for n in range(2) for c in range(2)]

    def c0(j):
        return _job_c0(x32.at[j], h_slot(j), par.at[j % 4], par.at[4 + j % 4], ab_slot(j), const)

    def a1(j, k):
        return _job_a1(h_slot(j), ab_slot(j), _Rows((t0, t1, t2)[k]), const, k)

    def a2(v, g, k, rows=ROWS):
        return _job_a2(_Rows((t0, t1, t2)[k]), _Rows(v.at[g]), const, rows)

    def c1(j):
        return _job_c1(m_in(j), h_slot(j), emb.at[j], par.at[8 + j % 4], par.at[12 + j % 4], ab_slot(j))

    def c2(j, c):
        m = m_in(8 + j)
        return _job_c2(_Rows(mbuf, m.base + c * (256 // XCH)), _Rows(x32.at[j, c]))

    def block(fn):
        pl.when(slots[0] == 0)(fn)

    def half_step(out_half, in_half, jobs, rows=ROWS):
        ins = (2 * in_half, 2 * in_half + 1)
        outs = (2 * out_half, 2 * out_half + 1)
        block(lambda: _step([_Rows(v0.at[c]) for c in ins], [[_Rows(u1.at[n * 4 + c]) for c in ins] for n in outs],
                            m_out(outs[0], 2), jobs, add=bool(in_half), tile_rows=rows, rows=8, tail=8))

    def step(slot, v, u, n, jobs, **kwargs):
        block(lambda: _step([_Rows(v.at[c]) for c in range(4)], [[_Rows(u.at[n * 4 + c]) for c in range(4)]],
                            m_out(slot), jobs, **kwargs))

    @pl.loop(0, 2)
    def _(j):
        def unpack_chunk(c, sums):
            x_chunk_copy(j, c).wait()
            h = _Rows(hbuf, j * 4096 + c * (4096 // XCH))
            s, q = sums
            for y in range(64 // XCH):
                ds, dq = _unpack_row(_Rows(x32.at[j, c], y * 32), h, y, _unpack)
                s, q = s + ds, q + dq
            return s, q

        s, q = lax.fori_loop(0, XCH, unpack_chunk, (jnp.zeros((8, 128), F32),) * 2)

        @pl.when(j == 0)
        def _():
            load_params((0, 1))
            x_copy(2).start()
            _gn_coeffs(s, q, None, par[0], par[4], ab_slot(0))

        @pl.when(j == 1)
        def _():
            _gn_coeffs(s, q, None, par[1], par[5], ab_slot(1))
            _run(_job_a2(_Rows(t0), _Rows(v0.at[0]), fixed, ROWS[4:]))

        _run(_job_a1(h_slot(j), ab_slot(j), _Rows(t0), fixed, 0),
             _job_a2(_Rows(t0), _Rows(v0.at[j]), fixed, ROWS[:4]))

        @pl.when(j == 0)
        def _():
            start(w1_copies(1, 0))

    @pl.loop(0, 2)
    def _(c):
        w1_copy(0, c).wait()
        _run(*u1_jobs([(0, c), (1, c)], (0, 5), fixed))

    const = m_in(0)
    every = (0, 5, 1, 3)
    start([x_copy(3)] + w1_copies(0, 1))
    half_step(0, 0, u1_jobs(quad(0, 0), (1,), const) + [a2(v0, 1, 0, ROWS[4:])]
              + u1_jobs(quad(0, 0)[:2], (3,), const), ROWS[:2])
    wait([x_copy(2)])
    start(w1_copies(1, 1) + [x_copy(j) for j in range(4, 8)])
    half_step(0, 0, [c0(2)] + u1_jobs(quad(0, 0)[2:], (3,), const), ROWS[2:3])
    wait(w1_copies(1, 0))
    half_step(0, 0, [a1(2, 1)] + u1_jobs(quad(1, 0), every, const), ROWS[3:])
    wait([x_copy(3)] + w1_copies(0, 1))
    half_step(1, 0, [c0(3), a2(v0, 2, 1), a1(3, 0), a2(v0, 3, 0)] + u1_jobs(quad(0, 1), every, const))
    wait(w1_copies(1, 1) + [x_copy(j) for j in range(4, 8)])
    start(p_copies((5, 2, 3, 4)) + w2_copies((0, 1)))
    half_step(0, 1, [job for i, b in enumerate(quad(1, 1)) for job in [c0(4 + i)] + u1_jobs([b], every, const)]
              + [a1(4, 1)])
    half_step(1, 1, [a2(v1, 0, 1), a1(5, 0), a1(6, 1), a1(7, 2)] + [a2(v1, 1 + k, k, ROWS[:3]) for k in range(3)])

    load_params((2, 3))
    wait(p_copies((4, 5)) + w2_copies((0, 1)))
    start(w2_copies((2, 3)))

    def embed():
        th = t_ref[...].astype(F32) * 0.5
        e = jnp.dot((th * jnp.tanh(th) + th).astype(BF16), webuf[...], preferred_element_type=F32)
        for j in range(8):
            emb[j] = e[j // 4:j // 4 + 1, (j % 4) * 128:(j % 4 + 1) * 128]
        yield 0

    step(4, v1, u1, 0, [(embed(), 0)] + [a2(v1, 1 + k, k, (i,)) for i in ROWS[3:] for k in range(3)] + [c1(0), c1(1)]
         + u2_jobs(u2, 0, 0, (0, 1)))
    wait(w2_copies((2, 3)))
    step(5, v1, u1, 1, [a1(0, 0), a2(v0, 0, 0), c1(2), c1(3)] + u2_jobs(u2, 0, 0, (2, 3)))
    step(6, v1, u1, 2, [a1(1, 1), a2(v0, 1, 1), a1(2, 2), a2(v0, 2, 2), c1(4), (iter([500]), 500)])
    step(7, v1, u1, 3, [a1(3, 0), a2(v0, 3, 0), c1(5)] + u2_jobs(u2, 1, 0, range(4)))

    @pl.loop(0, 2)
    def _(n):
        step(8 + n, v0, u2, n, [a1(4 + n, 1), a2(v1, n, 1), c1(6 + n)] + u2_jobs(u1, 2 + n, 0, range(4)))

    @pl.loop(2, 4)
    def _(n):
        step(8 + n, v0, u1, n, [a1(4 + n, 0), a2(v1, n, 0)] + [c2(n - 2, c) for c in range(XCH)])
        o_copy(0, n - 2).start()

    step(14, v1, u1, 2, [c2(j, c) for j in (2, 3) for c in range(XCH)])
    start([o_copy(0, 2), o_copy(0, 3)])

    @pl.loop(0, 2)
    def _(n):
        done = 2 - 2 * n
        step(12 + n, v1, u2, n, [c2(4 + done, c) for c in range(XCH)])
        o_copy(1, done).start()

    step(15, v1, u1, 3, [c2(5, c) for c in range(XCH)], tiles=(0, 128))
    o_copy(1, 1).start()
    step(15, v1, u1, 3, [c2(7, 0), c2(7, 1)], tiles=(128, 64))
    start([o_chunk_copy(0), o_chunk_copy(1)])
    step(15, v1, u1, 3, [c2(7, 2)], tiles=(192, 64))
    o_chunk_copy(2).start()
    _run(c2(7, 3))
    o_chunk_copy(3).start()

    wait([o_copy(j // 4, j % 4) for j in range(7)] + [o_chunk_copy(c) for c in range(XCH)])


@jax.jit
def pallas_standalone__adm_resblock__diffusion_kernel(
    x: jax.Array,
    t_emb: jax.Array,
    g1: jax.Array,
    be1: jax.Array,
    w1: jax.Array,
    w_emb: jax.Array,
    g2: jax.Array,
    be2: jax.Array,
    w2: jax.Array,
):
    B, C, H, W = x.shape
    assert (B, C, H, W) == (2, 512, 64, 64)
    xt = jnp.transpose(x, (0, 2, 3, 1)).reshape(B, XCH, H * W // XCH, C)
    w1t = jnp.transpose(w1, (2, 3, 0, 1)).reshape(9, C, C)
    w2t = jnp.transpose(w2, (2, 3, 0, 1)).reshape(9, C, C)
    hbm = pl.BlockSpec(memory_space=pl.ANY)
    out = pl.pallas_call(
        _kernel,
        out_shape=jax.ShapeDtypeStruct(xt.shape, x.dtype),
        in_specs=[hbm] * 9,
        out_specs=hbm,
        scratch_shapes=[
            pltpu.VMEM(t_emb.shape, BF16),
            pltpu.VMEM(g1.shape, BF16),
            pltpu.VMEM(be1.shape, BF16),
            pltpu.VMEM(g2.shape, BF16),
            pltpu.VMEM(be2.shape, BF16),
            pltpu.VMEM((8, XCH, 4096 // XCH, 128), BF16),
            pltpu.VMEM((8, 9, 512, 128), BF16),
            pltpu.VMEM(w_emb.shape, BF16),
            pltpu.VMEM((8 * 4096, 128), F32),
            pltpu.VMEM((8 * 16, 128), F32),
            pltpu.VMEM((96 * TREC, 128), F32),
            pltpu.VMEM((96 * TREC, 128), F32),
            pltpu.VMEM((96 * TREC, 128), F32),
            pltpu.VMEM((4, 36 * 128, 128), U32),
            pltpu.VMEM((4, 36 * 128, 128), U32),
            pltpu.VMEM((16, 36 * 64, 128), U32),
            pltpu.VMEM((8, 36 * 64, 128), U32),
            pltpu.VMEM((5 * MSLOT, 128), F32),
            pltpu.VMEM((16, 1, 128), F32),
            pltpu.VMEM((8, 1, 128), F32),
            pltpu.SMEM((32,), jnp.int32),
            pltpu.SemaphoreType.DMA((8,)),
            pltpu.SemaphoreType.DMA((2, XCH)),
            pltpu.SemaphoreType.DMA((3, 4)),
            pltpu.SemaphoreType.DMA((6,)),
            pltpu.SemaphoreType.DMA((7,)),
        ],
        compiler_params=pltpu.CompilerParams(vmem_limit_bytes=120 * 2**20, disable_bounds_checks=True),
        name="resblk",
    )(xt, t_emb, g1, be1, w1t, w_emb, g2, be2, w2t)
    return jnp.transpose(out.reshape(B, H, W, C), (0, 3, 1, 2))
```

```python
import itertools

import jax
import jax.numpy as jnp
import numpy as np
from jax import lax
import jax.experimental.pallas as pl
import jax.experimental.pallas.tpu as pltpu

F32 = jnp.float32
BF16 = jnp.bfloat16
U32 = jnp.uint32

PA = 2.0 / 3.0
PB = 1.5
A2, B2 = PA * PA, PB * PB
NA = 1.0 / (2 * A2 * (A2 - B2))
NB = 1.0 / (2 * B2 * (B2 - A2))
RT = PB / PA
GS = PA ** 3
ROWS = (0, 5, 1, 2, 3, 4)

TPOS = (0, 24, 32, 40, 48, 56, 64, 16)
TREC = 72
XCH = 4
MROW = 264
MSLOT = 36 * MROW
M_SLOT = (0, 1, 2, 3, 4, 0, 1, 2, 3, 4, 0, 1, 3, 4, 2, 0)
K_A2, K_B2, K_BITS, K_ZERO, K_SUM, K_SQ, K_GN = (i * MROW + 256 for i in range(7))

K_G = K_GN + 3 * MROW
C0COST, A1COST, A2COST = 38, 34, 46


def _bt(d0, d1, d2, d3, d4, d5, a2=A2, b2=B2):
    t, u = a2 * d2, b2 * d2
    ea, eb = d4 - u, d4 - t
    v0 = ea - t
    if d0 is not None:
        v0 = v0 + d0
    t3, u3 = a2 * d3, b2 * d3
    pa, pb = t3 - d1, u3 - d1
    v5 = (d5 - pa) - u3 if d5 is not None else (d1 - t3) - u3
    oa, ob = PB * pa, PA * pb
    return v0, ea + oa, ea - oa, eb + ob, eb - ob, v5


def _at(m0, m1, m2, m3, m4, m5):
    sa, ta, sb, tb = m1 + m2, m1 - m2, m3 + m4, m3 - m4
    return (m0 + sa) + sb, ta + RT * tb, sa + (RT * RT) * sb, (ta + m5) + (RT * RT * RT) * tb


def _gt(g0, g1, g2, k):
    ea, oa = (k * NA) * g0 + (k * NA * A2) * g2, (k * NA * PA) * g1
    eb, ob = (k * NB) * g0 + (k * NB * B2) * g2, (k * NB * PB) * g1
    k5 = k / PA ** 3
    u0 = g0 if abs(k - 1.0) < 1e-12 else k * g0
    u5 = g2 if abs(k5 - 1.0) < 1e-12 else k5 * g2
    return u0, ea + oa, ea - oa, eb + ob, eb - ob, u5


def _stack(top, bottom):
    return jnp.concatenate([top, bottom], axis=0).astype(BF16)


def _pair(lo, hi):
    bits = lax.bitcast_convert_type(_stack(lo, hi).astype(F32), U32)
    return (bits[:8] >> 16) | (bits[8:] & np.uint32(0xFFFF0000))


def _unpair(w, shift=16, mask=np.uint32(0xFFFF0000)):
    return lax.bitcast_convert_type(w << shift, F32), lax.bitcast_convert_type(w & mask, F32)


def _tree(xs):
    while len(xs) > 1:
        xs = [xs[i] + xs[i + 1] for i in range(0, len(xs), 2)]
    return xs[0]


def _acc(a, x):
    return x if a is None else a + x


class _Rows:
    def __init__(self, ref, base=0):
        self.ref, self.base = ref, base

    def ld(self, off, n=8, stride=1):
        return self.ref[pl.ds(self.base + off, n, stride=stride), :]

    def st(self, off, val, stride=1):
        self.ref[pl.ds(self.base + off, val.shape[0], stride=stride), :] = val


def _splitter(const):
    bits = lax.bitcast_convert_type(const.ld(K_BITS), U32)
    shift, mask = bits & 16, bits << 16
    return lambda w: _unpair(w, shift, mask)


def _job_u(w, u, const, rows):
    needed = sorted({i for row in rows for i in {0: (0,), 5: (2,)}.get(row, (0, 1, 2))})
    cost = 9 * len(needed) + sum(32 if row in (0, 5) else 100 for row in rows)

    def gen():
        for r in range(0, 64, 8):
            zero = lax.bitcast_convert_type(const.ld(K_ZERO), U32)
            g = {}
            for i in needed:
                taps = [pltpu.bitcast(w[3 * i + j].ld(r) | zero, BF16).astype(F32) for j in range(3)]
                g[i] = [v[:8] for v in taps], [v[8:] for v in taps]

            def emit(i, vals, k):
                top, bottom = _gt(*vals[0], k), _gt(*vals[1], k)
                for j in range(6):
                    u.st((i * 6 + j) * 128 + 2 * r, _stack(top[j], bottom[j]))

            for n, row in enumerate(rows):
                if row == 0:
                    emit(0, g[0], GS)
                elif row == 5:
                    emit(5, g[2], 1.0)
                else:
                    k0, k1, k2 = (const.ld(K_G + (3 * (row // 2) + i) * MROW) for i in range(3))
                    e = [[k0 * g[0][h][j] + k2 * g[2][h][j] for j in range(3)] for h in range(2)]
                    o = [[k1 * g[1][h][j] for j in range(3)] for h in range(2)]
                    emit(row, [[e[h][j] + o[h][j] for j in range(3)] for h in range(2)], GS)
                    emit(row + 1, [[e[h][j] - o[h][j] for j in range(3)] for h in range(2)], GS)
                yield (32 if row in (0, 5) else 100) + (9 * len(needed) if n == 0 else 0)

    return gen(), 8 * cost


def _gn_coeffs(s, q, e, gamma, beta, ab):
    s = jnp.sum(s, axis=0, keepdims=True) * (1.0 / 4096)
    q = jnp.sum(q, axis=0, keepdims=True) * (1.0 / 4096)
    var_c = jnp.maximum(q - s * s, 0.0)
    mean_c = s if e is None else s + e
    mu = jnp.sum(mean_c, axis=1, keepdims=True) * (1.0 / 128)
    second = jnp.sum(var_c + mean_c * mean_c, axis=1, keepdims=True) * (1.0 / 128)
    var = jnp.maximum(second - mu * mu, 0.0)
    a = 0.5 * gamma * lax.rsqrt(var + 1e-5)
    b = 0.5 * beta + a * (-mu if e is None else e - mu)
    ab.st(0, jnp.broadcast_to(a, (8, 128)))
    ab.st(8, jnp.broadcast_to(b, (8, 128)))


def _unpack_row(x, h, y, split):
    vals = [v for k in range(4) for v in split(x.ld(k, 8, 4))]
    for q, v in enumerate(vals):
        h.st(y * 64 + q * 8, v)
    return _tree(vals), _tree([v * v for v in vals])


def _job_c0(x, h, gamma, beta, ab, const):
    def gen():
        s = q = None
        for y in range(64):
            ds, dq = _unpack_row(_Rows(x[y // (64 // XCH)], (y % (64 // XCH)) * 32), h, y, _splitter(const))
            if y % 4 == 0 and y > 0:
                const.st(K_SUM, old[0])
                const.st(K_SQ, old[1])
            old = (s, q)
            s, q = _acc(s, ds), _acc(q, dq)
            yield C0COST
        _gn_coeffs(s, q, None, gamma[...], beta[...], ab)
        yield 40

    return gen(), 64 * C0COST + 40


def _job_a1(h, ab, t, const, k):
    def gen():
        scale = K_GN + k * MROW
        const.st(scale, ab.ld(0))
        b = ab.ld(8)

        def act(y, q, a):
            if y > 63:
                return None
            u = h.ld(y * 64 + q * 8) * a + b
            return u * jnp.tanh(u) + u

        for q in range(8):
            d4, d5 = None, act(0, q, const.ld(scale))
            for ty in range(16):
                a = const.ld(scale)
                d0, d1 = d4, d5
                d2, d3, d4, d5 = (act(4 * ty + k, q, a) for k in range(1, 5))
                for i, val in enumerate(_bt(d0, d1, d2, d3, d4, d5)):
                    t.st((ty * 6 + i) * TREC + TPOS[q], val)
                yield A1COST

    return gen(), 128 * A1COST


def _job_a2(t, v, const, rows):
    def gen():
        for i in rows:
            for ty in range(16):
                offs = (TPOS[7] - 1,) + TPOS + (TPOS[0] + 1,)
                d = [t.ld((ty * 6 + i) * TREC + o) for o in offs]
                a2, b2 = const.ld(K_A2), const.ld(K_B2)
                for j, (lo, hi) in enumerate(zip(_bt(*d[0:6], a2, b2), _bt(*d[4:10], a2, b2))):
                    v.st((i * 6 + j) * 256 + ty * 16, _stack(lo, hi))
                yield A2COST

    return gen(), 16 * len(rows) * A2COST


def _tiles_out(m, r0, finish, cost):
    def row(i):
        return _at(*[m.ld((i * 6 + j) * MROW + r0) for j in range(6)])

    def done(i, ys):
        finish(i, [y if i + j == 3 else (PA ** (i + j) / GS) * y for j, y in enumerate(ys)])

    r1 = row(1)
    yield 13
    r2 = row(2)
    sa, ta = [x + y for x, y in zip(r1, r2)], [x - y for x, y in zip(r1, r2)]
    yield 21
    r3 = row(3)
    yield 13
    r4 = row(4)
    sb, tb = [x + y for x, y in zip(r3, r4)], [x - y for x, y in zip(r3, r4)]
    done(1, [x + RT * y for x, y in zip(ta, tb)])
    yield 32 + cost
    done(2, [x + (RT * RT) * y for x, y in zip(sa, sb)])
    done(0, [(x + y) + w for x, y, w in zip(sa, sb, row(0))])
    yield 35 + 2 * cost
    done(3, [(x + (RT * RT * RT) * y) + w for x, y, w in zip(ta, tb, row(5))])
    yield 28 + cost


def _job_c1(m, h, e, gamma, beta, ab):
    def gen():
        sq = [None, None]
        for ty in range(16):
            for sub in range(2):
                def finish(i, ys):
                    sq[0] = _acc(sq[0], _tree(ys))
                    sq[1] = _acc(sq[1], _tree([y * y for y in ys]))
                    for j in range(4):
                        h.st((4 * ty + i) * 64 + (4 * sub + j) * 8, ys[j])

                before = tuple(sq)
                for n, cost in enumerate(_tiles_out(m, ty * 16 + sub * 8, finish, 12)):
                    if n == 1 and before[0] is not None:
                        m.st(K_SUM, before[0])
                        m.st(K_SQ, before[1])
                    yield cost
        _gn_coeffs(sq[0], sq[1], e[...], gamma[...], beta[...], ab)
        yield 40

    return gen(), 32 * (142 + 48) + 40


def _residual_out(m, x):
    for ty in range(16 // XCH):
        for sub in range(2):
            def finish(i, ys):
                for k in range(2):
                    off = (4 * ty + i) * 32 + 2 * sub + k
                    lo, hi = _unpair(x.ld(off, 8, 4))
                    x.st(off, _pair(lo + ys[2 * k], hi + ys[2 * k + 1]), 4)

            yield from _tiles_out(m, ty * 16 + sub * 8, finish, 18)


def _job_c2(m, x):
    return _residual_out(m, x), (32 // XCH) * (142 + 72)


def _run(*jobs):
    for gen, _ in jobs:
        for _ in gen:
            pass


def _step(v, u, m, jobs, add=False, tile_rows=ROWS, tiles=(0, 256), rows=16, tail=5):
    total = sum(c for _, c in jobs)
    pieces = itertools.chain(*[g for g, _ in jobs])
    first, count = tiles
    span = len(tile_rows) * 6 * count // rows - tail
    lead = 7 * total / span
    spent = 0

    def advance(limit):
        nonlocal spent
        while spent < limit:
            cost = next(pieces, None)
            if cost is None:
                return
            spent += cost

    tick = 0
    advance(lead)
    for xi in (6 * i + j for i in tile_rows for j in range(6)):
        lhs = jnp.concatenate([pltpu.bitcast(r.ld(xi * 128 + first // 2, count // 2), BF16) for r in v], axis=1)
        rhs = jnp.concatenate(
            [jnp.concatenate([pltpu.bitcast(r.ld(xi * 64, 64), BF16) for r in un], axis=1) for un in u], axis=0)
        res = lax.dot_general(lhs, rhs, (((1,), (1,)), ((), ())), preferred_element_type=F32)
        for r in range(0, count, rows):
            for n, mn in enumerate(m):
                val = res[r:r + rows, n * 128:(n + 1) * 128]
                at = xi * MROW + first + r
                mn.st(at, val + mn.ld(at, rows) if add else val)
            tick += 1
            advance(lead + (total - lead) * tick / span)
    advance(float("inf"))


def _kernel(x_hbm, t_hbm, g1_hbm, be1_hbm, w1_hbm, we_hbm, g2_hbm, be2_hbm, w2_hbm, o_hbm,
            t_ref, g1_ref, be1_ref, g2_ref, be2_ref,
            xbuf, wbuf, webuf, hbuf, abuf, t0, t1, t2, v0, v1, u1, u2, mbuf, par, emb, slots,
            xsem, csem, wsem, psem, osem):

    def x_words(j, c):
        return xbuf.at[j, c].bitcast(U32)

    def words(ref, k):
        return _Rows(ref.at[k].bitcast(U32))

    body = pl.ds(0, 4096 // XCH)

    def lanes(g):
        return pl.ds(g * 128 if isinstance(g, int) else pl.multiple_of(g * 128, 128), 128)

    def x_copy(j):
        return pltpu.make_async_copy(x_hbm.at[j // 4, :, :, lanes(j % 4)], xbuf.at[j, :, body], xsem.at[j])

    def x_chunk_copy(j, c):
        return pltpu.make_async_copy(x_hbm.at[0, c, :, lanes(j)], xbuf.at[j, c, body], csem.at[j, c])

    def o_copy(b, g):
        return pltpu.make_async_copy(xbuf.at[b * 4 + g, :, body], o_hbm.at[b, :, :, lanes(g)], osem.at[b * 4 + g])

    def o_chunk_copy(c):
        return pltpu.make_async_copy(xbuf.at[7, c, body], o_hbm.at[1, c, :, lanes(3)], csem.at[0, c])

    def w1_copy(out_half, c):
        rows = pl.ds(out_half * 256, 256)
        return pltpu.make_async_copy(w1_hbm.at[:, rows, lanes(c)], wbuf.at[c, :, rows], wsem.at[out_half, c])

    def w1_copies(out_half, in_half):
        return [w1_copy(out_half, 2 * in_half + c) for c in range(2)]

    def w2_copies(cs):
        return [pltpu.make_async_copy(w2_hbm.at[:, :, lanes(c)], wbuf.at[4 + c], wsem.at[2, c]) for c in cs]

    def p_copies(ks):
        pairs = ((g1_hbm, g1_ref), (be1_hbm, be1_ref), (g2_hbm, g2_ref), (be2_hbm, be2_ref), (t_hbm, t_ref),
                 (we_hbm, webuf))
        return [pltpu.make_async_copy(*pairs[k], psem.at[k]) for k in ks]

    def start(copies):
        for cp in copies:
            cp.start()

    def wait(copies):
        for cp in copies:
            cp.wait()

    def load_params(ks):
        wait(p_copies(ks))
        for k in ks:
            val = (g1_ref, be1_ref, g2_ref, be2_ref)[k][...].astype(F32).reshape(4, 128)
            for g in range(4):
                par[k * 4 + g] = val[g:g + 1]

    start(p_copies((0, 1)))

    @pl.loop(0, 2 * XCH)
    def _(i):
        x_chunk_copy(i // XCH, i % XCH).start()

    @pl.loop(0, 2)
    def _(c):
        w1_copy(0, c).start()

    for t in (t0, t1, t2):
        for r in range(96):
            _Rows(t).st(r * TREC + 8, jnp.zeros((8, 128), F32))
    for k, slot in enumerate(M_SLOT):
        slots[k] = slot * MSLOT
        slots[16 + k] = slot * MSLOT
    fixed = _Rows(mbuf)
    fixed.st(K_A2, jnp.full((8, 128), A2, F32))
    fixed.st(K_B2, jnp.full((8, 128), B2, F32))
    fixed.st(K_BITS, lax.bitcast_convert_type(jnp.full((8, 128), 0x3F80FFFF, U32), F32))
    for i, value in enumerate((NA, NA * PA, NA * A2, NB, NB * PB, NB * B2)):
        fixed.st(K_G + i * MROW, jnp.full((8, 128), value, F32))
    fixed.st(K_ZERO, jnp.zeros((8, 128), F32))

    def m_in(k):
        return _Rows(mbuf, pl.multiple_of(slots[k], 8))

    def m_out(k, count=1):
        base = pl.multiple_of(slots[16 + k], 8)
        return [_Rows(mbuf, base + i * MSLOT) for i in range(count)]

    def h_slot(j):
        return _Rows(hbuf, j * 4096)

    def ab_slot(j):
        return _Rows(abuf, j * 16)

    def taps(conv, n, c):
        return [_Rows(wbuf.at[conv * 4 + c, k, lanes(n)].bitcast(U32)) for k in range(9)]

    every = [(0, 1), (5, 3)]

    def u1_jobs(blocks, rows, const):
        return [_job_u(taps(0, n, c), _Rows(u1.at[n * 4 + c]), const, row) for n, c in blocks for row in rows]

    def u2_jobs(u, n, first, cs):
        return [_job_u(taps(1, n, c), _Rows(u.at[(n - first) * 4 + c]), const, row)
                for c in cs for row in every]

    def quad(out_half, in_half):
        return [(2 * out_half + n, 2 * in_half + c) for n in range(2) for c in range(2)]

    def c0(j):
        return _job_c0([x_words(j, c) for c in range(XCH)], h_slot(j), par.at[j % 4], par.at[4 + j % 4], ab_slot(j), const)

    def a1(j, k):
        return _job_a1(h_slot(j), ab_slot(j), _Rows((t0, t1, t2)[k]), const, k)

    def a2(v, g, k, rows=ROWS):
        return _job_a2(_Rows((t0, t1, t2)[k]), _Rows(v.at[g]), const, rows)

    def c1(j):
        return _job_c1(m_in(j), h_slot(j), emb.at[j], par.at[8 + j % 4], par.at[12 + j % 4], ab_slot(j))

    def c2(j, c):
        m = m_in(8 + j)
        return _job_c2(_Rows(mbuf, m.base + c * (256 // XCH)), _Rows(x_words(j, c)))

    def block(fn):
        pl.when(slots[0] == 0)(fn)

    def half_step(out_half, in_half, jobs, rows=ROWS):
        ins = (2 * in_half, 2 * in_half + 1)
        outs = (2 * out_half, 2 * out_half + 1)
        block(lambda: _step([words(v0, c) for c in ins], [[words(u1, n * 4 + c) for c in ins] for n in outs],
                            m_out(outs[0], 2), jobs, add=bool(in_half), tile_rows=rows, rows=8, tail=8))

    def step(slot, v, u, n, jobs, **kwargs):
        block(lambda: _step([words(v, c) for c in range(4)], [[words(u, n * 4 + c) for c in range(4)]],
                            m_out(slot), jobs, **kwargs))

    @pl.loop(0, 2)
    def _(j):
        def unpack_chunk(c, sums):
            x_chunk_copy(j, c).wait()
            h = _Rows(hbuf, j * 4096 + c * (4096 // XCH))
            s, q = sums
            for y in range(64 // XCH):
                ds, dq = _unpack_row(_Rows(x_words(j, c), y * 32), h, y, _unpair)
                s, q = s + ds, q + dq
            return s, q

        s, q = lax.fori_loop(0, XCH, unpack_chunk, (jnp.zeros((8, 128), F32),) * 2)

        @pl.when(j == 0)
        def _():
            load_params((0, 1))
            x_copy(2).start()
            _gn_coeffs(s, q, None, par[0], par[4], ab_slot(0))

        @pl.when(j == 1)
        def _():
            _gn_coeffs(s, q, None, par[1], par[5], ab_slot(1))
            _run(_job_a2(_Rows(t0), _Rows(v0.at[0]), fixed, ROWS[4:]))

        _run(_job_a1(h_slot(j), ab_slot(j), _Rows(t0), fixed, 0),
             _job_a2(_Rows(t0), _Rows(v0.at[j]), fixed, ROWS[:4]))

        @pl.when(j == 0)
        def _():
            start(w1_copies(1, 0))

    @pl.loop(0, 2)
    def _(c):
        w1_copy(0, c).wait()
        _run(*u1_jobs([(0, c), (1, c)], [(0, 5)], fixed))

    const = m_in(0)
    start([x_copy(3)] + w1_copies(0, 1))
    half_step(0, 0, u1_jobs(quad(0, 0), [(1,)], const) + [a2(v0, 1, 0, ROWS[4:])]
              + u1_jobs(quad(0, 0)[:2], [(3,)], const), ROWS[:2])
    wait([x_copy(2)])
    start(w1_copies(1, 1) + [x_copy(j) for j in range(4, 8)])
    half_step(0, 0, [c0(2)] + u1_jobs(quad(0, 0)[2:], [(3,)], const), ROWS[2:3])
    wait(w1_copies(1, 0))
    half_step(0, 0, [a1(2, 1)] + u1_jobs(quad(1, 0), every, const), ROWS[3:])
    wait([x_copy(3)] + w1_copies(0, 1))
    half_step(1, 0, [c0(3), a2(v0, 2, 1), a1(3, 0), a2(v0, 3, 0)] + u1_jobs(quad(0, 1), every, const))
    wait(w1_copies(1, 1) + [x_copy(j) for j in range(4, 8)])
    start(p_copies((5, 2, 3, 4)) + w2_copies((0, 1)))
    half_step(0, 1, [job for i, b in enumerate(quad(1, 1)) for job in [c0(4 + i)] + u1_jobs([b], every, const)]
              + [a1(4, 1)])
    half_step(1, 1, [a2(v1, 0, 1), a1(5, 0), a1(6, 1), a1(7, 2)] + [a2(v1, 1 + k, k, ROWS[:3]) for k in range(3)])

    load_params((2, 3))
    wait(p_copies((4, 5)) + w2_copies((0, 1)))
    start(w2_copies((2, 3)))

    def embed():
        th = t_ref[...].astype(F32) * 0.5
        e = jnp.dot((th * jnp.tanh(th) + th).astype(BF16), webuf[...], preferred_element_type=F32)
        for j in range(8):
            emb[j] = e[j // 4:j // 4 + 1, (j % 4) * 128:(j % 4 + 1) * 128]
        yield 0

    step(4, v1, u1, 0, [(embed(), 0)] + [a2(v1, 1 + k, k, (i,)) for i in ROWS[3:] for k in range(3)] + [c1(0), c1(1)]
         + u2_jobs(u2, 0, 0, (0, 1)))
    wait(w2_copies((2, 3)))
    step(5, v1, u1, 1, [a1(0, 0), a2(v0, 0, 0), c1(2), c1(3)] + u2_jobs(u2, 0, 0, (2, 3)))
    step(6, v1, u1, 2, [a1(1, 1), a2(v0, 1, 1), a1(2, 2), a2(v0, 2, 2), c1(4), (iter([500]), 500)])
    step(7, v1, u1, 3, [a1(3, 0), a2(v0, 3, 0), c1(5)] + u2_jobs(u2, 1, 0, range(4)))

    @pl.loop(0, 2)
    def _(n):
        step(8 + n, v0, u2, n, [a1(4 + n, 1), a2(v1, n, 1), c1(6 + n)] + u2_jobs(u1, 2 + n, 0, range(4)))

    @pl.loop(2, 4)
    def _(n):
        step(8 + n, v0, u1, n, [a1(4 + n, 0), a2(v1, n, 0)] + [c2(n - 2, c) for c in range(XCH)])
        o_copy(0, n - 2).start()

    step(14, v1, u1, 2, [c2(j, c) for j in (2, 3) for c in range(XCH)])
    start([o_copy(0, 2), o_copy(0, 3)])

    @pl.loop(0, 2)
    def _(n):
        done = 2 - 2 * n
        step(12 + n, v1, u2, n, [c2(4 + done, c) for c in range(XCH)])
        o_copy(1, done).start()

    step(15, v1, u1, 3, [c2(5, c) for c in range(XCH)], tiles=(0, 128))
    o_copy(1, 1).start()
    step(15, v1, u1, 3, [c2(7, 0), c2(7, 1)], tiles=(128, 64))
    start([o_chunk_copy(0), o_chunk_copy(1)])
    step(15, v1, u1, 3, [c2(7, 2)], tiles=(192, 64))
    o_chunk_copy(2).start()
    _run(c2(7, 3))
    o_chunk_copy(3).start()

    wait([o_copy(j // 4, j % 4) for j in range(7)] + [o_chunk_copy(c) for c in range(XCH)])


@jax.jit
def pallas_standalone__adm_resblock__diffusion_kernel(
    x: jax.Array,
    t_emb: jax.Array,
    g1: jax.Array,
    be1: jax.Array,
    w1: jax.Array,
    w_emb: jax.Array,
    g2: jax.Array,
    be2: jax.Array,
    w2: jax.Array,
):
    B, C, H, W = x.shape
    assert (B, C, H, W) == (2, 512, 64, 64)
    xt = jnp.transpose(x, (0, 2, 3, 1)).reshape(B, XCH, H * W // XCH, C)
    w1t = jnp.transpose(w1, (2, 3, 0, 1)).reshape(9, C, C)
    w2t = jnp.transpose(w2, (2, 3, 0, 1)).reshape(9, C, C)
    hbm = pl.BlockSpec(memory_space=pl.ANY)
    out = pl.pallas_call(
        _kernel,
        out_shape=jax.ShapeDtypeStruct(xt.shape, x.dtype),
        in_specs=[hbm] * 9,
        out_specs=hbm,
        scratch_shapes=[
            pltpu.VMEM(t_emb.shape, BF16),
            pltpu.VMEM(g1.shape, BF16),
            pltpu.VMEM(be1.shape, BF16),
            pltpu.VMEM(g2.shape, BF16),
            pltpu.VMEM(be2.shape, BF16),
            pltpu.VMEM((8, XCH, 4096 // XCH + 16, 128), BF16),
            pltpu.VMEM((8, 9, 512, 128), BF16),
            pltpu.VMEM(w_emb.shape, BF16),
            pltpu.VMEM((8 * 4096, 128), F32),
            pltpu.VMEM((8 * 16, 128), F32),
            pltpu.VMEM((96 * TREC, 128), F32),
            pltpu.VMEM((96 * TREC, 128), F32),
            pltpu.VMEM((96 * TREC, 128), F32),
            pltpu.VMEM((4, 36 * 256, 128), BF16),
            pltpu.VMEM((4, 36 * 256, 128), BF16),
            pltpu.VMEM((16, 36 * 128, 128), BF16),
            pltpu.VMEM((8, 36 * 128, 128), BF16),
            pltpu.VMEM((5 * MSLOT, 128), F32),
            pltpu.VMEM((16, 1, 128), F32),
            pltpu.VMEM((8, 1, 128), F32),
            pltpu.SMEM((32,), jnp.int32),
            pltpu.SemaphoreType.DMA((8,)),
            pltpu.SemaphoreType.DMA((2, XCH)),
            pltpu.SemaphoreType.DMA((3, 4)),
            pltpu.SemaphoreType.DMA((6,)),
            pltpu.SemaphoreType.DMA((7,)),
        ],
        compiler_params=pltpu.CompilerParams(vmem_limit_bytes=120 * 2**20, disable_bounds_checks=True),
        name="resblk",
    )(xt, t_emb, g1, be1, w1t, w_emb, g2, be2, w2t)
    return jnp.transpose(out.reshape(B, H, W, C), (0, 3, 1, 2))
```

```python
import itertools

import jax
import jax.numpy as jnp
import numpy as np
from jax import lax
import jax.experimental.pallas as pl
import jax.experimental.pallas.tpu as pltpu

F32 = jnp.float32
BF16 = jnp.bfloat16
U32 = jnp.uint32

PA = 2.0 / 3.0
PB = 1.5
A2, B2 = PA * PA, PB * PB
NA = 1.0 / (2 * A2 * (A2 - B2))
NB = 1.0 / (2 * B2 * (B2 - A2))
RT = PB / PA
GS = PA ** 3
ROWS = (0, 5, 1, 2, 3, 4)

TPOS = (0, 24, 32, 40, 48, 56, 64, 16)
TREC = 72
XCH = 4
MROW = 264
MSLOT = 36 * MROW
M_SLOT = (0, 1, 2, 3, 4, 0, 1, 2, 3, 4, 0, 1, 3, 4, 2, 0)
K_A2, K_B2, K_BITS, K_ZERO, K_SUM, K_SQ, K_GN = (i * MROW + 256 for i in range(7))

K_G = K_GN + 3 * MROW
C0COST, A1COST, A2COST = 38, 34, 46


def _bt(d0, d1, d2, d3, d4, d5, a2=A2, b2=B2):
    t, u = a2 * d2, b2 * d2
    ea, eb = d4 - u, d4 - t
    v0 = ea - t
    if d0 is not None:
        v0 = v0 + d0
    t3, u3 = a2 * d3, b2 * d3
    pa, pb = t3 - d1, u3 - d1
    v5 = (d5 - pa) - u3 if d5 is not None else (d1 - t3) - u3
    oa, ob = PB * pa, PA * pb
    return v0, ea + oa, ea - oa, eb + ob, eb - ob, v5


def _at(m0, m1, m2, m3, m4, m5):
    sa, ta, sb, tb = m1 + m2, m1 - m2, m3 + m4, m3 - m4
    return (m0 + sa) + sb, ta + RT * tb, sa + (RT * RT) * sb, (ta + m5) + (RT * RT * RT) * tb


def _gt(g0, g1, g2, k):
    ea, oa = (k * NA) * g0 + (k * NA * A2) * g2, (k * NA * PA) * g1
    eb, ob = (k * NB) * g0 + (k * NB * B2) * g2, (k * NB * PB) * g1
    k5 = k / PA ** 3
    u0 = g0 if abs(k - 1.0) < 1e-12 else k * g0
    u5 = g2 if abs(k5 - 1.0) < 1e-12 else k5 * g2
    return u0, ea + oa, ea - oa, eb + ob, eb - ob, u5


def _stack(top, bottom):
    return jnp.concatenate([top, bottom], axis=0).astype(BF16)


def _pair(lo, hi):
    bits = lax.bitcast_convert_type(_stack(lo, hi).astype(F32), U32)
    return (bits[:8] >> 16) | (bits[8:] & np.uint32(0xFFFF0000))


def _unpair(w, shift=16, mask=np.uint32(0xFFFF0000)):
    return lax.bitcast_convert_type(w << shift, F32), lax.bitcast_convert_type(w & mask, F32)


def _tree(xs):
    while len(xs) > 1:
        xs = [xs[i] + xs[i + 1] for i in range(0, len(xs), 2)]
    return xs[0]


def _acc(a, x):
    return x if a is None else a + x


class _Rows:
    def __init__(self, ref, base=0):
        self.ref, self.base = ref, base

    def ld(self, off, n=8, stride=1):
        return self.ref[pl.ds(self.base + off, n, stride=stride), :]

    def st(self, off, val, stride=1):
        self.ref[pl.ds(self.base + off, val.shape[0], stride=stride), :] = val


def _splitter(const):
    bits = lax.bitcast_convert_type(const.ld(K_BITS), U32)
    shift, mask = bits & 16, bits << 16
    return lambda w: _unpair(w, shift, mask)


def _job_u(w, u, const, rows):
    needed = sorted({i for row in rows for i in {0: (0,), 5: (2,)}.get(row, (0, 1, 2))})
    cost = 9 * len(needed) + sum(32 if row in (0, 5) else 100 for row in rows)

    def gen():
        for r in range(0, 64, 8):
            zero = lax.bitcast_convert_type(const.ld(K_ZERO), U32)
            g = {}
            for i in needed:
                taps = [pltpu.bitcast(w[3 * i + j].ld(r) | zero, BF16).astype(F32) for j in range(3)]
                g[i] = [v[:8] for v in taps], [v[8:] for v in taps]

            def emit(i, vals, k):
                top, bottom = _gt(*vals[0], k), _gt(*vals[1], k)
                for j in range(6):
                    u.st((i * 6 + j) * 128 + 2 * r, _stack(top[j], bottom[j]))

            for n, row in enumerate(rows):
                if row == 0:
                    emit(0, g[0], GS)
                elif row == 5:
                    emit(5, g[2], 1.0)
                else:
                    k0, k1, k2 = (const.ld(K_G + (3 * (row // 2) + i) * MROW) for i in range(3))
                    e = [[k0 * g[0][h][j] + k2 * g[2][h][j] for j in range(3)] for h in range(2)]
                    o = [[k1 * g[1][h][j] for j in range(3)] for h in range(2)]
                    emit(row, [[e[h][j] + o[h][j] for j in range(3)] for h in range(2)], GS)
                    emit(row + 1, [[e[h][j] - o[h][j] for j in range(3)] for h in range(2)], GS)
                yield (32 if row in (0, 5) else 100) + (9 * len(needed) if n == 0 else 0)

    return gen(), 8 * cost


def _gn_coeffs(s, q, e, gamma, beta, ab):
    s = jnp.sum(s, axis=0, keepdims=True) * (1.0 / 4096)
    q = jnp.sum(q, axis=0, keepdims=True) * (1.0 / 4096)
    var_c = jnp.maximum(q - s * s, 0.0)
    mean_c = s if e is None else s + e
    mu = jnp.sum(mean_c, axis=1, keepdims=True) * (1.0 / 128)
    second = jnp.sum(var_c + mean_c * mean_c, axis=1, keepdims=True) * (1.0 / 128)
    var = jnp.maximum(second - mu * mu, 0.0)
    a = 0.5 * gamma * lax.rsqrt(var + 1e-5)
    b = 0.5 * beta + a * (-mu if e is None else e - mu)
    ab.st(0, jnp.broadcast_to(a, (8, 128)))
    ab.st(8, jnp.broadcast_to(b, (8, 128)))


def _unpack_row(x, h, y, split):
    vals = [v for k in range(4) for v in split(x.ld(k, 8, 4))]
    for q, v in enumerate(vals):
        h.st(y * 64 + q * 8, v)
    return _tree(vals), _tree([v * v for v in vals])


def _job_c0(x, h, gamma, beta, ab, const):
    def gen():
        s = q = None
        for y in range(64):
            ds, dq = _unpack_row(_Rows(x[y // (64 // XCH)], (y % (64 // XCH)) * 32), h, y, _splitter(const))
            if y % 4 == 0 and y > 0:
                const.st(K_SUM, old[0])
                const.st(K_SQ, old[1])
            old = (s, q)
            s, q = _acc(s, ds), _acc(q, dq)
            yield C0COST
        _gn_coeffs(s, q, None, gamma[...], beta[...], ab)
        yield 40

    return gen(), 64 * C0COST + 40


def _job_a1(h, ab, t, const, k):
    def gen():
        scale = K_GN + k * MROW
        const.st(scale, ab.ld(0))
        b = ab.ld(8)

        def act(y, q, a):
            if y > 63:
                return None
            u = h.ld(y * 64 + q * 8) * a + b
            return u * jnp.tanh(u) + u

        for q in range(8):
            d4, d5 = None, act(0, q, const.ld(scale))
            for ty in range(16):
                a = const.ld(scale)
                d0, d1 = d4, d5
                d2, d3, d4, d5 = (act(4 * ty + k, q, a) for k in range(1, 5))
                for i, val in enumerate(_bt(d0, d1, d2, d3, d4, d5)):
                    t.st((ty * 6 + i) * TREC + TPOS[q], val)
                yield A1COST

    return gen(), 128 * A1COST


def _job_a2(t, v, const, rows):
    def gen():
        for i in rows:
            for ty in range(16):
                offs = (TPOS[7] - 1,) + TPOS + (TPOS[0] + 1,)
                d = [t.ld((ty * 6 + i) * TREC + o) for o in offs]
                a2, b2 = const.ld(K_A2), const.ld(K_B2)
                for j, (lo, hi) in enumerate(zip(_bt(*d[0:6], a2, b2), _bt(*d[4:10], a2, b2))):
                    v.st((i * 6 + j) * 256 + ty * 16, _stack(lo, hi))
                yield A2COST

    return gen(), 16 * len(rows) * A2COST


def _tiles_out(m, r0, finish, cost):
    def row(i):
        return _at(*[m.ld((i * 6 + j) * MROW + r0) for j in range(6)])

    def done(i, ys):
        finish(i, [y if i + j == 3 else (PA ** (i + j) / GS) * y for j, y in enumerate(ys)])

    r1 = row(1)
    yield 13
    r2 = row(2)
    sa, ta = [x + y for x, y in zip(r1, r2)], [x - y for x, y in zip(r1, r2)]
    yield 21
    r3 = row(3)
    yield 13
    r4 = row(4)
    sb, tb = [x + y for x, y in zip(r3, r4)], [x - y for x, y in zip(r3, r4)]
    done(1, [x + RT * y for x, y in zip(ta, tb)])
    yield 32 + cost
    done(2, [x + (RT * RT) * y for x, y in zip(sa, sb)])
    done(0, [(x + y) + w for x, y, w in zip(sa, sb, row(0))])
    yield 35 + 2 * cost
    done(3, [(x + (RT * RT * RT) * y) + w for x, y, w in zip(ta, tb, row(5))])
    yield 28 + cost


def _job_c1(m, h, e, gamma, beta, ab):
    def gen():
        sq = [None, None]
        for ty in range(16):
            for sub in range(2):
                def finish(i, ys):
                    sq[0] = _acc(sq[0], _tree(ys))
                    sq[1] = _acc(sq[1], _tree([y * y for y in ys]))
                    for j in range(4):
                        h.st((4 * ty + i) * 64 + (4 * sub + j) * 8, ys[j])

                before = tuple(sq)
                for n, cost in enumerate(_tiles_out(m, ty * 16 + sub * 8, finish, 12)):
                    if n == 1 and before[0] is not None:
                        m.st(K_SUM, before[0])
                        m.st(K_SQ, before[1])
                    yield cost
        _gn_coeffs(sq[0], sq[1], e[...], gamma[...], beta[...], ab)
        yield 40

    return gen(), 32 * (142 + 48) + 40


def _residual_out(m, x):
    for ty in range(16 // XCH):
        for sub in range(2):
            def finish(i, ys):
                for k in range(2):
                    off = (4 * ty + i) * 32 + 2 * sub + k
                    lo, hi = _unpair(x.ld(off, 8, 4))
                    x.st(off, _pair(lo + ys[2 * k], hi + ys[2 * k + 1]), 4)

            yield from _tiles_out(m, ty * 16 + sub * 8, finish, 18)


def _job_c2(m, x):
    return _residual_out(m, x), (32 // XCH) * (142 + 72)


def _run(*jobs):
    for gen, _ in jobs:
        for _ in gen:
            pass


def _step(v, u, m, jobs, add=False, tile_rows=ROWS, tiles=(0, 256), rows=16, tail=5):
    total = sum(c for _, c in jobs)
    pieces = itertools.chain(*[g for g, _ in jobs])
    first, count = tiles
    span = len(tile_rows) * 6 * count // rows - tail
    lead = 7 * total / span
    spent = 0

    def advance(limit):
        nonlocal spent
        while spent < limit:
            cost = next(pieces, None)
            if cost is None:
                return
            spent += cost

    tick = 0
    advance(lead)
    for xi in (6 * i + j for i in tile_rows for j in range(6)):
        lhs = jnp.concatenate([pltpu.bitcast(r.ld(xi * 128 + first // 2, count // 2), BF16) for r in v], axis=1)
        rhs = jnp.concatenate(
            [jnp.concatenate([pltpu.bitcast(r.ld(xi * 64, 64), BF16) for r in un], axis=1) for un in u], axis=0)
        res = lax.dot_general(lhs, rhs, (((1,), (1,)), ((), ())), preferred_element_type=F32)
        for r in range(0, count, rows):
            for n, mn in enumerate(m):
                val = res[r:r + rows, n * 128:(n + 1) * 128]
                at = xi * MROW + first + r
                mn.st(at, val + mn.ld(at, rows) if add else val)
            tick += 1
            advance(lead + (total - lead) * tick / span)
    advance(float("inf"))


def _kernel(x_hbm, t_hbm, g1_hbm, be1_hbm, w1_hbm, we_hbm, g2_hbm, be2_hbm, w2_hbm, o_hbm,
            t_ref, g1_ref, be1_ref, g2_ref, be2_ref,
            xbuf, wbuf, webuf, hbuf, abuf, t0, t1, t2, v0, v1, u1, u2, mbuf, par, emb, slots,
            xsem, csem, wsem, psem, osem):

    def x_words(j, c):
        return xbuf.at[j, c].bitcast(U32)

    def words(ref, k):
        return _Rows(ref.at[k].bitcast(U32))

    body = pl.ds(0, 4096 // XCH)

    def lanes(g):
        return pl.ds(g * 128 if isinstance(g, int) else pl.multiple_of(g * 128, 128), 128)

    def x_copy(j):
        return pltpu.make_async_copy(x_hbm.at[j // 4, :, :, lanes(j % 4)], xbuf.at[j, :, body], xsem.at[j])

    def x_chunk_copy(j, c):
        return pltpu.make_async_copy(x_hbm.at[0, c, :, lanes(j)], xbuf.at[j, c, body], csem.at[j, c])

    def o_copy(b, g):
        return pltpu.make_async_copy(xbuf.at[b * 4 + g, :, body], o_hbm.at[b, :, :, lanes(g)], osem.at[b * 4 + g])

    def o_chunk_copy(c):
        return pltpu.make_async_copy(xbuf.at[7, c, body], o_hbm.at[1, c, :, lanes(3)], csem.at[0, c])

    def w1_copy(out_half, c):
        rows = pl.ds(out_half * 256, 256)
        return pltpu.make_async_copy(w1_hbm.at[:, rows, lanes(c)], wbuf.at[c, :, rows], wsem.at[out_half, c])

    def w1_copies(out_half, in_half):
        return [w1_copy(out_half, 2 * in_half + c) for c in range(2)]

    def w2_copies(cs):
        return [pltpu.make_async_copy(w2_hbm.at[:, :, lanes(c)], wbuf.at[4 + c], wsem.at[2, c]) for c in cs]

    def p_copies(ks):
        pairs = ((g1_hbm, g1_ref), (be1_hbm, be1_ref), (g2_hbm, g2_ref), (be2_hbm, be2_ref), (t_hbm, t_ref),
                 (we_hbm, webuf))
        return [pltpu.make_async_copy(*pairs[k], psem.at[k]) for k in ks]

    def start(copies):
        for cp in copies:
            cp.start()

    def wait(copies):
        for cp in copies:
            cp.wait()

    def load_params(ks):
        wait(p_copies(ks))
        for k in ks:
            val = (g1_ref, be1_ref, g2_ref, be2_ref)[k][...].astype(F32).reshape(4, 128)
            for g in range(4):
                par[k * 4 + g] = val[g:g + 1]

    start(p_copies((0, 1)))

    @pl.loop(0, 2 * XCH)
    def _(i):
        x_chunk_copy(i // XCH, i % XCH).start()

    @pl.loop(0, 2)
    def _(c):
        w1_copy(0, c).start()

    for t in (t0, t1, t2):
        for r in range(96):
            _Rows(t).st(r * TREC + 8, jnp.zeros((8, 128), F32))
    for k, slot in enumerate(M_SLOT):
        slots[k] = slot * MSLOT
        slots[16 + k] = slot * MSLOT
    for j in range(8):
        slots[32 + j] = j * 4096
    fixed = _Rows(mbuf)
    fixed.st(K_A2, jnp.full((8, 128), A2, F32))
    fixed.st(K_B2, jnp.full((8, 128), B2, F32))
    fixed.st(K_BITS, lax.bitcast_convert_type(jnp.full((8, 128), 0x3F80FFFF, U32), F32))
    for i, value in enumerate((NA, NA * PA, NA * A2, NB, NB * PB, NB * B2)):
        fixed.st(K_G + i * MROW, jnp.full((8, 128), value, F32))
    fixed.st(K_ZERO, jnp.zeros((8, 128), F32))

    def m_in(k):
        return _Rows(mbuf, pl.multiple_of(slots[k], 8))

    def m_out(k, count=1):
        base = pl.multiple_of(slots[16 + k], 8)
        return [_Rows(mbuf, base + i * MSLOT) for i in range(count)]

    def h_slot(j, conv):
        return _Rows(hbuf, pl.multiple_of(slots[32 + j], 8) if conv else j * 4096)

    def ab_slot(j):
        return _Rows(abuf, j * 16)

    def taps(conv, n, c):
        return [_Rows(wbuf.at[conv * 4 + c, k, lanes(n)].bitcast(U32)) for k in range(9)]

    every = [(0, 1), (5, 3)]

    def u1_jobs(blocks, rows, const):
        return [_job_u(taps(0, n, c), _Rows(u1.at[n * 4 + c]), const, row) for n, c in blocks for row in rows]

    def u2_jobs(u, n, first, cs):
        return [_job_u(taps(1, n, c), _Rows(u.at[(n - first) * 4 + c]), const, row)
                for c in cs for row in every]

    def quad(out_half, in_half):
        return [(2 * out_half + n, 2 * in_half + c) for n in range(2) for c in range(2)]

    def c0(j):
        return _job_c0([x_words(j, c) for c in range(XCH)], h_slot(j, 0), par.at[j % 4], par.at[4 + j % 4], ab_slot(j), const)

    def a1(j, k, conv=1):
        return _job_a1(h_slot(j, conv), ab_slot(j), _Rows((t0, t1, t2)[k]), const, k)

    def a2(v, g, k, rows=ROWS):
        return _job_a2(_Rows((t0, t1, t2)[k]), _Rows(v.at[g]), const, rows)

    def c1(j):
        return _job_c1(m_in(j), h_slot(j, 1), emb.at[j], par.at[8 + j % 4], par.at[12 + j % 4], ab_slot(j))

    def c2(j, c):
        m = m_in(8 + j)
        return _job_c2(_Rows(mbuf, m.base + c * (256 // XCH)), _Rows(x_words(j, c)))

    def block(fn):
        pl.when(slots[0] == 0)(fn)

    def half_step(out_half, in_half, jobs, rows=ROWS):
        ins = (2 * in_half, 2 * in_half + 1)
        outs = (2 * out_half, 2 * out_half + 1)
        block(lambda: _step([words(v0, c) for c in ins], [[words(u1, n * 4 + c) for c in ins] for n in outs],
                            m_out(outs[0], 2), jobs, add=bool(in_half), tile_rows=rows, rows=8, tail=8))

    def step(slot, v, u, n, jobs, **kwargs):
        block(lambda: _step([words(v, c) for c in range(4)], [[words(u, n * 4 + c) for c in range(4)]],
                            m_out(slot), jobs, **kwargs))

    @pl.loop(0, 2)
    def _(j):
        def unpack_chunk(c, sums):
            x_chunk_copy(j, c).wait()
            h = _Rows(hbuf, j * 4096 + c * (4096 // XCH))
            s, q = sums
            for y in range(64 // XCH):
                ds, dq = _unpack_row(_Rows(x_words(j, c), y * 32), h, y, _unpair)
                s, q = s + ds, q + dq
            return s, q

        s, q = lax.fori_loop(0, XCH, unpack_chunk, (jnp.zeros((8, 128), F32),) * 2)

        @pl.when(j == 0)
        def _():
            load_params((0, 1))
            x_copy(2).start()
            _gn_coeffs(s, q, None, par[0], par[4], ab_slot(0))

        @pl.when(j == 1)
        def _():
            _gn_coeffs(s, q, None, par[1], par[5], ab_slot(1))
            _run(_job_a2(_Rows(t0), _Rows(v0.at[0]), fixed, ROWS[4:]))

        _run(_job_a1(h_slot(j, 0), ab_slot(j), _Rows(t0), fixed, 0),
             _job_a2(_Rows(t0), _Rows(v0.at[j]), fixed, ROWS[:4]))

        @pl.when(j == 0)
        def _():
            start(w1_copies(1, 0))

    @pl.loop(0, 2)
    def _(c):
        w1_copy(0, c).wait()
        _run(*u1_jobs([(0, c), (1, c)], [(0, 5)], fixed))

    const = m_in(0)
    start([x_copy(3)] + w1_copies(0, 1))
    half_step(0, 0, u1_jobs(quad(0, 0), [(1,)], const) + [a2(v0, 1, 0, ROWS[4:])]
              + u1_jobs(quad(0, 0)[:2], [(3,)], const), ROWS[:2])
    wait([x_copy(2)])
    start(w1_copies(1, 1) + [x_copy(j) for j in range(4, 8)])
    half_step(0, 0, [c0(2)] + u1_jobs(quad(0, 0)[2:], [(3,)], const), ROWS[2:3])
    wait(w1_copies(1, 0))
    half_step(0, 0, [a1(2, 1, 0)] + u1_jobs(quad(1, 0), every, const), ROWS[3:])
    wait([x_copy(3)] + w1_copies(0, 1))
    half_step(1, 0, [c0(3), a2(v0, 2, 1), a1(3, 0, 0), a2(v0, 3, 0)] + u1_jobs(quad(0, 1), every, const))
    wait(w1_copies(1, 1) + [x_copy(j) for j in range(4, 8)])
    start(p_copies((5, 2, 3, 4)) + w2_copies((0, 1)))
    half_step(0, 1, [job for i, b in enumerate(quad(1, 1)) for job in [c0(4 + i)] + u1_jobs([b], every, const)]
              + [a1(4, 1, 0)])
    half_step(1, 1, [a2(v1, 0, 1), a1(5, 0, 0), a1(6, 1, 0), a1(7, 2, 0)] + [a2(v1, 1 + k, k, ROWS[:3]) for k in range(3)])

    load_params((2, 3))
    wait(p_copies((4, 5)) + w2_copies((0, 1)))
    start(w2_copies((2, 3)))

    def embed():
        th = t_ref[...].astype(F32) * 0.5
        e = jnp.dot((th * jnp.tanh(th) + th).astype(BF16), webuf[...], preferred_element_type=F32)
        for j in range(8):
            emb[j] = e[j // 4:j // 4 + 1, (j % 4) * 128:(j % 4 + 1) * 128]
        yield 0

    step(4, v1, u1, 0, [(embed(), 0)] + [a2(v1, 1 + k, k, (i,)) for i in ROWS[3:] for k in range(3)] + [c1(0), c1(1)]
         + u2_jobs(u2, 0, 0, (0, 1)))
    wait(w2_copies((2, 3)))
    step(5, v1, u1, 1, [a1(0, 0), a2(v0, 0, 0), c1(2), c1(3)] + u2_jobs(u2, 0, 0, (2, 3)))
    step(6, v1, u1, 2, [a1(1, 1), a2(v0, 1, 1), a1(2, 2), a2(v0, 2, 2), c1(4), (iter([500]), 500)])
    step(7, v1, u1, 3, [a1(3, 0), a2(v0, 3, 0), c1(5)] + u2_jobs(u2, 1, 0, range(4)))

    @pl.loop(0, 2)
    def _(n):
        step(8 + n, v0, u2, n, [a1(4 + n, 1), a2(v1, n, 1), c1(6 + n)] + u2_jobs(u1, 2 + n, 0, range(4)))

    @pl.loop(2, 4)
    def _(n):
        step(8 + n, v0, u1, n, [a1(4 + n, 0), a2(v1, n, 0)] + [c2(n - 2, c) for c in range(XCH)])
        o_copy(0, n - 2).start()

    step(14, v1, u1, 2, [c2(j, c) for j in (2, 3) for c in range(XCH)])
    start([o_copy(0, 2), o_copy(0, 3)])

    @pl.loop(0, 2)
    def _(n):
        done = 2 - 2 * n
        step(12 + n, v1, u2, n, [c2(4 + done, c) for c in range(XCH)])
        o_copy(1, done).start()

    step(15, v1, u1, 3, [c2(5, c) for c in range(XCH)], tiles=(0, 128))
    o_copy(1, 1).start()
    step(15, v1, u1, 3, [c2(7, 0), c2(7, 1)], tiles=(128, 64))
    start([o_chunk_copy(0), o_chunk_copy(1)])
    step(15, v1, u1, 3, [c2(7, 2)], tiles=(192, 64))
    o_chunk_copy(2).start()
    _run(c2(7, 3))
    o_chunk_copy(3).start()

    wait([o_copy(j // 4, j % 4) for j in range(7)] + [o_chunk_copy(c) for c in range(XCH)])


@jax.jit
def pallas_standalone__adm_resblock__diffusion_kernel(
    x: jax.Array,
    t_emb: jax.Array,
    g1: jax.Array,
    be1: jax.Array,
    w1: jax.Array,
    w_emb: jax.Array,
    g2: jax.Array,
    be2: jax.Array,
    w2: jax.Array,
):
    B, C, H, W = x.shape
    assert (B, C, H, W) == (2, 512, 64, 64)
    xt = jnp.transpose(x, (0, 2, 3, 1)).reshape(B, XCH, H * W // XCH, C)
    w1t = jnp.transpose(w1, (2, 3, 0, 1)).reshape(9, C, C)
    w2t = jnp.transpose(w2, (2, 3, 0, 1)).reshape(9, C, C)
    hbm = pl.BlockSpec(memory_space=pl.ANY)
    out = pl.pallas_call(
        _kernel,
        out_shape=jax.ShapeDtypeStruct(xt.shape, x.dtype),
        in_specs=[hbm] * 9,
        out_specs=hbm,
        scratch_shapes=[
            pltpu.VMEM(t_emb.shape, BF16),
            pltpu.VMEM(g1.shape, BF16),
            pltpu.VMEM(be1.shape, BF16),
            pltpu.VMEM(g2.shape, BF16),
            pltpu.VMEM(be2.shape, BF16),
            pltpu.VMEM((8, XCH, 4096 // XCH + 16, 128), BF16),
            pltpu.VMEM((8, 9, 512, 128), BF16),
            pltpu.VMEM(w_emb.shape, BF16),
            pltpu.VMEM((8 * 4096, 128), F32),
            pltpu.VMEM((8 * 16, 128), F32),
            pltpu.VMEM((96 * TREC, 128), F32),
            pltpu.VMEM((96 * TREC, 128), F32),
            pltpu.VMEM((96 * TREC, 128), F32),
            pltpu.VMEM((4, 36 * 256, 128), BF16),
            pltpu.VMEM((4, 36 * 256, 128), BF16),
            pltpu.VMEM((16, 36 * 128, 128), BF16),
            pltpu.VMEM((8, 36 * 128, 128), BF16),
            pltpu.VMEM((5 * MSLOT, 128), F32),
            pltpu.VMEM((16, 1, 128), F32),
            pltpu.VMEM((8, 1, 128), F32),
            pltpu.SMEM((40,), jnp.int32),
            pltpu.SemaphoreType.DMA((8,)),
            pltpu.SemaphoreType.DMA((2, XCH)),
            pltpu.SemaphoreType.DMA((3, 4)),
            pltpu.SemaphoreType.DMA((6,)),
            pltpu.SemaphoreType.DMA((7,)),
        ],
        compiler_params=pltpu.CompilerParams(vmem_limit_bytes=120 * 2**20),
        name="resblk",
    )(xt, t_emb, g1, be1, w1t, w_emb, g2, be2, w2t)
    return jnp.transpose(out.reshape(B, H, W, C), (0, 3, 1, 2))
```

```python
import itertools

import jax
import jax.numpy as jnp
import numpy as np
from jax import lax
import jax.experimental.pallas as pl
import jax.experimental.pallas.tpu as pltpu

F32 = jnp.float32
BF16 = jnp.bfloat16
U32 = jnp.uint32

PA = 2.0 / 3.0
PB = 1.5
A2, B2 = PA * PA, PB * PB
NA = 1.0 / (2 * A2 * (A2 - B2))
NB = 1.0 / (2 * B2 * (B2 - A2))
RT = PB / PA
GS = PA ** 3
ROWS = (0, 5, 1, 2, 3, 4)

TPOS = (0, 24, 32, 40, 48, 56, 64, 16)
TREC = 72
XCH = 4
MROW = 264
MSLOT = 36 * MROW
M_SLOT = (0, 1, 2, 3, 4, 0, 1, 2, 3, 4, 0, 1, 3, 4, 2, 0)
K_A2, K_B2, K_BITS, K_ZERO, K_SUM, K_SQ, K_GN = (i * MROW + 256 for i in range(7))
K_G = K_GN + 3 * MROW
C0COST, A1COST, A2COST = 38, 34, 46


def _bt(d0, d1, d2, d3, d4, d5, a2=A2, b2=B2):
    t, u = a2 * d2, b2 * d2
    ea, eb = d4 - u, d4 - t
    v0 = ea - t
    if d0 is not None:
        v0 = v0 + d0
    t3, u3 = a2 * d3, b2 * d3
    pa, pb = t3 - d1, u3 - d1
    v5 = (d5 - pa) - u3 if d5 is not None else (d1 - t3) - u3
    oa, ob = PB * pa, PA * pb
    return v0, ea + oa, ea - oa, eb + ob, eb - ob, v5


def _at(m0, m1, m2, m3, m4, m5):
    sa, ta, sb, tb = m1 + m2, m1 - m2, m3 + m4, m3 - m4
    return (m0 + sa) + sb, ta + RT * tb, sa + (RT * RT) * sb, (ta + m5) + (RT * RT * RT) * tb


def _gt(g0, g1, g2, k):
    ea, oa = (k * NA) * g0 + (k * NA * A2) * g2, (k * NA * PA) * g1
    eb, ob = (k * NB) * g0 + (k * NB * B2) * g2, (k * NB * PB) * g1
    k5 = k / PA ** 3
    u0 = g0 if abs(k - 1.0) < 1e-12 else k * g0
    u5 = g2 if abs(k5 - 1.0) < 1e-12 else k5 * g2
    return u0, ea + oa, ea - oa, eb + ob, eb - ob, u5


def _stack(top, bottom):
    return jnp.concatenate([top, bottom], axis=0).astype(BF16)


def _pair(lo, hi):
    bits = lax.bitcast_convert_type(_stack(lo, hi).astype(F32), U32)
    return (bits[:8] >> 16) | (bits[8:] & np.uint32(0xFFFF0000))


def _unpair(w, shift=16, mask=np.uint32(0xFFFF0000)):
    return lax.bitcast_convert_type(w << shift, F32), lax.bitcast_convert_type(w & mask, F32)


def _tree(xs):
    while len(xs) > 1:
        xs = [xs[i] + xs[i + 1] for i in range(0, len(xs), 2)]
    return xs[0]


def _acc(a, x):
    return x if a is None else a + x


class _Rows:
    def __init__(self, ref, base=0):
        self.ref, self.base = ref, base

    def ld(self, off, n=8, stride=1):
        return self.ref[pl.ds(self.base + off, n, stride=stride), :]

    def st(self, off, val, stride=1):
        self.ref[pl.ds(self.base + off, val.shape[0], stride=stride), :] = val


def _splitter(const):
    bits = lax.bitcast_convert_type(const.ld(K_BITS), U32)
    shift, mask = bits & 16, bits << 16
    return lambda w: _unpair(w, shift, mask)


def _job_u(w, u, const, rows):
    needed = sorted({i for row in rows for i in {0: (0,), 5: (2,)}.get(row, (0, 1, 2))})
    cost = 9 * len(needed) + sum(32 if row in (0, 5) else 100 for row in rows)

    def gen():
        for r in range(0, 64, 8):
            zero = lax.bitcast_convert_type(const.ld(K_ZERO), U32)
            g = {}
            for i in needed:
                taps = [pltpu.bitcast(w[3 * i + j].ld(r) | zero, BF16).astype(F32) for j in range(3)]
                g[i] = [v[:8] for v in taps], [v[8:] for v in taps]

            def emit(i, vals, k):
                top, bottom = _gt(*vals[0], k), _gt(*vals[1], k)
                for j in range(6):
                    u.st((i * 6 + j) * 128 + 2 * r, _stack(top[j], bottom[j]))

            for n, row in enumerate(rows):
                if row == 0:
                    emit(0, g[0], GS)
                elif row == 5:
                    emit(5, g[2], 1.0)
                else:
                    k0, k1, k2 = (const.ld(K_G + (3 * (row // 2) + i) * MROW) for i in range(3))
                    e = [[k0 * g[0][h][j] + k2 * g[2][h][j] for j in range(3)] for h in range(2)]
                    o = [[k1 * g[1][h][j] for j in range(3)] for h in range(2)]
                    emit(row, [[e[h][j] + o[h][j] for j in range(3)] for h in range(2)], GS)
                    emit(row + 1, [[e[h][j] - o[h][j] for j in range(3)] for h in range(2)], GS)
                yield (32 if row in (0, 5) else 100) + (9 * len(needed) if n == 0 else 0)

    return gen(), 8 * cost


def _gn_coeffs(s, q, e, gamma, beta, ab):
    s = jnp.sum(s, axis=0, keepdims=True) * (1.0 / 4096)
    q = jnp.sum(q, axis=0, keepdims=True) * (1.0 / 4096)
    var_c = jnp.maximum(q - s * s, 0.0)
    mean_c = s if e is None else s + e
    mu = jnp.sum(mean_c, axis=1, keepdims=True) * (1.0 / 128)
    dev = mean_c - mu
    var = jnp.sum(var_c + dev * dev, axis=1, keepdims=True) * (1.0 / 128)
    a = 0.5 * gamma * lax.rsqrt(var + 1e-5)
    b = 0.5 * beta + a * (-mu if e is None else e - mu)
    ab.st(0, jnp.broadcast_to(a, (8, 128)))
    ab.st(8, jnp.broadcast_to(b, (8, 128)))


def _unpack_row(x, h, y, split):
    vals = [v for k in range(4) for v in split(x.ld(k, 8, 4))]
    for q, v in enumerate(vals):
        h.st(y * 64 + q * 8, v)
    return _tree(vals), _tree([v * v for v in vals])


def _job_c0(x, h, gamma, beta, ab, const):
    def gen():
        s = q = None
        for y in range(64):
            ds, dq = _unpack_row(_Rows(x[y // (64 // XCH)], (y % (64 // XCH)) * 32), h, y, _splitter(const))
            if y % 4 == 0 and y > 0:
                const.st(K_SUM, old[0])
                const.st(K_SQ, old[1])
            old = (s, q)
            s, q = _acc(s, ds), _acc(q, dq)
            yield C0COST
        _gn_coeffs(s, q, None, gamma[...], beta[...], ab)
        yield 40

    return gen(), 64 * C0COST + 40


def _job_a1(h, ab, t, const, k):
    def gen():
        scale = K_GN + k * MROW
        const.st(scale, ab.ld(0))
        b = ab.ld(8)

        def act(y, q, a):
            if y > 63:
                return None
            u = h.ld(y * 64 + q * 8) * a + b
            return u * jnp.tanh(u) + u

        for q in range(8):
            d4, d5 = None, act(0, q, const.ld(scale))
            for ty in range(16):
                a = const.ld(scale)
                d0, d1 = d4, d5
                d2, d3, d4, d5 = (act(4 * ty + k, q, a) for k in range(1, 5))
                for i, val in enumerate(_bt(d0, d1, d2, d3, d4, d5)):
                    t.st((ty * 6 + i) * TREC + TPOS[q], val)
                yield A1COST

    return gen(), 128 * A1COST


def _job_a2(t, v, const, rows):
    def gen():
        for i in rows:
            for ty in range(16):
                offs = (TPOS[7] - 1,) + TPOS + (TPOS[0] + 1,)
                d = [t.ld((ty * 6 + i) * TREC + o) for o in offs]
                a2, b2 = const.ld(K_A2), const.ld(K_B2)
                for j, (lo, hi) in enumerate(zip(_bt(*d[0:6], a2, b2), _bt(*d[4:10], a2, b2))):
                    v.st((i * 6 + j) * 256 + ty * 16, _stack(lo, hi))
                yield A2COST

    return gen(), 16 * len(rows) * A2COST


def _tiles_out(m, r0, finish, cost):
    def row(i):
        return _at(*[m.ld((i * 6 + j) * MROW + r0) for j in range(6)])

    def done(i, ys):
        finish(i, [y if i + j == 3 else (PA ** (i + j) / GS) * y for j, y in enumerate(ys)])

    r1 = row(1)
    yield 13
    r2 = row(2)
    sa, ta = [x + y for x, y in zip(r1, r2)], [x - y for x, y in zip(r1, r2)]
    yield 21
    r3 = row(3)
    yield 13
    r4 = row(4)
    sb, tb = [x + y for x, y in zip(r3, r4)], [x - y for x, y in zip(r3, r4)]
    done(1, [x + RT * y for x, y in zip(ta, tb)])
    yield 32 + cost
    done(2, [x + (RT * RT) * y for x, y in zip(sa, sb)])
    done(0, [(x + y) + w for x, y, w in zip(sa, sb, row(0))])
    yield 35 + 2 * cost
    done(3, [(x + (RT * RT * RT) * y) + w for x, y, w in zip(ta, tb, row(5))])
    yield 28 + cost


def _job_c1(m, h, e, gamma, beta, ab):
    def gen():
        sq = [None, None]
        for ty in range(16):
            for sub in range(2):
                def finish(i, ys):
                    sq[0] = _acc(sq[0], _tree(ys))
                    sq[1] = _acc(sq[1], _tree([y * y for y in ys]))
                    for j in range(4):
                        h.st((4 * ty + i) * 64 + (4 * sub + j) * 8, ys[j])

                before = tuple(sq)
                for n, cost in enumerate(_tiles_out(m, ty * 16 + sub * 8, finish, 12)):
                    if n == 1 and before[0] is not None:
                        m.st(K_SUM, before[0])
                        m.st(K_SQ, before[1])
                    yield cost
        _gn_coeffs(sq[0], sq[1], e[...], gamma[...], beta[...], ab)
        yield 40

    return gen(), 32 * (142 + 48) + 40


def _residual_out(m, x):
    for ty in range(16 // XCH):
        for sub in range(2):
            def finish(i, ys):
                for k in range(2):
                    off = (4 * ty + i) * 32 + 2 * sub + k
                    lo, hi = _unpair(x.ld(off, 8, 4))
                    x.st(off, _pair(lo + ys[2 * k], hi + ys[2 * k + 1]), 4)

            yield from _tiles_out(m, ty * 16 + sub * 8, finish, 18)


def _job_c2(m, x):
    return _residual_out(m, x), (32 // XCH) * (142 + 72)


def _run(*jobs):
    for gen, _ in jobs:
        for _ in gen:
            pass


def _step(v, u, m, jobs, add=False, tile_rows=ROWS, tiles=(0, 256), rows=16, tail=5):
    total = sum(c for _, c in jobs)
    pieces = itertools.chain(*[g for g, _ in jobs])
    first, count = tiles
    span = len(tile_rows) * 6 * count // rows - tail
    lead = 7 * total / span
    spent = 0

    def advance(limit):
        nonlocal spent
        while spent < limit:
            cost = next(pieces, None)
            if cost is None:
                return
            spent += cost

    tick = 0
    advance(lead)
    for xi in (6 * i + j for i in tile_rows for j in range(6)):
        lhs = jnp.concatenate([pltpu.bitcast(r.ld(xi * 128 + first // 2, count // 2), BF16) for r in v], axis=1)
        rhs = jnp.concatenate(
            [jnp.concatenate([pltpu.bitcast(r.ld(xi * 64, 64), BF16) for r in un], axis=1) for un in u], axis=0)
        res = lax.dot_general(lhs, rhs, (((1,), (1,)), ((), ())), preferred_element_type=F32)
        for r in range(0, count, rows):
            for n, mn in enumerate(m):
                val = res[r:r + rows, n * 128:(n + 1) * 128]
                at = xi * MROW + first + r
                mn.st(at, val + mn.ld(at, rows) if add else val)
            tick += 1
            advance(lead + (total - lead) * tick / span)
    advance(float("inf"))


def _kernel(x_hbm, t_hbm, g1_hbm, be1_hbm, w1_hbm, we_hbm, g2_hbm, be2_hbm, w2_hbm, o_hbm,
            t_ref, g1_ref, be1_ref, g2_ref, be2_ref,
            xbuf, wbuf, webuf, hbuf, abuf, t0, t1, t2, v0, v1, u1, u2, mbuf, par, emb, slots,
            xsem, csem, wsem, psem, osem):

    def x_words(j, c):
        return xbuf.at[j, c].bitcast(U32)

    def words(ref, k):
        return _Rows(ref.at[k].bitcast(U32))

    body = pl.ds(0, 4096 // XCH)

    def lanes(g):
        return pl.ds(g * 128 if isinstance(g, int) else pl.multiple_of(g * 128, 128), 128)

    def x_copy(j):
        return pltpu.make_async_copy(x_hbm.at[j // 4, :, :, lanes(j % 4)], xbuf.at[j, :, body], xsem.at[j])

    def x_chunk_copy(j, c):
        return pltpu.make_async_copy(x_hbm.at[0, c, :, lanes(j)], xbuf.at[j, c, body], csem.at[j, c])

    def o_copy(b, g):
        return pltpu.make_async_copy(xbuf.at[b * 4 + g, :, body], o_hbm.at[b, :, :, lanes(g)], osem.at[b * 4 + g])

    def o_chunk_copy(c):
        return pltpu.make_async_copy(xbuf.at[7, c, body], o_hbm.at[1, c, :, lanes(3)], csem.at[0, c])

    def w1_copy(out_half, c):
        rows = pl.ds(out_half * 256, 256)
        return pltpu.make_async_copy(w1_hbm.at[:, rows, lanes(c)], wbuf.at[c, :, rows], wsem.at[out_half, c])

    def w1_copies(out_half, in_half):
        return [w1_copy(out_half, 2 * in_half + c) for c in range(2)]

    def w2_copies(cs):
        return [pltpu.make_async_copy(w2_hbm.at[:, :, lanes(c)], wbuf.at[4 + c], wsem.at[2, c]) for c in cs]

    def p_copies(ks):
        pairs = ((g1_hbm, g1_ref), (be1_hbm, be1_ref), (g2_hbm, g2_ref), (be2_hbm, be2_ref), (t_hbm, t_ref),
                 (we_hbm, webuf))
        return [pltpu.make_async_copy(*pairs[k], psem.at[k]) for k in ks]

    def start(copies):
        for cp in copies:
            cp.start()

    def wait(copies):
        for cp in copies:
            cp.wait()

    def load_params(ks):
        wait(p_copies(ks))
        for k in ks:
            val = (g1_ref, be1_ref, g2_ref, be2_ref)[k][...].astype(F32).reshape(4, 128)
            for g in range(4):
                par[k * 4 + g] = val[g:g + 1]

    start(p_copies((0, 1)))

    @pl.loop(0, 2 * XCH)
    def _(i):
        x_chunk_copy(i // XCH, i % XCH).start()

    @pl.loop(0, 2)
    def _(c):
        w1_copy(0, c).start()

    for t in (t0, t1, t2):
        for r in range(96):
            _Rows(t).st(r * TREC + 8, jnp.zeros((8, 128), F32))
    for k, slot in enumerate(M_SLOT):
        slots[k] = slot * MSLOT
        slots[16 + k] = slot * MSLOT
    for j in range(8):
        slots[32 + j] = j * 4096
    fixed = _Rows(mbuf)
    fixed.st(K_A2, jnp.full((8, 128), A2, F32))
    fixed.st(K_B2, jnp.full((8, 128), B2, F32))
    fixed.st(K_BITS, lax.bitcast_convert_type(jnp.full((8, 128), 0x3F80FFFF, U32), F32))
    for i, value in enumerate((NA, NA * PA, NA * A2, NB, NB * PB, NB * B2)):
        fixed.st(K_G + i * MROW, jnp.full((8, 128), value, F32))
    fixed.st(K_ZERO, jnp.zeros((8, 128), F32))

    def m_in(k):
        return _Rows(mbuf, pl.multiple_of(slots[k], 8))

    def m_out(k, count=1):
        base = pl.multiple_of(slots[16 + k], 8)
        return [_Rows(mbuf, base + i * MSLOT) for i in range(count)]

    def h_slot(j, conv):
        return _Rows(hbuf, pl.multiple_of(slots[32 + j], 8) if conv else j * 4096)

    def ab_slot(j):
        return _Rows(abuf, j * 16)

    def taps(conv, n, c):
        return [_Rows(wbuf.at[conv * 4 + c, k, lanes(n)].bitcast(U32)) for k in range(9)]

    every = [(0, 1), (5, 3)]

    def u1_jobs(blocks, rows, const):
        return [_job_u(taps(0, n, c), _Rows(u1.at[n * 4 + c]), const, row) for n, c in blocks for row in rows]

    def u2_jobs(u, n, cs):
        return [_job_u(taps(1, n, c), _Rows(u.at[n * 4 + c]), const, row) for c in cs for row in every]

    def quad(out_half, in_half):
        return [(2 * out_half + n, 2 * in_half + c) for n in range(2) for c in range(2)]

    def c0(j):
        x = [x_words(j, c) for c in range(XCH)]
        return _job_c0(x, h_slot(j, 0), par.at[j % 4], par.at[4 + j % 4], ab_slot(j), const)

    def a1(j, k, conv=1):
        return _job_a1(h_slot(j, conv), ab_slot(j), _Rows((t0, t1, t2)[k]), const, k)

    def a2(v, g, k, rows=ROWS):
        return _job_a2(_Rows((t0, t1, t2)[k]), _Rows(v.at[g]), const, rows)

    def c1(j):
        return _job_c1(m_in(j), h_slot(j, 1), emb.at[j], par.at[8 + j % 4], par.at[12 + j % 4], ab_slot(j))

    def c2(j, c):
        m = m_in(8 + j)
        return _job_c2(_Rows(mbuf, m.base + c * (256 // XCH)), _Rows(x_words(j, c)))

    def block(fn):
        pl.when(slots[0] == 0)(fn)

    def half_step(out_half, in_half, jobs, rows=ROWS):
        ins = (2 * in_half, 2 * in_half + 1)
        outs = (2 * out_half, 2 * out_half + 1)
        block(lambda: _step([words(v0, c) for c in ins], [[words(u1, n * 4 + c) for c in ins] for n in outs],
                            m_out(outs[0], 2), jobs, add=bool(in_half), tile_rows=rows, rows=8, tail=8))

    def step(slot, v, u, n, jobs, **kwargs):
        block(lambda: _step([words(v, c) for c in range(4)], [[words(u, n * 4 + c) for c in range(4)]],
                            m_out(slot), jobs, **kwargs))

    @pl.loop(0, 2)
    def _(j):
        def unpack_chunk(c, sums):
            x_chunk_copy(j, c).wait()
            h = _Rows(hbuf, j * 4096 + c * (4096 // XCH))
            s, q = sums
            for y in range(64 // XCH):
                ds, dq = _unpack_row(_Rows(x_words(j, c), y * 32), h, y, _unpair)
                s, q = s + ds, q + dq
            return s, q

        s, q = lax.fori_loop(0, XCH, unpack_chunk, (jnp.zeros((8, 128), F32),) * 2)

        @pl.when(j == 0)
        def _():
            load_params((0, 1))
            x_copy(2).start()
            _gn_coeffs(s, q, None, par[0], par[4], ab_slot(0))

        @pl.when(j == 1)
        def _():
            _gn_coeffs(s, q, None, par[1], par[5], ab_slot(1))
            _run(_job_a2(_Rows(t0), _Rows(v0.at[0]), fixed, ROWS[4:]))

        _run(_job_a1(h_slot(j, 0), ab_slot(j), _Rows(t0), fixed, 0),
             _job_a2(_Rows(t0), _Rows(v0.at[j]), fixed, ROWS[:4]))

        @pl.when(j == 0)
        def _():
            start(w1_copies(1, 0))

    @pl.loop(0, 2)
    def _(c):
        w1_copy(0, c).wait()
        _run(*u1_jobs([(0, c), (1, c)], [(0, 5)], fixed))

    const = m_in(0)
    start([x_copy(3)] + w1_copies(0, 1))
    half_step(0, 0, u1_jobs(quad(0, 0), [(1,)], const) + [a2(v0, 1, 0, ROWS[4:])]
              + u1_jobs(quad(0, 0)[:2], [(3,)], const), ROWS[:2])
    wait([x_copy(2)])
    start(w1_copies(1, 1) + [x_copy(j) for j in range(4, 8)])
    half_step(0, 0, [c0(2)] + u1_jobs(quad(0, 0)[2:], [(3,)], const), ROWS[2:3])
    wait(w1_copies(1, 0))
    half_step(0, 0, [a1(2, 1, 0)] + u1_jobs(quad(1, 0), every, const), ROWS[3:])
    wait([x_copy(3)] + w1_copies(0, 1))
    half_step(1, 0, [c0(3), a2(v0, 2, 1), a1(3, 0, 0), a2(v0, 3, 0)] + u1_jobs(quad(0, 1), every, const))
    wait(w1_copies(1, 1) + [x_copy(j) for j in range(4, 8)])
    start(p_copies((5, 2, 3, 4)) + w2_copies((0, 1)))
    half_step(0, 1, [job for i, b in enumerate(quad(1, 1)) for job in [c0(4 + i)] + u1_jobs([b], every, const)]
              + [a1(4, 1, 0)])
    half_step(1, 1, [a2(v1, 0, 1), a1(5, 0, 0), a1(6, 1, 0), a1(7, 2, 0)]
              + [a2(v1, 1 + k, k, ROWS[:3]) for k in range(3)])

    load_params((2, 3))
    wait(p_copies((4, 5)) + w2_copies((0, 1)))
    start(w2_copies((2, 3)))

    def embed():
        th = t_ref[...].astype(F32) * 0.5
        e = jnp.dot((th * jnp.tanh(th) + th).astype(BF16), webuf[...], preferred_element_type=F32)
        for j in range(8):
            emb[j] = e[j // 4:j // 4 + 1, (j % 4) * 128:(j % 4 + 1) * 128]
        yield 0

    step(4, v1, u1, 0, [(embed(), 0)] + [a2(v1, 1 + k, k, (i,)) for i in ROWS[3:] for k in range(3)] + [c1(0), c1(1)]
         + u2_jobs(u2, 0, (0, 1)))
    wait(w2_copies((2, 3)))
    step(5, v1, u1, 1, [a1(0, 0), a2(v0, 0, 0), c1(2), c1(3)] + u2_jobs(u2, 0, (2, 3)))
    step(6, v1, u1, 2, [a1(1, 1), a2(v0, 1, 1), a1(2, 2), a2(v0, 2, 2), c1(4), (iter([500]), 500)])
    step(7, v1, u1, 3, [a1(3, 0), a2(v0, 3, 0), c1(5)] + u2_jobs(u2, 1, range(4)))

    @pl.loop(0, 2)
    def _(n):
        step(8 + n, v0, u2, n, [a1(4 + n, 1), a2(v1, n, 1), c1(6 + n)] + u2_jobs(u1, 2 + n, range(4)))

    @pl.loop(2, 4)
    def _(n):
        step(8 + n, v0, u1, n, [a1(4 + n, 0), a2(v1, n, 0)] + [c2(n - 2, c) for c in range(XCH)])
        o_copy(0, n - 2).start()

    step(14, v1, u1, 2, [c2(j, c) for j in (2, 3) for c in range(XCH)])
    start([o_copy(0, 2), o_copy(0, 3)])

    @pl.loop(0, 2)
    def _(n):
        done = 2 - 2 * n
        step(12 + n, v1, u2, n, [c2(4 + done, c) for c in range(XCH)])
        o_copy(1, done).start()

    step(15, v1, u1, 3, [c2(5, c) for c in range(XCH)], tiles=(0, 128))
    o_copy(1, 1).start()
    step(15, v1, u1, 3, [c2(7, 0), c2(7, 1)], tiles=(128, 64))
    start([o_chunk_copy(0), o_chunk_copy(1)])
    step(15, v1, u1, 3, [c2(7, 2)], tiles=(192, 64))
    o_chunk_copy(2).start()
    _run(c2(7, 3))
    o_chunk_copy(3).start()

    wait([o_copy(j // 4, j % 4) for j in range(7)] + [o_chunk_copy(c) for c in range(XCH)])


@jax.jit
def pallas_standalone__adm_resblock__diffusion_kernel(
    x: jax.Array,
    t_emb: jax.Array,
    g1: jax.Array,
    be1: jax.Array,
    w1: jax.Array,
    w_emb: jax.Array,
    g2: jax.Array,
    be2: jax.Array,
    w2: jax.Array,
):
    B, C, H, W = x.shape
    assert (B, C, H, W) == (2, 512, 64, 64)
    xt = jnp.transpose(x, (0, 2, 3, 1)).reshape(B, XCH, H * W // XCH, C)
    w1t = jnp.transpose(w1, (2, 3, 0, 1)).reshape(9, C, C)
    w2t = jnp.transpose(w2, (2, 3, 0, 1)).reshape(9, C, C)
    hbm = pl.BlockSpec(memory_space=pl.ANY)
    out = pl.pallas_call(
        _kernel,
        out_shape=jax.ShapeDtypeStruct(xt.shape, x.dtype),
        in_specs=[hbm] * 9,
        out_specs=hbm,
        scratch_shapes=[
            pltpu.VMEM(t_emb.shape, BF16),
            pltpu.VMEM(g1.shape, BF16),
            pltpu.VMEM(be1.shape, BF16),
            pltpu.VMEM(g2.shape, BF16),
            pltpu.VMEM(be2.shape, BF16),
            pltpu.VMEM((8, XCH, 4096 // XCH + 16, 128), BF16),
            pltpu.VMEM((8, 9, 512, 128), BF16),
            pltpu.VMEM(w_emb.shape, BF16),
            pltpu.VMEM((8 * 4096, 128), F32),
            pltpu.VMEM((8 * 16, 128), F32),
            pltpu.VMEM((96 * TREC, 128), F32),
            pltpu.VMEM((96 * TREC, 128), F32),
            pltpu.VMEM((96 * TREC, 128), F32),
            pltpu.VMEM((4, 36 * 256, 128), BF16),
            pltpu.VMEM((4, 36 * 256, 128), BF16),
            pltpu.VMEM((16, 36 * 128, 128), BF16),
            pltpu.VMEM((8, 36 * 128, 128), BF16),
            pltpu.VMEM((5 * MSLOT, 128), F32),
            pltpu.VMEM((16, 1, 128), F32),
            pltpu.VMEM((8, 1, 128), F32),
            pltpu.SMEM((40,), jnp.int32),
            pltpu.SemaphoreType.DMA((8,)),
            pltpu.SemaphoreType.DMA((2, XCH)),
            pltpu.SemaphoreType.DMA((3, 4)),
            pltpu.SemaphoreType.DMA((6,)),
            pltpu.SemaphoreType.DMA((7,)),
        ],
        compiler_params=pltpu.CompilerParams(vmem_limit_bytes=120 * 2**20),
        name="resblk",
    )(xt, t_emb, g1, be1, w1t, w_emb, g2, be2, w2t)
    return jnp.transpose(out.reshape(B, H, W, C), (0, 3, 1, 2))
```

```python
import itertools

import jax
import jax.numpy as jnp
import numpy as np
from jax import lax
import jax.experimental.pallas as pl
import jax.experimental.pallas.tpu as pltpu

F32 = jnp.float32
BF16 = jnp.bfloat16
U32 = jnp.uint32

PA = 2.0 / 3.0
PB = 1.5
A2, B2 = PA * PA, PB * PB
NA = 1.0 / (2 * A2 * (A2 - B2))
NB = 1.0 / (2 * B2 * (B2 - A2))
RT = PB / PA
GS = PA ** 3
ROWS = (0, 5, 1, 2, 3, 4)

TPOS = (0, 24, 32, 40, 48, 56, 64, 16)
TREC = 72
XCH = 4
MROW = 264
MSLOT = 36 * MROW
M_SLOT = (0, 1, 2, 3, 4, 0, 1, 2, 3, 4, 0, 1, 3, 4, 2, 0)
K_A2, K_B2, K_BITS, K_ZERO, K_SUM, K_SQ, K_GN = (i * MROW + 256 for i in range(7))
K_G = K_GN + 3 * MROW
C0COST, A1COST, A2COST = 38, 34, 46


def _bt(d0, d1, d2, d3, d4, d5, a2=A2, b2=B2):
    t, u = a2 * d2, b2 * d2
    ea, eb = d4 - u, d4 - t
    v0 = ea - t
    if d0 is not None:
        v0 = v0 + d0
    t3, u3 = a2 * d3, b2 * d3
    pa, pb = t3 - d1, u3 - d1
    v5 = (d5 - pa) - u3 if d5 is not None else (d1 - t3) - u3
    oa, ob = PB * pa, PA * pb
    return v0, ea + oa, ea - oa, eb + ob, eb - ob, v5


def _at(m0, m1, m2, m3, m4, m5):
    sa, ta, sb, tb = m1 + m2, m1 - m2, m3 + m4, m3 - m4
    return (m0 + sa) + sb, ta + RT * tb, sa + (RT * RT) * sb, (ta + m5) + (RT * RT * RT) * tb


def _gt(g0, g1, g2, k):
    ea, oa = (k * NA) * g0 + (k * NA * A2) * g2, (k * NA * PA) * g1
    eb, ob = (k * NB) * g0 + (k * NB * B2) * g2, (k * NB * PB) * g1
    k5 = k / PA ** 3
    u0 = g0 if abs(k - 1.0) < 1e-12 else k * g0
    u5 = g2 if abs(k5 - 1.0) < 1e-12 else k5 * g2
    return u0, ea + oa, ea - oa, eb + ob, eb - ob, u5


def _stack(top, bottom):
    return jnp.concatenate([top, bottom], axis=0).astype(BF16)


def _pair(lo, hi):
    bits = lax.bitcast_convert_type(_stack(lo, hi).astype(F32), U32)
    return (bits[:8] >> 16) | (bits[8:] & np.uint32(0xFFFF0000))


def _unpair(w, shift=16, mask=np.uint32(0xFFFF0000)):
    return lax.bitcast_convert_type(w << shift, F32), lax.bitcast_convert_type(w & mask, F32)


def _tree(xs):
    while len(xs) > 1:
        xs = [xs[i] + xs[i + 1] for i in range(0, len(xs), 2)]
    return xs[0]


def _acc(a, x):
    return x if a is None else a + x


class _Rows:
    def __init__(self, ref, base=0):
        self.ref, self.base = ref, base

    def ld(self, off, n=8, stride=1):
        return self.ref[pl.ds(self.base + off, n, stride=stride), :]

    def st(self, off, val, stride=1):
        self.ref[pl.ds(self.base + off, val.shape[0], stride=stride), :] = val


def _splitter(const):
    bits = lax.bitcast_convert_type(const.ld(K_BITS), U32)
    shift, mask = bits & 16, bits << 16
    return lambda w: _unpair(w, shift, mask)


def _job_u(w, u, const, rows):
    needed = sorted({i for row in rows for i in {0: (0,), 5: (2,)}.get(row, (0, 1, 2))})
    cost = 9 * len(needed) + sum(32 if row in (0, 5) else 100 for row in rows)

    def gen():
        if 0 in rows:
            zero = lax.bitcast_convert_type(const.ld(K_ZERO), U32)
            tap = pltpu.bitcast(w[0].ld(0, 64) | jnp.concatenate([zero] * 8, axis=0), BF16)
            u.st(0, (GS * tap.T.astype(F32)).astype(BF16))
            yield 48
        for r in range(0, 64, 8):
            zero = lax.bitcast_convert_type(const.ld(K_ZERO), U32)
            g = {}
            for i in needed:
                taps = [pltpu.bitcast(w[3 * i + j].ld(r) | zero, BF16).astype(F32) for j in range(3)]
                g[i] = [v[:8] for v in taps], [v[8:] for v in taps]

            def emit(i, vals, k):
                top, bottom = _gt(*vals[0], k), _gt(*vals[1], k)
                for j in range(0 if i else 1, 6):
                    u.st((i * 6 + j) * 128 + 2 * r, _stack(top[j], bottom[j]))

            for n, row in enumerate(rows):
                if row == 0:
                    emit(0, g[0], GS)
                elif row == 5:
                    emit(5, g[2], 1.0)
                else:
                    k0, k1, k2 = (const.ld(K_G + (3 * (row // 2) + i) * MROW) for i in range(3))
                    e = [[k0 * g[0][h][j] + k2 * g[2][h][j] for j in range(3)] for h in range(2)]
                    o = [[k1 * g[1][h][j] for j in range(3)] for h in range(2)]
                    emit(row, [[e[h][j] + o[h][j] for j in range(3)] for h in range(2)], GS)
                    emit(row + 1, [[e[h][j] - o[h][j] for j in range(3)] for h in range(2)], GS)
                yield (32 if row in (0, 5) else 100) + (9 * len(needed) if n == 0 else 0)

    return gen(), 8 * cost + (48 if 0 in rows else 0)


def _gn_coeffs(s, q, e, gamma, beta, ab):
    s = jnp.sum(s, axis=0, keepdims=True) * (1.0 / 4096)
    q = jnp.sum(q, axis=0, keepdims=True) * (1.0 / 4096)
    var_c = jnp.maximum(q - s * s, 0.0)
    mean_c = s if e is None else s + e
    mu = jnp.sum(mean_c, axis=1, keepdims=True) * (1.0 / 128)
    dev = mean_c - mu
    var = jnp.sum(var_c + dev * dev, axis=1, keepdims=True) * (1.0 / 128)
    a = 0.5 * gamma * lax.rsqrt(var + 1e-5)
    b = 0.5 * beta + a * (-mu if e is None else e - mu)
    ab.st(0, jnp.broadcast_to(a, (8, 128)))
    ab.st(8, jnp.broadcast_to(b, (8, 128)))


def _unpack_row(x, h, y, split):
    vals = [v for k in range(4) for v in split(x.ld(k, 8, 4))]
    for q, v in enumerate(vals):
        h.st(y * 64 + q * 8, v)
    return _tree(vals), _tree([v * v for v in vals])


def _job_c0(x, h, gamma, beta, ab, const):
    def gen():
        s = q = None
        for y in range(64):
            ds, dq = _unpack_row(_Rows(x[y // (64 // XCH)], (y % (64 // XCH)) * 32), h, y, _splitter(const))
            if y % 4 == 0 and y > 0:
                const.st(K_SUM, old[0])
                const.st(K_SQ, old[1])
            old = (s, q)
            s, q = _acc(s, ds), _acc(q, dq)
            yield C0COST
        _gn_coeffs(s, q, None, gamma[...], beta[...], ab)
        yield 40

    return gen(), 64 * C0COST + 40


def _job_a1(h, ab, t, const, k):
    def gen():
        scale = K_GN + k * MROW
        const.st(scale, ab.ld(0))
        b = ab.ld(8)

        def act(y, q, a):
            if y > 63:
                return None
            u = h.ld(y * 64 + q * 8) * a + b
            return u * jnp.tanh(u) + u

        for q in range(8):
            d4, d5 = None, act(0, q, const.ld(scale))
            for ty in range(16):
                a = const.ld(scale)
                d0, d1 = d4, d5
                d2, d3, d4, d5 = (act(4 * ty + k, q, a) for k in range(1, 5))
                for i, val in enumerate(_bt(d0, d1, d2, d3, d4, d5)):
                    t.st((ty * 6 + i) * TREC + TPOS[q], val)
                yield A1COST

    return gen(), 128 * A1COST


def _job_a2(t, v, const, rows):
    def gen():
        for i in rows:
            for ty in range(16):
                offs = (TPOS[7] - 1,) + TPOS + (TPOS[0] + 1,)
                d = [t.ld((ty * 6 + i) * TREC + o) for o in offs]
                a2, b2 = const.ld(K_A2), const.ld(K_B2)
                for j, (lo, hi) in enumerate(zip(_bt(*d[0:6], a2, b2), _bt(*d[4:10], a2, b2))):
                    v.st((i * 6 + j) * 256 + ty * 16, _stack(lo, hi))
                yield A2COST

    return gen(), 16 * len(rows) * A2COST


def _tiles_out(m, r0, finish, cost):
    def row(i):
        return _at(*[m.ld((i * 6 + j) * MROW + r0) for j in range(6)])

    def done(i, ys):
        finish(i, [y if i + j == 3 else (PA ** (i + j) / GS) * y for j, y in enumerate(ys)])

    r1 = row(1)
    yield 13
    r2 = row(2)
    sa, ta = [x + y for x, y in zip(r1, r2)], [x - y for x, y in zip(r1, r2)]
    yield 21
    r3 = row(3)
    yield 13
    r4 = row(4)
    sb, tb = [x + y for x, y in zip(r3, r4)], [x - y for x, y in zip(r3, r4)]
    done(1, [x + RT * y for x, y in zip(ta, tb)])
    yield 32 + cost
    done(2, [x + (RT * RT) * y for x, y in zip(sa, sb)])
    done(0, [(x + y) + w for x, y, w in zip(sa, sb, row(0))])
    yield 35 + 2 * cost
    done(3, [(x + (RT * RT * RT) * y) + w for x, y, w in zip(ta, tb, row(5))])
    yield 28 + cost


def _job_c1(m, h, e, gamma, beta, ab):
    def gen():
        sq = [None, None]
        for ty in range(16):
            for sub in range(2):
                def finish(i, ys):
                    sq[0] = _acc(sq[0], _tree(ys))
                    sq[1] = _acc(sq[1], _tree([y * y for y in ys]))
                    for j in range(4):
                        h.st((4 * ty + i) * 64 + (4 * sub + j) * 8, ys[j])

                before = tuple(sq)
                for n, cost in enumerate(_tiles_out(m, ty * 16 + sub * 8, finish, 12)):
                    if n == 1 and before[0] is not None:
                        m.st(K_SUM, before[0])
                        m.st(K_SQ, before[1])
                    yield cost
        _gn_coeffs(sq[0], sq[1], e[...], gamma[...], beta[...], ab)
        yield 40

    return gen(), 32 * (142 + 48) + 40


def _residual_out(m, x):
    for ty in range(16 // XCH):
        for sub in range(2):
            def finish(i, ys):
                for k in range(2):
                    off = (4 * ty + i) * 32 + 2 * sub + k
                    lo, hi = _unpair(x.ld(off, 8, 4))
                    x.st(off, _pair(lo + ys[2 * k], hi + ys[2 * k + 1]), 4)

            yield from _tiles_out(m, ty * 16 + sub * 8, finish, 18)


def _job_c2(m, x):
    return _residual_out(m, x), (32 // XCH) * (142 + 72)


def _timed(job, factor):
    return (cost * factor for cost in job[0]), job[1] * factor


def _run(*jobs):
    for gen, _ in jobs:
        for _ in gen:
            pass


def _step(v, u, m, jobs, add=False, tile_rows=ROWS, tiles=(0, 256), rows=16, tail=5, between=lambda xi: None):
    total = sum(c for _, c in jobs)
    pieces = itertools.chain(*[g for g, _ in jobs])
    first, count = tiles
    span = len(tile_rows) * 6 * count // rows - tail
    lead = 7 * total / span
    spent = 0

    def advance(limit):
        nonlocal spent
        while spent < limit:
            cost = next(pieces, None)
            if cost is None:
                return
            spent += cost

    tick = 0
    advance(lead)
    for xi in (6 * i + j for i in tile_rows for j in range(6)):
        lhs = jnp.concatenate([pltpu.bitcast(r.ld(xi * 128 + first // 2, count // 2), BF16) for r in v], axis=1)
        k = 1 if xi else 0
        rhs = jnp.concatenate(
            [jnp.concatenate([pltpu.bitcast(r.ld(xi * 64, 64), BF16) for r in un], axis=k) for un in u], axis=1 - k)
        res = lax.dot_general(lhs, rhs, (((1,), (k,)), ((), ())), preferred_element_type=F32)
        between(xi)
        for r in range(0, count, rows):
            for n, mn in enumerate(m):
                val = res[r:r + rows, n * 128:(n + 1) * 128]
                at = xi * MROW + first + r
                mn.st(at, val + mn.ld(at, rows) if add else val)
            tick += 1
            advance(lead + (total - lead) * tick / span)
    advance(float("inf"))


def _kernel(x_hbm, t_hbm, g1_hbm, be1_hbm, w1_hbm, we_hbm, g2_hbm, be2_hbm, w2_hbm, o_hbm,
            xbuf, wbuf, webuf, hbuf, abuf, t0, t1, t2, v0, v1, u1, u2, mbuf, par, emb,
            t_ref, g1_ref, be1_ref, g2_ref, be2_ref, slots,
            xsem, csem, wsem, psem, osem):

    def x_words(j, c):
        return xbuf.at[j, c].bitcast(U32)

    def words(ref, k):
        return _Rows(ref.at[k].bitcast(U32))

    body = pl.ds(0, 4096 // XCH)

    def lanes(g):
        return pl.ds(g * 128 if isinstance(g, int) else pl.multiple_of(g * 128, 128), 128)

    def x_copy(j):
        return pltpu.make_async_copy(x_hbm.at[j // 4, :, :, lanes(j % 4)], xbuf.at[j, :, body], xsem.at[j])

    def x_chunk_copy(j, c):
        return pltpu.make_async_copy(x_hbm.at[0, c, :, lanes(j)], xbuf.at[j, c, body], csem.at[j, c])

    def o_copy(b, g):
        return pltpu.make_async_copy(xbuf.at[b * 4 + g, :, body], o_hbm.at[b, :, :, lanes(g)], osem.at[b * 4 + g])

    def o_chunk_copy(c):
        return pltpu.make_async_copy(xbuf.at[7, c, body], o_hbm.at[1, c, :, lanes(3)], csem.at[0, c])

    def w1_copy(out_half, c):
        rows = pl.ds(out_half * 256, 256)
        return pltpu.make_async_copy(w1_hbm.at[:, rows, lanes(c)], wbuf.at[c, :, rows], wsem.at[out_half, c])

    def w1_copies(out_half, in_half):
        return [w1_copy(out_half, 2 * in_half + c) for c in range(2)]

    def w2_copies(cs):
        return [pltpu.make_async_copy(w2_hbm.at[:, :, lanes(c)], wbuf.at[4 + c], wsem.at[2, c]) for c in cs]

    def p_copies(ks):
        pairs = ((g1_hbm, g1_ref), (be1_hbm, be1_ref), (g2_hbm, g2_ref), (be2_hbm, be2_ref), (t_hbm, t_ref))
        return [pltpu.make_async_copy(*pairs[k], psem.at[k]) for k in ks]

    def e_copies():
        return [pltpu.make_async_copy(we_hbm.at[:, lanes(g)], webuf.at[g], wsem.at[3, g]) for g in range(4)]

    def start(copies):
        for cp in copies:
            cp.start()

    def wait(copies):
        for cp in copies:
            cp.wait()

    def load_params(ks):
        wait(p_copies(ks))
        for k in ks:
            val = (g1_ref, be1_ref, g2_ref, be2_ref)[k][...].astype(F32).reshape(4, 128)
            for g in range(4):
                par[k * 4 + g] = val[g:g + 1]

    start(p_copies((0, 1)))

    @pl.loop(0, 2 * XCH)
    def _(i):
        x_chunk_copy(i // XCH, i % XCH).start()

    @pl.loop(0, 2)
    def _(c):
        w1_copy(0, c).start()

    for t in (t0, t1, t2):
        for r in range(96):
            _Rows(t).st(r * TREC + 8, jnp.zeros((8, 128), F32))
    for k, slot in enumerate(M_SLOT):
        slots[k] = slot * MSLOT
        slots[16 + k] = slot * MSLOT
    for j in range(8):
        slots[32 + j] = j * 4096
    fixed = _Rows(mbuf)
    fixed.st(K_A2, jnp.full((8, 128), A2, F32))
    fixed.st(K_B2, jnp.full((8, 128), B2, F32))
    fixed.st(K_BITS, lax.bitcast_convert_type(jnp.full((8, 128), 0x3F80FFFF, U32), F32))
    for i, value in enumerate((NA, NA * PA, NA * A2, NB, NB * PB, NB * B2)):
        fixed.st(K_G + i * MROW, jnp.full((8, 128), value, F32))
    fixed.st(K_ZERO, jnp.zeros((8, 128), F32))

    def m_in(k):
        return _Rows(mbuf, pl.multiple_of(slots[k], 8))

    def m_out(k, count=1):
        base = pl.multiple_of(slots[16 + k], 8)
        return [_Rows(mbuf, base + i * MSLOT) for i in range(count)]

    def h_slot(j, conv):
        return _Rows(hbuf, pl.multiple_of(slots[32 + j], 8) if conv else j * 4096)

    def ab_slot(j):
        return _Rows(abuf, j * 16)

    def taps(conv, n, c):
        return [_Rows(wbuf.at[conv * 4 + c, k, lanes(n)].bitcast(U32)) for k in range(9)]

    every = [(0, 1), (5, 3)]

    def u1_jobs(blocks, rows, const):
        return [_job_u(taps(0, n, c), _Rows(u1.at[n * 4 + c]), const, row) for n, c in blocks for row in rows]

    def u2_jobs(u, n, cs):
        return [_job_u(taps(1, n, c), _Rows(u.at[n * 4 + c]), const, row) for c in cs for row in every]

    def quad(out_half, in_half):
        return [(2 * out_half + n, 2 * in_half + c) for n in range(2) for c in range(2)]

    def c0(j):
        x = [x_words(j, c) for c in range(XCH)]
        return _job_c0(x, h_slot(j, 0), par.at[j % 4], par.at[4 + j % 4], ab_slot(j), const)

    def a1(j, k, conv=1):
        return _job_a1(h_slot(j, conv), ab_slot(j), _Rows((t0, t1, t2)[k]), const, k)

    def a2(v, g, k, rows=ROWS):
        return _job_a2(_Rows((t0, t1, t2)[k]), _Rows(v.at[g]), const, rows)

    def c1(j):
        return _job_c1(m_in(j), h_slot(j, 1), emb.at[j], par.at[8 + j % 4], par.at[12 + j % 4], ab_slot(j))

    def c2(j, c):
        m = m_in(8 + j)
        return _job_c2(_Rows(mbuf, m.base + c * (256 // XCH)), _Rows(x_words(j, c)))

    def block(fn):
        pl.when(slots[0] == 0)(fn)

    def half_step(out_half, in_half, jobs, tile_rows=ROWS, rows=8, tail=8):
        ins = (2 * in_half, 2 * in_half + 1)
        outs = (2 * out_half, 2 * out_half + 1)
        block(lambda: _step([words(v0, c) for c in ins], [[words(u1, n * 4 + c) for c in ins] for n in outs],
                            m_out(outs[0], 2), jobs, add=bool(in_half), tile_rows=tile_rows, rows=rows, tail=tail))

    def step(slot, v, u, n, jobs, **kwargs):
        block(lambda: _step([words(v, c) for c in range(4)], [[words(u, n * 4 + c) for c in range(4)]],
                            m_out(slot), jobs, **kwargs))

    @pl.loop(0, 2)
    def _(j):
        def unpack_chunk(c, sums):
            x_chunk_copy(j, c).wait()
            h = _Rows(hbuf, j * 4096 + c * (4096 // XCH))
            s, q = sums
            for y in range(64 // XCH):
                ds, dq = _unpack_row(_Rows(x_words(j, c), y * 32), h, y, _unpair)
                s, q = s + ds, q + dq
            return s, q

        s, q = lax.fori_loop(0, XCH, unpack_chunk, (jnp.zeros((8, 128), F32),) * 2)

        @pl.when(j == 0)
        def _():
            load_params((0, 1))
            x_copy(2).start()
            _gn_coeffs(s, q, None, par[0], par[4], ab_slot(0))

        @pl.when(j == 1)
        def _():
            _gn_coeffs(s, q, None, par[1], par[5], ab_slot(1))
            _run(_job_a2(_Rows(t0), _Rows(v0.at[0]), fixed, ROWS[4:]))

        _run(_job_a1(h_slot(j, 0), ab_slot(j), _Rows(t0), fixed, 0),
             _job_a2(_Rows(t0), _Rows(v0.at[j]), fixed, ROWS[:4]))

        @pl.when(j == 0)
        def _():
            start(w1_copies(1, 0))

    @pl.loop(0, 2)
    def _(c):
        w1_copy(0, c).wait()
        _run(*u1_jobs([(0, c), (1, c)], [(0, 5)], fixed))

    const = m_in(0)

    def u1_block(out_half, in_half, k, time, rows=every):
        return [_timed(job, time) for job in u1_jobs([quad(out_half, in_half)[k]], rows, const)]

    start([x_copy(3)] + w1_copies(0, 1))
    half_step(0, 0, [job for k in (2, 1, 3) for job in u1_block(0, 0, k, 1.075, [(1,)])] + [a2(v0, 1, 0, ROWS[4:])]
              + u1_block(0, 0, 0, 1.075, [(1,), (3,)]) + u1_block(0, 0, 1, 1.075, [(3,)]), ROWS[:2], tail=4)
    wait([x_copy(2)])
    start(w1_copies(1, 1) + [x_copy(j) for j in range(4, 8)])
    half_step(0, 0, [_timed(c0(2), 0.94)] + u1_jobs(quad(0, 0)[2:], [(3,)], const), ROWS[2:3], rows=16, tail=4)
    wait(w1_copies(1, 0))
    half_step(0, 0, [job for k in (2, 3, 1) for job in u1_block(1, 0, k, 0.88)] + [a1(2, 1, 0)]
              + u1_block(1, 0, 0, 0.88), ROWS[3:], tail=4)
    wait([x_copy(3)] + w1_copies(0, 1))
    half_step(1, 0, [_timed(c0(3), 0.83)] + u1_block(0, 1, 0, 1) + [_timed(a1(3, 0, 0), 1.14)] + u1_block(0, 1, 1, 1)
              + [_timed(a2(v0, 3, 0), 0.94)] + u1_block(0, 1, 3, 1) + [_timed(a2(v0, 2, 1), 0.94)]
              + u1_block(0, 1, 2, 1), tail=6)
    wait(w1_copies(1, 1) + [x_copy(j) for j in range(4, 8)])
    start(p_copies((2, 3, 4)) + e_copies() + w2_copies((0, 1)))
    half_step(0, 1, [c0(5), c0(4)] + u1_block(1, 1, 1, 1.14) + u1_block(1, 1, 0, 1.14) + [c0(6)]
              + u1_block(1, 1, 2, 1.14) + [c0(7)] + u1_block(1, 1, 3, 1.14) + [a1(4, 1, 0)])
    half_step(1, 1, [_timed(a2(v1, 0, 1), 1.14), _timed(a1(5, 0, 0), 0.94), _timed(a2(v1, 1, 0, ROWS[:3]), 1.14),
                     _timed(a1(6, 1, 0), 0.94), _timed(a1(7, 2, 0), 0.94), _timed(a2(v1, 2, 1, ROWS[:3]), 1.14),
                     _timed(a2(v1, 3, 2, ROWS[:3]), 1.14)], tail=4)

    load_params((2, 3))
    wait(p_copies((4,)) + e_copies() + w2_copies((0, 1)))
    start(w2_copies((2, 3)))

    partial = []

    def embed(xi):
        k = len(partial)
        if k * 128 < t_ref.shape[1]:
            th = t_ref[:, lanes(k)].astype(F32) * 0.5
            zero = jnp.concatenate([lax.bitcast_convert_type(const.ld(K_ZERO), U32)] * 8, axis=0)
            we = jnp.concatenate([pltpu.bitcast(words(webuf, g).ld(k * 64, 64) | zero, BF16) for g in range(4)], axis=1)
            part = jnp.dot((th * jnp.tanh(th) + th).astype(BF16), we, preferred_element_type=F32)
            partial.append(partial[-1] + part if partial else part)
            if (k + 1) * 128 == t_ref.shape[1]:
                for j in range(8):
                    emb[j] = partial[-1][j // 4:j // 4 + 1, (j % 4) * 128:(j % 4 + 1) * 128]

    step(4, v1, u1, 0, [a2(v1, 1 + k, k, (i,)) for i in ROWS[3:] for k in range(3)] + [c1(0), c1(1)]
         + u2_jobs(u2, 0, (0, 1)), between=embed)
    wait(w2_copies((2, 3)))
    step(5, v1, u1, 1, [a1(0, 0), a2(v0, 0, 0), c1(2), c1(3)] + u2_jobs(u2, 0, (2, 3)))
    step(6, v1, u1, 2, [a1(1, 1), a2(v0, 1, 1), a1(2, 2), a2(v0, 2, 2), c1(4), (iter([500]), 500)])
    step(7, v1, u1, 3, [a1(3, 0), a2(v0, 3, 0), c1(5)] + u2_jobs(u2, 1, range(4)))

    @pl.loop(0, 2)
    def _(n):
        step(8 + n, v0, u2, n, [a1(4 + n, 1), a2(v1, n, 1), c1(6 + n)] + u2_jobs(u1, 2 + n, range(4)))

    @pl.loop(2, 4)
    def _(n):
        step(8 + n, v0, u1, n, [a1(4 + n, 0), a2(v1, n, 0)] + [c2(n - 2, c) for c in range(XCH)])
        o_copy(0, n - 2).start()

    step(14, v1, u1, 2, [c2(j, c) for j in (2, 3) for c in range(XCH)])
    start([o_copy(0, 2), o_copy(0, 3)])

    @pl.loop(0, 2)
    def _(n):
        done = 2 - 2 * n
        step(12 + n, v1, u2, n, [c2(4 + done, c) for c in range(XCH)])
        o_copy(1, done).start()

    step(15, v1, u1, 3, [c2(5, c) for c in range(XCH)], tiles=(0, 128))
    o_copy(1, 1).start()
    step(15, v1, u1, 3, [c2(7, 0), c2(7, 1)], tiles=(128, 64))
    start([o_chunk_copy(0), o_chunk_copy(1)])
    step(15, v1, u1, 3, [c2(7, 2)], tiles=(192, 64))
    o_chunk_copy(2).start()
    _run(c2(7, 3))
    o_chunk_copy(3).start()

    wait([o_copy(j // 4, j % 4) for j in range(7)] + [o_chunk_copy(c) for c in range(XCH)])


@jax.jit
def pallas_standalone__adm_resblock__diffusion_kernel(
    x: jax.Array,
    t_emb: jax.Array,
    g1: jax.Array,
    be1: jax.Array,
    w1: jax.Array,
    w_emb: jax.Array,
    g2: jax.Array,
    be2: jax.Array,
    w2: jax.Array,
):
    B, C, H, W = x.shape
    assert (B, C, H, W) == (2, 512, 64, 64)
    xt = jnp.transpose(x, (0, 2, 3, 1)).reshape(B, XCH, H * W // XCH, C)
    w1t = jnp.transpose(w1, (2, 3, 0, 1)).reshape(9, C, C)
    w2t = jnp.transpose(w2, (2, 3, 0, 1)).reshape(9, C, C)
    hbm = pl.BlockSpec(memory_space=pl.ANY)
    out = pl.pallas_call(
        _kernel,
        out_shape=jax.ShapeDtypeStruct(xt.shape, x.dtype),
        in_specs=[hbm] * 9,
        out_specs=hbm,
        scratch_shapes=[
            pltpu.VMEM((8, XCH, 4096 // XCH + 16, 128), BF16),
            pltpu.VMEM((8, 9, 512, 128), BF16),
            pltpu.VMEM((4, w_emb.shape[0], 128), BF16),
            pltpu.VMEM((8 * 4096, 128), F32),
            pltpu.VMEM((8 * 16, 128), F32),
            pltpu.VMEM((96 * TREC, 128), F32),
            pltpu.VMEM((96 * TREC, 128), F32),
            pltpu.VMEM((96 * TREC, 128), F32),
            pltpu.VMEM((4, 36 * 256, 128), BF16),
            pltpu.VMEM((4, 36 * 256, 128), BF16),
            pltpu.VMEM((16, 36 * 128, 128), BF16),
            pltpu.VMEM((8, 36 * 128, 128), BF16),
            pltpu.VMEM((5 * MSLOT, 128), F32),
            pltpu.VMEM((16, 1, 128), F32),
            pltpu.VMEM((8, 1, 128), F32),
            pltpu.VMEM(t_emb.shape, BF16),
            pltpu.VMEM(g1.shape, BF16),
            pltpu.VMEM(be1.shape, BF16),
            pltpu.VMEM(g2.shape, BF16),
            pltpu.VMEM(be2.shape, BF16),
            pltpu.SMEM((40,), jnp.int32),
            pltpu.SemaphoreType.DMA((8,)),
            pltpu.SemaphoreType.DMA((2, XCH)),
            pltpu.SemaphoreType.DMA((4, 4)),
            pltpu.SemaphoreType.DMA((5,)),
            pltpu.SemaphoreType.DMA((7,)),
        ],
        compiler_params=pltpu.CompilerParams(vmem_limit_bytes=120 * 2**20),
        name="resblk",
    )(xt, t_emb, g1, be1, w1t, w_emb, g2, be2, w2t)
    return jnp.transpose(out.reshape(B, H, W, C), (0, 3, 1, 2))
```

```python
import itertools

import jax
import jax.numpy as jnp
import numpy as np
from jax import lax
import jax.experimental.pallas as pl
import jax.experimental.pallas.tpu as pltpu

F32 = jnp.float32
BF16 = jnp.bfloat16
U32 = jnp.uint32

PA = 2.0 / 3.0
PB = 1.5
A2, B2 = PA * PA, PB * PB
NA = 1.0 / (2 * A2 * (A2 - B2))
NB = 1.0 / (2 * B2 * (B2 - A2))
RT = PB / PA
GS = PA ** 3
ROWS = (0, 5, 1, 2, 3, 4)

TPOS = (0, 24, 32, 40, 48, 56, 64, 16)
TREC = 72
XCH = 4
MROW = 264
MSLOT = 36 * MROW
M_SLOT = (0, 1, 2, 3, 4, 0, 1, 2, 3, 4, 0, 1, 3, 4, 2, 0)
K_A2, K_B2, K_BITS, K_ZERO, K_SUM, K_SQ, K_GN = (i * MROW + 256 for i in range(7))
K_G = K_GN + 3 * MROW
C0COST, A1COST, A2COST = 44, 34, 46


def _bt(d0, d1, d2, d3, d4, d5, a2=A2, b2=B2):
    t, u = a2 * d2, b2 * d2
    ea, eb = d4 - u, d4 - t
    v0 = ea - t
    if d0 is not None:
        v0 = v0 + d0
    t3, u3 = a2 * d3, b2 * d3
    pa, pb = t3 - d1, u3 - d1
    v5 = (d5 - pa) - u3 if d5 is not None else (d1 - t3) - u3
    oa, ob = PB * pa, PA * pb
    return v0, ea + oa, ea - oa, eb + ob, eb - ob, v5


def _at(m0, m1, m2, m3, m4, m5):
    sa, ta, sb, tb = m1 + m2, m1 - m2, m3 + m4, m3 - m4
    return (m0 + sa) + sb, ta + RT * tb, sa + (RT * RT) * sb, (ta + m5) + (RT * RT * RT) * tb


def _gt(g0, g1, g2, k):
    ea, oa = (k * NA) * g0 + (k * NA * A2) * g2, (k * NA * PA) * g1
    eb, ob = (k * NB) * g0 + (k * NB * B2) * g2, (k * NB * PB) * g1
    k5 = k / PA ** 3
    u0 = g0 if abs(k - 1.0) < 1e-12 else k * g0
    u5 = g2 if abs(k5 - 1.0) < 1e-12 else k5 * g2
    return u0, ea + oa, ea - oa, eb + ob, eb - ob, u5


def _stack(top, bottom):
    return jnp.concatenate([top, bottom], axis=0).astype(BF16)


def _pair(lo, hi):
    bits = lax.bitcast_convert_type(_stack(lo, hi).astype(F32), U32)
    return (bits[:8] >> 16) | (bits[8:] & np.uint32(0xFFFF0000))


def _unpair(w, shift=16, mask=np.uint32(0xFFFF0000)):
    return lax.bitcast_convert_type(w << shift, F32), lax.bitcast_convert_type(w & mask, F32)


def _tree(xs):
    while len(xs) > 1:
        xs = [xs[i] + xs[i + 1] for i in range(0, len(xs), 2)]
    return xs[0]


def _acc(a, x):
    return x if a is None else a + x


class _Rows:
    def __init__(self, ref, base=0):
        self.ref, self.base = ref, base

    def ld(self, off, n=8, stride=1):
        return self.ref[pl.ds(self.base + off, n, stride=stride), :]

    def st(self, off, val, stride=1):
        self.ref[pl.ds(self.base + off, val.shape[0], stride=stride), :] = val


def _splitter(const):
    bits = lax.bitcast_convert_type(const.ld(K_BITS), U32)
    shift, mask = bits & 16, bits << 16
    return lambda w: _unpair(w, shift, mask)


def _job_u(w, u, const, rows):
    needed = sorted({i for row in rows for i in {0: (0,), 5: (2,)}.get(row, (0, 1, 2))})
    cost = 9 * len(needed) + sum(32 if row in (0, 5) else 100 for row in rows)

    def gen():
        if 0 in rows:
            zero = lax.bitcast_convert_type(const.ld(K_ZERO), U32)
            tap = pltpu.bitcast(w[0].ld(0, 64) | jnp.concatenate([zero] * 8, axis=0), BF16)
            u.st(0, (GS * tap.T.astype(F32)).astype(BF16))
            yield 48
        for r in range(0, 64, 8):
            zero = lax.bitcast_convert_type(const.ld(K_ZERO), U32)
            g = {}
            for i in needed:
                taps = [pltpu.bitcast(w[3 * i + j].ld(r) | zero, BF16).astype(F32) for j in range(3)]
                g[i] = [v[:8] for v in taps], [v[8:] for v in taps]

            def emit(i, vals, k):
                top, bottom = _gt(*vals[0], k), _gt(*vals[1], k)
                for j in range(0 if i else 1, 6):
                    u.st((i * 6 + j) * 128 + 2 * r, _stack(top[j], bottom[j]))

            for n, row in enumerate(rows):
                if row == 0:
                    emit(0, g[0], GS)
                elif row == 5:
                    emit(5, g[2], 1.0)
                else:
                    k0, k1, k2 = (const.ld(K_G + (3 * (row // 2) + i) * MROW) for i in range(3))
                    e = [[k0 * g[0][h][j] + k2 * g[2][h][j] for j in range(3)] for h in range(2)]
                    o = [[k1 * g[1][h][j] for j in range(3)] for h in range(2)]
                    emit(row, [[e[h][j] + o[h][j] for j in range(3)] for h in range(2)], GS)
                    emit(row + 1, [[e[h][j] - o[h][j] for j in range(3)] for h in range(2)], GS)
                yield (32 if row in (0, 5) else 100) + (9 * len(needed) if n == 0 else 0)

    return gen(), 8 * cost + (48 if 0 in rows else 0)


def _shifted_sums(vals, pivot):
    dev = [v - pivot for v in vals]
    return _tree(dev), _tree([d * d for d in dev])


def _gn_coeffs(pivot, s, q, e, gamma, beta, ab):
    def mean(x):
        return jnp.sum(jnp.sum(x, axis=0, keepdims=True), axis=1, keepdims=True) * (1.0 / 1024)

    s, q = s * (1.0 / 512), q * (1.0 / 512)
    part_var = jnp.maximum(q - s * s, 0.0)
    part_mean = pivot + s if e is None else (pivot + s) + e
    mu = mean(part_mean)
    dev = part_mean - mu
    a = 0.5 * gamma * lax.rsqrt(mean(part_var + dev * dev) + 1e-5)
    b = 0.5 * beta + a * (-mu if e is None else e - mu)
    ab.st(0, jnp.broadcast_to(a, (8, 128)))
    ab.st(8, jnp.broadcast_to(b, (8, 128)))


def _unpack_row(x, h, y, split):
    vals = [v for k in range(4) for v in split(x.ld(k, 8, 4))]
    for q, v in enumerate(vals):
        h.st(y * 64 + q * 8, v)
    return vals


def _job_c0(x, h, gamma, beta, ab, const):
    def gen():
        s = q = None
        for y in range(64):
            vals = _unpack_row(_Rows(x[y // (64 // XCH)], (y % (64 // XCH)) * 32), h, y, _splitter(const))
            if y == 0:
                pivot = vals[0]
            ds, dq = _shifted_sums(vals, pivot)
            if y % 4 == 0 and y > 0:
                const.st(K_SUM, old[0])
                const.st(K_SQ, old[1])
            old = (s, q)
            s, q = _acc(s, ds), _acc(q, dq)
            yield C0COST
        _gn_coeffs(pivot, s, q, None, gamma[...], beta[...], ab)
        yield 40

    return gen(), 64 * C0COST + 40


def _job_a1(h, ab, t, const, k):
    def gen():
        scale = K_GN + k * MROW
        const.st(scale, ab.ld(0))
        b = ab.ld(8)

        def act(y, q, a):
            if y > 63:
                return None
            u = h.ld(y * 64 + q * 8) * a + b
            return u * jnp.tanh(u) + u

        for q in range(8):
            d4, d5 = None, act(0, q, const.ld(scale))
            for ty in range(16):
                a = const.ld(scale)
                d0, d1 = d4, d5
                d2, d3, d4, d5 = (act(4 * ty + k, q, a) for k in range(1, 5))
                for i, val in enumerate(_bt(d0, d1, d2, d3, d4, d5)):
                    t.st((ty * 6 + i) * TREC + TPOS[q], val)
                yield A1COST

    return gen(), 128 * A1COST


def _job_a2(t, v, const, rows):
    def gen():
        for i in rows:
            for ty in range(16):
                offs = (TPOS[7] - 1,) + TPOS + (TPOS[0] + 1,)
                d = [t.ld((ty * 6 + i) * TREC + o) for o in offs]
                a2, b2 = const.ld(K_A2), const.ld(K_B2)
                for j, (lo, hi) in enumerate(zip(_bt(*d[0:6], a2, b2), _bt(*d[4:10], a2, b2))):
                    v.st((i * 6 + j) * 256 + ty * 16, _stack(lo, hi))
                yield A2COST

    return gen(), 16 * len(rows) * A2COST


def _tiles_out(m, r0, finish, cost):
    def row(i):
        return _at(*[m.ld((i * 6 + j) * MROW + r0) for j in range(6)])

    def done(i, ys):
        finish(i, [y if i + j == 3 else (PA ** (i + j) / GS) * y for j, y in enumerate(ys)])

    r1 = row(1)
    yield 13
    r2 = row(2)
    sa, ta = [x + y for x, y in zip(r1, r2)], [x - y for x, y in zip(r1, r2)]
    yield 21
    r3 = row(3)
    yield 13
    r4 = row(4)
    sb, tb = [x + y for x, y in zip(r3, r4)], [x - y for x, y in zip(r3, r4)]
    done(1, [x + RT * y for x, y in zip(ta, tb)])
    yield 32 + cost
    done(2, [x + (RT * RT) * y for x, y in zip(sa, sb)])
    done(0, [(x + y) + w for x, y, w in zip(sa, sb, row(0))])
    yield 35 + 2 * cost
    done(3, [(x + (RT * RT * RT) * y) + w for x, y, w in zip(ta, tb, row(5))])
    yield 28 + cost


def _job_c1(m, h, e, gamma, beta, ab):
    def gen():
        sq = [None, None]
        pivot = []
        for ty in range(16):
            for sub in range(2):
                def finish(i, ys):
                    if not pivot:
                        pivot.append(ys[0])
                    ds, dq = _shifted_sums(ys, pivot[0])
                    sq[:] = _acc(sq[0], ds), _acc(sq[1], dq)
                    for j in range(4):
                        h.st((4 * ty + i) * 64 + (4 * sub + j) * 8, ys[j])

                before = tuple(sq)
                for n, cost in enumerate(_tiles_out(m, ty * 16 + sub * 8, finish, 16)):
                    if n == 1 and before[0] is not None:
                        m.st(K_SUM, before[0])
                        m.st(K_SQ, before[1])
                    yield cost
        _gn_coeffs(pivot[0], sq[0], sq[1], e[...], gamma[...], beta[...], ab)
        yield 40

    return gen(), 32 * (142 + 64) + 40


def _residual_out(m, x):
    for ty in range(16 // XCH):
        for sub in range(2):
            def finish(i, ys):
                for k in range(2):
                    off = (4 * ty + i) * 32 + 2 * sub + k
                    lo, hi = _unpair(x.ld(off, 8, 4))
                    x.st(off, _pair(lo + ys[2 * k], hi + ys[2 * k + 1]), 4)

            yield from _tiles_out(m, ty * 16 + sub * 8, finish, 18)


def _job_c2(m, x):
    return _residual_out(m, x), (32 // XCH) * (142 + 72)


def _timed(job, factor):
    return (cost * factor for cost in job[0]), job[1] * factor


def _run(*jobs):
    for gen, _ in jobs:
        for _ in gen:
            pass


def _step(v, u, m, jobs, add=False, tile_rows=ROWS, tiles=(0, 256), rows=16, tail=5, between=lambda xi: None):
    total = sum(c for _, c in jobs)
    pieces = itertools.chain(*[g for g, _ in jobs])
    first, count = tiles
    span = len(tile_rows) * 6 * count // rows - tail
    lead = 7 * total / span
    spent = 0

    def advance(limit):
        nonlocal spent
        while spent < limit:
            cost = next(pieces, None)
            if cost is None:
                return
            spent += cost

    tick = 0
    advance(lead)
    for xi in (6 * i + j for i in tile_rows for j in range(6)):
        lhs = jnp.concatenate([pltpu.bitcast(r.ld(xi * 128 + first // 2, count // 2), BF16) for r in v], axis=1)
        k = 1 if xi else 0
        rhs = jnp.concatenate(
            [jnp.concatenate([pltpu.bitcast(r.ld(xi * 64, 64), BF16) for r in un], axis=k) for un in u], axis=1 - k)
        res = lax.dot_general(lhs, rhs, (((1,), (k,)), ((), ())), preferred_element_type=F32)
        between(xi)
        for r in range(0, count, rows):
            for n, mn in enumerate(m):
                val = res[r:r + rows, n * 128:(n + 1) * 128]
                at = xi * MROW + first + r
                mn.st(at, val + mn.ld(at, rows) if add else val)
            tick += 1
            advance(lead + (total - lead) * tick / span)
    advance(float("inf"))


def _kernel(x_hbm, t_hbm, g1_hbm, be1_hbm, w1_hbm, we_hbm, g2_hbm, be2_hbm, w2_hbm, o_hbm,
            xbuf, wbuf, webuf, hbuf, abuf, t0, t1, t2, v0, v1, u1, u2, mbuf, par, emb,
            t_ref, g1_ref, be1_ref, g2_ref, be2_ref, slots,
            xsem, csem, wsem, psem, osem):

    def x_words(j, c):
        return xbuf.at[j, c].bitcast(U32)

    def words(ref, k):
        return _Rows(ref.at[k].bitcast(U32))

    body = pl.ds(0, 4096 // XCH)

    def lanes(g):
        return pl.ds(g * 128 if isinstance(g, int) else pl.multiple_of(g * 128, 128), 128)

    def x_copy(j):
        return pltpu.make_async_copy(x_hbm.at[j // 4, :, :, lanes(j % 4)], xbuf.at[j, :, body], xsem.at[j])

    def x_chunk_copy(j, c):
        return pltpu.make_async_copy(x_hbm.at[0, c, :, lanes(j)], xbuf.at[j, c, body], csem.at[j, c])

    def o_copy(b, g):
        return pltpu.make_async_copy(xbuf.at[b * 4 + g, :, body], o_hbm.at[b, :, :, lanes(g)], osem.at[b * 4 + g])

    def o_chunk_copy(c):
        return pltpu.make_async_copy(xbuf.at[7, c, body], o_hbm.at[1, c, :, lanes(3)], csem.at[0, c])

    def w1_copy(out_half, c):
        rows = pl.ds(out_half * 256, 256)
        return pltpu.make_async_copy(w1_hbm.at[:, rows, lanes(c)], wbuf.at[c, :, rows], wsem.at[out_half, c])

    def w1_copies(out_half, in_half):
        return [w1_copy(out_half, 2 * in_half + c) for c in range(2)]

    def w2_copies(cs):
        return [pltpu.make_async_copy(w2_hbm.at[:, :, lanes(c)], wbuf.at[4 + c], wsem.at[2, c]) for c in cs]

    def p_copies(ks):
        pairs = ((g1_hbm, g1_ref), (be1_hbm, be1_ref), (g2_hbm, g2_ref), (be2_hbm, be2_ref), (t_hbm, t_ref))
        return [pltpu.make_async_copy(*pairs[k], psem.at[k]) for k in ks]

    def e_copies():
        return [pltpu.make_async_copy(we_hbm.at[:, lanes(g)], webuf.at[g], wsem.at[3, g]) for g in range(4)]

    def start(copies):
        for cp in copies:
            cp.start()

    def wait(copies):
        for cp in copies:
            cp.wait()

    def load_params(ks):
        wait(p_copies(ks))
        for k in ks:
            val = (g1_ref, be1_ref, g2_ref, be2_ref)[k][...].astype(F32).reshape(4, 128)
            for g in range(4):
                par[k * 4 + g] = val[g:g + 1]

    start(p_copies((0, 1)))

    @pl.loop(0, 2 * XCH)
    def _(i):
        x_chunk_copy(i // XCH, i % XCH).start()

    @pl.loop(0, 2)
    def _(c):
        w1_copy(0, c).start()

    for t in (t0, t1, t2):
        for r in range(96):
            _Rows(t).st(r * TREC + 8, jnp.zeros((8, 128), F32))
    for k, slot in enumerate(M_SLOT):
        slots[k] = slot * MSLOT
        slots[16 + k] = slot * MSLOT
    for j in range(8):
        slots[32 + j] = j * 4096
    fixed = _Rows(mbuf)
    fixed.st(K_A2, jnp.full((8, 128), A2, F32))
    fixed.st(K_B2, jnp.full((8, 128), B2, F32))
    fixed.st(K_BITS, lax.bitcast_convert_type(jnp.full((8, 128), 0x3F80FFFF, U32), F32))
    for i, value in enumerate((NA, NA * PA, NA * A2, NB, NB * PB, NB * B2)):
        fixed.st(K_G + i * MROW, jnp.full((8, 128), value, F32))
    fixed.st(K_ZERO, jnp.zeros((8, 128), F32))

    def m_in(k):
        return _Rows(mbuf, pl.multiple_of(slots[k], 8))

    def m_out(k, count=1):
        base = pl.multiple_of(slots[16 + k], 8)
        return [_Rows(mbuf, base + i * MSLOT) for i in range(count)]

    def h_slot(j, conv):
        return _Rows(hbuf, pl.multiple_of(slots[32 + j], 8) if conv else j * 4096)

    def ab_slot(j):
        return _Rows(abuf, j * 16)

    def taps(conv, n, c):
        return [_Rows(wbuf.at[conv * 4 + c, k, lanes(n)].bitcast(U32)) for k in range(9)]

    every = [(0, 1), (5, 3)]

    def u1_jobs(blocks, rows, const):
        return [_job_u(taps(0, n, c), _Rows(u1.at[n * 4 + c]), const, row) for n, c in blocks for row in rows]

    def u2_jobs(u, n, cs, time=1):
        return [_timed(_job_u(taps(1, n, c), _Rows(u.at[n * 4 + c]), const, row), time) for c in cs for row in every]

    def quad(out_half, in_half):
        return [(2 * out_half + n, 2 * in_half + c) for n in range(2) for c in range(2)]

    def c0(j):
        x = [x_words(j, c) for c in range(XCH)]
        return _job_c0(x, h_slot(j, 0), par.at[j % 4], par.at[4 + j % 4], ab_slot(j), const)

    def a1(j, k, conv=1):
        return _job_a1(h_slot(j, conv), ab_slot(j), _Rows((t0, t1, t2)[k]), const, k)

    def a2(v, g, k, rows=ROWS):
        return _job_a2(_Rows((t0, t1, t2)[k]), _Rows(v.at[g]), const, rows)

    def c1(j):
        return _job_c1(m_in(j), h_slot(j, 1), emb.at[j], par.at[8 + j % 4], par.at[12 + j % 4], ab_slot(j))

    def c2(j, c):
        m = m_in(8 + j)
        return _job_c2(_Rows(mbuf, m.base + c * (256 // XCH)), _Rows(x_words(j, c)))

    def idle(cost):
        return iter([cost]), cost

    def block(fn):
        pl.when(slots[0] == 0)(fn)

    def half_step(out_half, in_half, jobs, tile_rows=ROWS, rows=8, tail=8):
        ins = (2 * in_half, 2 * in_half + 1)
        outs = (2 * out_half, 2 * out_half + 1)
        block(lambda: _step([words(v0, c) for c in ins], [[words(u1, n * 4 + c) for c in ins] for n in outs],
                            m_out(outs[0], 2), jobs, add=bool(in_half), tile_rows=tile_rows, rows=rows, tail=tail))

    def step(slot, v, u, n, jobs, **kwargs):
        block(lambda: _step([words(v, c) for c in range(4)], [[words(u, n * 4 + c) for c in range(4)]],
                            m_out(slot), jobs, **kwargs))

    @pl.loop(0, 2)
    def _(j):
        def pivot():
            return _unpair(_Rows(x_words(j, 0)).ld(0))[0]

        def unpack_chunk(c, sums):
            x_chunk_copy(j, c).wait()
            h = _Rows(hbuf, j * 4096 + c * (4096 // XCH))
            s, q = sums
            p = pivot()
            for y in range(64 // XCH):
                ds, dq = _shifted_sums(_unpack_row(_Rows(x_words(j, c), y * 32), h, y, _unpair), p)
                s, q = s + ds, q + dq
            return s, q

        s, q = lax.fori_loop(0, XCH, unpack_chunk, (jnp.zeros((8, 128), F32),) * 2)

        @pl.when(j == 0)
        def _():
            load_params((0, 1))
            x_copy(2).start()
            _gn_coeffs(pivot(), s, q, None, par[0], par[4], ab_slot(0))

        @pl.when(j == 1)
        def _():
            _gn_coeffs(pivot(), s, q, None, par[1], par[5], ab_slot(1))
            _run(_job_a2(_Rows(t0), _Rows(v0.at[0]), fixed, ROWS[4:]))

        _run(_job_a1(h_slot(j, 0), ab_slot(j), _Rows(t0), fixed, 0),
             _job_a2(_Rows(t0), _Rows(v0.at[j]), fixed, ROWS[:4]))

        @pl.when(j == 0)
        def _():
            start(w1_copies(1, 0))

    @pl.loop(0, 2)
    def _(c):
        w1_copy(0, c).wait()
        _run(*u1_jobs([(0, c), (1, c)], [(0, 5)], fixed))

    const = m_in(0)

    def u1_block(out_half, in_half, k, time, rows=every):
        return [_timed(job, time) for job in u1_jobs([quad(out_half, in_half)[k]], rows, const)]

    start([x_copy(3)] + w1_copies(0, 1))
    half_step(0, 0, [job for k in (2, 1, 3) for job in u1_block(0, 0, k, 1.075, [(1,)])] + [a2(v0, 1, 0, ROWS[4:])]
              + u1_block(0, 0, 0, 1.075, [(1,), (3,)]) + u1_block(0, 0, 1, 1.075, [(3,)]), ROWS[:2], tail=4)
    wait([x_copy(2)])
    start(w1_copies(1, 1) + [x_copy(j) for j in range(4, 8)])
    half_step(0, 0, [_timed(c0(2), 0.83)] + u1_block(0, 0, 2, 1.06, [(3,)]) + u1_block(0, 0, 3, 1.06, [(3,)]),
              ROWS[2:3], tail=10)
    wait(w1_copies(1, 0))
    half_step(0, 0, [job for k in (2, 3, 1) for job in u1_block(1, 0, k, 0.88)] + [a1(2, 1, 0)]
              + u1_block(1, 0, 0, 0.88), ROWS[3:], tail=4)
    wait([x_copy(3)] + w1_copies(0, 1))
    half_step(1, 0, [_timed(c0(3), 0.83)] + u1_block(0, 1, 0, 1) + [_timed(a1(3, 0, 0), 1.14)] + u1_block(0, 1, 1, 1)
              + [_timed(a2(v0, 3, 0), 1.01)] + u1_block(0, 1, 3, 1) + [_timed(a2(v0, 2, 1), 1.01)]
              + u1_block(0, 1, 2, 1), tail=6)
    wait(w1_copies(1, 1) + [x_copy(j) for j in range(4, 8)])
    start(p_copies((2, 3, 4)) + e_copies() + w2_copies((0, 1)))
    half_step(0, 1, [c0(4)] + u1_block(1, 1, 0, 1.21) + [c0(5), _timed(a1(4, 1, 0), 1.14), c0(6)]
              + u1_block(1, 1, 2, 1.21) + u1_block(1, 1, 1, 1.21) + [c0(7)] + u1_block(1, 1, 3, 1.21))
    half_step(1, 1, [_timed(a2(v1, 0, 1), 1.14), _timed(a1(5, 0, 0), 0.94), _timed(a2(v1, 1, 0, ROWS[:3]), 1.14),
                     _timed(a1(6, 1, 0), 0.94), _timed(a1(7, 2, 0), 0.94), _timed(a2(v1, 2, 1, ROWS[:3]), 1.14),
                     _timed(a2(v1, 3, 2, ROWS[:3]), 1.14)], tail=4)

    load_params((2, 3))
    wait(p_copies((4,)) + e_copies() + w2_copies((0, 1)))
    start(w2_copies((2, 3)))

    partial = []

    def embed(xi):
        k = len(partial)
        if k * 128 < t_ref.shape[1]:
            th = t_ref[:, lanes(k)].astype(F32) * 0.5
            zero = jnp.concatenate([lax.bitcast_convert_type(const.ld(K_ZERO), U32)] * 8, axis=0)
            we = jnp.concatenate([pltpu.bitcast(words(webuf, g).ld(k * 64, 64) | zero, BF16) for g in range(4)], axis=1)
            part = jnp.dot((th * jnp.tanh(th) + th).astype(BF16), we, preferred_element_type=F32)
            partial.append(partial[-1] + part if partial else part)
            if (k + 1) * 128 == t_ref.shape[1]:
                for j in range(8):
                    emb[j] = partial[-1][j // 4:j // 4 + 1, (j % 4) * 128:(j % 4 + 1) * 128]

    step(4, v1, u1, 0, [a2(v1, 1 + k, k, (i,)) for i in ROWS[3:] for k in range(3)] + [_timed(c1(1), 1.06)]
         + u2_jobs(u2, 0, (0,), 0.83) + [_timed(c1(0), 1.06)] + u2_jobs(u2, 0, (1,), 0.83),
         rows=8, tail=10, between=embed)
    wait(w2_copies((2, 3)))
    step(5, v1, u1, 1, u2_jobs(u2, 0, (2,)) + [_timed(a1(0, 0), 0.94), _timed(a2(v0, 0, 0), 0.88), c1(3), c1(2)]
         + u2_jobs(u2, 0, (3,)))
    step(6, v1, u1, 2, [a1(1, 1), a2(v0, 1, 1), a1(2, 2), a2(v0, 2, 2), c1(4), idle(500)])
    step(7, v1, u1, 3, [a1(3, 0), a2(v0, 3, 0)] + u2_jobs(u2, 1, (3,)) + [_timed(c1(5), 1.22)]
         + u2_jobs(u2, 1, (1, 2, 0)), rows=8, tail=18)

    @pl.loop(0, 2)
    def _(n):
        step(8 + n, v0, u2, n, [a1(4 + n, 1), a2(v1, n, 1)] + u2_jobs(u1, 2 + n, (2,)) + [_timed(c1(6 + n), 1.12)]
             + u2_jobs(u1, 2 + n, (1, 0, 3)), rows=8, tail=10)

    @pl.loop(2, 4)
    def _(n):
        step(8 + n, v0, u1, n, [a1(4 + n, 0), a2(v1, n, 0)] + [c2(n - 2, c) for c in range(XCH)])
        o_copy(0, n - 2).start()

    step(14, v1, u1, 2, [c2(j, c) for j in (2, 3) for c in range(XCH)])
    start([o_copy(0, 2), o_copy(0, 3)])

    @pl.loop(0, 2)
    def _(n):
        done = 2 - 2 * n
        step(12 + n, v1, u2, n, [c2(4 + done, c) for c in range(XCH)])
        o_copy(1, done).start()

    step(15, v1, u1, 3, [c2(5, c) for c in range(XCH)], tiles=(0, 128))
    o_copy(1, 1).start()
    step(15, v1, u1, 3, [c2(7, 0), c2(7, 1)], tiles=(128, 64))
    start([o_chunk_copy(0), o_chunk_copy(1)])
    step(15, v1, u1, 3, [c2(7, 2)], tiles=(192, 64))
    o_chunk_copy(2).start()
    _run(c2(7, 3))
    o_chunk_copy(3).start()

    wait([o_copy(j // 4, j % 4) for j in range(7)] + [o_chunk_copy(c) for c in range(XCH)])


@jax.jit
def pallas_standalone__adm_resblock__diffusion_kernel(
    x: jax.Array,
    t_emb: jax.Array,
    g1: jax.Array,
    be1: jax.Array,
    w1: jax.Array,
    w_emb: jax.Array,
    g2: jax.Array,
    be2: jax.Array,
    w2: jax.Array,
):
    B, C, H, W = x.shape
    assert (B, C, H, W) == (2, 512, 64, 64)
    xt = jnp.transpose(x, (0, 2, 3, 1)).reshape(B, XCH, H * W // XCH, C)
    w1t = jnp.transpose(w1, (2, 3, 0, 1)).reshape(9, C, C)
    w2t = jnp.transpose(w2, (2, 3, 0, 1)).reshape(9, C, C)
    hbm = pl.BlockSpec(memory_space=pl.ANY)
    out = pl.pallas_call(
        _kernel,
        out_shape=jax.ShapeDtypeStruct(xt.shape, x.dtype),
        in_specs=[hbm] * 9,
        out_specs=hbm,
        scratch_shapes=[
            pltpu.VMEM((8, XCH, 4096 // XCH + 16, 128), BF16),
            pltpu.VMEM((8, 9, 512, 128), BF16),
            pltpu.VMEM((4, w_emb.shape[0], 128), BF16),
            pltpu.VMEM((8 * 4096, 128), F32),
            pltpu.VMEM((8 * 16, 128), F32),
            pltpu.VMEM((96 * TREC, 128), F32),
            pltpu.VMEM((96 * TREC, 128), F32),
            pltpu.VMEM((96 * TREC, 128), F32),
            pltpu.VMEM((4, 36 * 256, 128), BF16),
            pltpu.VMEM((4, 36 * 256, 128), BF16),
            pltpu.VMEM((16, 36 * 128, 128), BF16),
            pltpu.VMEM((8, 36 * 128, 128), BF16),
            pltpu.VMEM((5 * MSLOT, 128), F32),
            pltpu.VMEM((16, 1, 128), F32),
            pltpu.VMEM((8, 1, 128), F32),
            pltpu.VMEM(t_emb.shape, BF16),
            pltpu.VMEM(g1.shape, BF16),
            pltpu.VMEM(be1.shape, BF16),
            pltpu.VMEM(g2.shape, BF16),
            pltpu.VMEM(be2.shape, BF16),
            pltpu.SMEM((40,), jnp.int32),
            pltpu.SemaphoreType.DMA((8,)),
            pltpu.SemaphoreType.DMA((2, XCH)),
            pltpu.SemaphoreType.DMA((4, 4)),
            pltpu.SemaphoreType.DMA((5,)),
            pltpu.SemaphoreType.DMA((7,)),
        ],
        compiler_params=pltpu.CompilerParams(vmem_limit_bytes=120 * 2**20),
        name="resblk",
    )(xt, t_emb, g1, be1, w1t, w_emb, g2, be2, w2t)
    return jnp.transpose(out.reshape(B, H, W, C), (0, 3, 1, 2))
```
